```python
import jax
import jax.numpy as jnp

def _softmax(x, axis=-1):
    return jax.nn.softmax(x, axis=axis)
def _gelu(x):
    return jax.nn.gelu(x, approximate=True)
def _silu(x):
    return jax.nn.silu(x)
def _sigmoid(x):
    return jax.nn.sigmoid(x)
def _layernorm(x, axis=-1, eps=1e-5):
    m = jnp.mean(x, axis=axis, keepdims=True)
    v = jnp.var(x, axis=axis, keepdims=True)
    return (x - m) / jnp.sqrt(v + eps)
def _scatter_add(tgt, idx, src, axis=0):
    return tgt.at[idx].add(src)
def _segment_sum(src, seg, n):
    return jax.ops.segment_sum(src, seg, n)
class _Rng:
    def __init__(self, key):
        self._k = key
    def _next(self):
        self._k, sub = jax.random.split(self._k)
        return sub
    def normal(self, shape):
        return jax.random.normal(self._next(), shape, dtype=jnp.bfloat16)
    def randint(self, lo, hi, shape):
        return jax.random.randint(self._next(), shape, lo, hi, dtype=jnp.int32)
    def uniform(self, shape, lo=0.0, hi=1.0):
        return jax.random.uniform(self._next(), shape, jnp.bfloat16, lo, hi)
    def permutation(self, n):
        return jax.random.permutation(self._next(), n)


kernel_name = 'sequential_preLN__sliding_local_dilated__glu_gated_geglu__prompt'

def setup_inputs():
    _rng = _Rng(jax.random.key(int.from_bytes(__import__("os").urandom(4), "little")))
    _w = (lambda a: (lambda t: t.astype(jnp.bfloat16) if jnp.issubdtype(t.dtype, jnp.floating) else t)(jnp.asarray(a)))
    def _A_setup():
        B, S, D = 1, 2048, 1024
        return {
            "x": _w((lambda *s: _rng.normal(s) * 0.05)(B, S, D)),
            "wqkv": _w((lambda *s: _rng.normal(s) * 0.05)(D, 3 * D)),
            "wo": _w((lambda *s: _rng.normal(s) * 0.05)(D, D)),
        }
    _A_in = _A_setup()

    def _B_setup():
        B, S, Dm, Df = 1, 2048, 1024, 3584
        return {
            "x": _w((lambda *s: _rng.normal(s) * 0.05)(B, S, Dm)),
            "w_gate": _w((lambda *s: _rng.normal(s) * 0.05)(Dm, Df) * (Dm ** -0.5)),
            "w_up": _w((lambda *s: _rng.normal(s) * 0.05)(Dm, Df) * (Dm ** -0.5)),
            "w_down": _w((lambda *s: _rng.normal(s) * 0.05)(Df, Dm) * (Df ** -0.5)),
        }
    _B_in = _B_setup()

    return {
        "A_x": _A_in["x"],
        "A_wqkv": _A_in["wqkv"],
        "A_wo": _A_in["wo"],
        "B_x": _B_in["x"],
        "B_w_gate": _B_in["w_gate"],
        "B_w_up": _B_in["w_up"],
        "B_w_down": _B_in["w_down"],
    }

def reference(A_x, A_wqkv, A_wo, B_x, B_w_gate, B_w_up, B_w_down):
    def _A_ref(x, wqkv, wo):
        B, S, D = x.shape
        H = 32; Dh = D // H
        W, dil = 8, 2
        qkv = (lambda x, *d: x.transpose(*d))((x @ wqkv).reshape(B, S, 3, H, Dh), 2, 0, 3, 1, 4)
        q, k, v = qkv[0], qkv[1], qkv[2]
        scale = Dh ** -0.5
        pos = jnp.arange(S)
        off = jnp.arange(W) * dil
        idx = pos[:, None] - off[None, :]
        mask = idx >= 0
        idx_c = jnp.where(mask, idx, 0).reshape(-1)
        kg = k[:, :, idx_c, :].reshape(B, H, S, W, Dh)
        vg = v[:, :, idx_c, :].reshape(B, H, S, W, Dh)
        logits = jnp.einsum("bhsd,bhswd->bhsw", q, kg) * scale
        logits = jnp.where(mask[None, None, :, :], logits, -1e9)
        attn = _softmax(logits, axis=-1)
        o = jnp.einsum("bhsw,bhswd->bhsd", attn, vg)
        return (lambda x, *d: x.transpose(*d))(o, 0, 2, 1, 3).reshape(B, S, D) @ wo

    def _B_ref(x, w_gate, w_up, w_down):
        g = jnp.einsum("bsd,df->bsf", x, w_gate)
        u = jnp.einsum("bsd,df->bsf", x, w_up)
        h = _gelu(g) * u
        return jnp.einsum("bsf,fd->bsd", h, w_down)

    x = A_x
    h = x + _A_ref(_layernorm(x, axis=-1), A_wqkv, A_wo)
    h2 = h + _B_ref(_layernorm(h, axis=-1), B_w_gate, B_w_up, B_w_down)
    return h2
```

```python
import jax
import jax.numpy as jnp
from jax import lax
import jax.experimental.pallas as pl
import jax.experimental.pallas.tpu as pltpu

HEAD_DIM = 32
WINDOW = 8
DILATION = 2
HALO = 16
LANES = 128
T = 256
RB = 16
TF = 512
F32 = jnp.float32
BF16 = jnp.bfloat16


def _dot(a, b):
    return jnp.dot(a, b, preferred_element_type=F32)


def _layernorm(x):
    m = jnp.mean(x, axis=-1, keepdims=True)
    c = x - m
    v = jnp.mean(c * c, axis=-1, keepdims=True)
    return c * lax.rsqrt(v + 1e-5)


def _gelu(x):
    c = 0.7978845608028654
    hx = 0.5 * x
    return hx + hx * jnp.tanh(x * (c + (c * 0.044715) * (x * x)))


def _permute_cols(w):
    u = pltpu.bitcast(w, jnp.uint32)
    blk = lax.broadcasted_iota(jnp.int32, (u.shape[0], LANES), 1) // 4
    a = [u[:, c * LANES:(c + 1) * LANES] for c in range(8)]
    a = [pltpu.roll(a[c], 4 * c, 1) if c else a[c] for c in range(8)]
    e = [a[(-i) % 8] for i in range(8)]
    for s in (1, 2, 4):
        m = (blk & s) != 0
        e = [jnp.where(m, e[(i - s) % 8], e[i]) for i in range(8)]
    e = [pltpu.roll(e[c], LANES - 4 * c, 1) if c else e[c] for c in range(8)]
    return pltpu.bitcast(jnp.concatenate(e, axis=1), BF16)


def _permute_rows(w):
    u = pltpu.bitcast(w, jnp.uint32)
    parts = []
    for c in range(8):
        for hl in range(4):
            for cp in range(8):
                r = cp * 64 + hl * 16 + c * 2
                parts.append(u[r:r + 2, :])
    return pltpu.bitcast(jnp.concatenate(parts, axis=0), BF16)


def _kernel(x_hbm, wqkv_hbm, wo_hbm, wg_hbm, wu_hbm, wd_hbm, out_hbm,
            x_v, wqkv_v, wo_raw, wo_v, wg_v, wu_v, wd_v,
            xn_v, q_v, k_v, v_v, o_v, h_v, hn_v, act_v, out_v,
            sem_x, sem_q, sem_kv, sem_o, sem_f, sem_out):
    S, D = x_v.shape
    F = wg_v.shape[1]
    NT = S // T
    KR = D // NT

    def rows(j, n=T):
        return pl.ds(pl.multiple_of(j * n, n), n)

    def x_copy(j):
        return pltpu.make_async_copy(x_hbm.at[rows(j)], x_v.at[rows(j)], sem_x.at[j])

    def wq_copy(j):
        return pltpu.make_async_copy(wqkv_hbm.at[rows(j, KR), pl.ds(0, D)],
                                     wqkv_v.at[rows(j, KR), pl.ds(0, D)], sem_q.at[j])

    def wkv_copy(j):
        return pltpu.make_async_copy(wqkv_hbm.at[rows(j, KR), pl.ds(D, 2 * D)],
                                     wqkv_v.at[rows(j, KR), pl.ds(D, 2 * D)], sem_kv.at[j])

    def wo_copy(j):
        return pltpu.make_async_copy(wo_hbm.at[:, rows(j, LANES)], wo_raw.at[j], sem_o.at[j])

    def out_copy(j):
        return pltpu.make_async_copy(out_v.at[rows(j)], out_hbm.at[rows(j)], sem_out.at[j])

    ffn_copies = [pltpu.make_async_copy(s, d, sem_f.at[i])
                  for i, (s, d) in enumerate(((wg_hbm, wg_v), (wu_hbm, wu_v), (wd_hbm, wd_v)))]

    x_copy(0).start()
    for j in range(NT):
        wq_copy(j).start()
    for j in range(NT):
        if j + 1 < NT:
            x_copy(j + 1).start()
        wkv_copy(j).start()
        wo_copy(j).start()
    for c in ffn_copies:
        c.start()

    x_copy(0).wait()
    xn_v[pl.ds(0, T), :] = _layernorm(x_v[pl.ds(0, T), :].astype(F32)).astype(BF16)

    def permute_q(j, carry):
        wq_copy(j).wait()
        wqkv_v[rows(j, KR), 0:D] = _permute_cols(wqkv_v[rows(j, KR), 0:D])
        return carry
    lax.fori_loop(0, NT, permute_q, 0)

    def phase_q(j, carry):
        @pl.when(j + 1 < NT)
        def _():
            x_copy(j + 1).wait()
        wkv_copy(j).wait()
        wo_copy(j).wait()
        q = _dot(xn_v[rows(j), :], wqkv_v[:, 0:D])
        for c in range(8):
            q_v[c, rows(j), :] = q[:, c * LANES:(c + 1) * LANES]
        for p in (1, 2):
            wqkv_v[rows(j, KR), p * D:(p + 1) * D] = _permute_cols(
                wqkv_v[rows(j, KR), p * D:(p + 1) * D])
        wo_v[:, rows(j, LANES)] = _permute_rows(wo_raw[j])
        jn = jnp.minimum(j + 1, NT - 1)
        xn_v[rows(jn), :] = _layernorm(x_v[rows(jn), :].astype(F32)).astype(BF16)
        return carry
    lax.fori_loop(0, NT, phase_q, 0)

    k_v[:, pl.ds(T, HALO), :] = jnp.zeros((8, HALO, LANES), F32)
    v_v[:, pl.ds(T, HALO), :] = jnp.zeros((8, HALO, LANES), F32)

    def phase_attn(j, carry):
        k_v[:, pl.ds(0, HALO), :] = k_v[:, pl.ds(T, HALO), :]
        v_tail = v_v[:, pl.ds(T, HALO), :]
        xn = xn_v[rows(j), :]
        k = _dot(xn, wqkv_v[:, D:2 * D])
        for c in range(8):
            k_v[c, pl.ds(HALO, T), :] = k[:, c * LANES:(c + 1) * LANES]
        v = _dot(xn, wqkv_v[:, 2 * D:3 * D])
        for c in range(8):
            vc = v[:, c * LANES:(c + 1) * LANES]
            v_v[c, pl.ds(HALO, T), :] = vc
            v_v[c, pl.ds(0, HALO), :] = jnp.where(
                j == 0, jnp.broadcast_to(vc[0:1, :], (HALO, LANES)), v_tail[c])

        lane = lax.broadcasted_iota(jnp.int32, (RB, LANES), 1)
        odd1 = (lane & 1) != 0
        odd2 = (lane & 2) != 0
        for r in range(0, T, RB):
            logits = [None] * WINDOW
            for c in range(8):
                qc = q_v[c, pl.ds(pl.multiple_of(j * T + r, RB), RB), :]
                for w in range(WINDOW):
                    t = qc * k_v[c, pl.ds(HALO + r - DILATION * w, RB), :]
                    logits[w] = t if c == 0 else logits[w] + t
            for w in range(WINDOW):
                l = logits[w]
                l = l + jnp.where(odd1, pltpu.roll(l, 1, 1), pltpu.roll(l, LANES - 1, 1))
                l = l + jnp.where(odd2, pltpu.roll(l, 2, 1), pltpu.roll(l, LANES - 2, 1))
                l = l * (HEAD_DIM ** -0.5)
                if r < DILATION * w:
                    pos = j * T + r + lax.broadcasted_iota(jnp.int32, (RB, LANES), 0)
                    l = jnp.where(pos >= DILATION * w, l, -1e9)
                logits[w] = l
            m = logits[0]
            for w in range(1, WINDOW):
                m = jnp.maximum(m, logits[w])
            e = [jnp.exp(l - m) for l in logits]
            s = e[0]
            for w in range(1, WINDOW):
                s = s + e[w]
            inv = 1.0 / s
            p = [t * inv for t in e]
            for c in range(8):
                o = None
                for w in range(WINDOW):
                    t = p[w] * v_v[c, pl.ds(HALO + r - DILATION * w, RB), :]
                    o = t if o is None else o + t
                o_v[pl.ds(r, RB), c * LANES:(c + 1) * LANES] = o.astype(BF16)
        h_v[rows(j), :] = x_v[rows(j), :].astype(F32) + _dot(o_v[...], wo_v[...])
        return carry
    lax.fori_loop(0, NT, phase_attn, 0)

    hn_v[...] = _layernorm(h_v[pl.ds(0, T), :]).astype(BF16)
    for c in ffn_copies:
        c.wait()

    def phase_ffn(j, carry):
        hn = hn_v[...]
        for f in range(0, F, TF):
            g = _dot(hn, wg_v[:, f:f + TF])
            u = _dot(hn, wu_v[:, f:f + TF])
            act_v[:, f:f + TF] = (_gelu(g) * u).astype(BF16)
        jn = jnp.minimum(j + 1, NT - 1)
        hn_v[...] = _layernorm(h_v[rows(jn), :]).astype(BF16)
        out_v[rows(j), :] = (h_v[rows(j), :] + _dot(act_v[...], wd_v[...])).astype(BF16)
        out_copy(j).start()
        return carry
    lax.fori_loop(0, NT, phase_ffn, 0)
    for j in range(NT):
        out_copy(j).wait()


@jax.jit
def pallas_sequential_preLN__sliding_local_dilated__glu_gated_geglu__prompt_kernel(
    A_x: jax.Array,
    A_wqkv: jax.Array,
    A_wo: jax.Array,
    B_x: jax.Array,
    B_w_gate: jax.Array,
    B_w_up: jax.Array,
    B_w_down: jax.Array,
):
    del B_x
    B, S, D = A_x.shape
    F = B_w_gate.shape[1]
    assert B == 1 and D == 8 * LANES and S == 8 * T and F % TF == 0
    NT = S // T
    any_spec = pl.BlockSpec(memory_space=pl.ANY)
    out = pl.pallas_call(
        _kernel,
        in_specs=[any_spec] * 6,
        out_specs=any_spec,
        out_shape=jax.ShapeDtypeStruct((S, D), A_x.dtype),
        scratch_shapes=[
            pltpu.VMEM((S, D), BF16),
            pltpu.VMEM((D, 3 * D), BF16),
            pltpu.VMEM((8, D, LANES), BF16),
            pltpu.VMEM((D, D), BF16),
            pltpu.VMEM((D, F), BF16),
            pltpu.VMEM((D, F), BF16),
            pltpu.VMEM((F, D), BF16),
            pltpu.VMEM((S, D), BF16),
            pltpu.VMEM((8, S, LANES), F32),
            pltpu.VMEM((8, HALO + T, LANES), F32),
            pltpu.VMEM((8, HALO + T, LANES), F32),
            pltpu.VMEM((T, D), BF16),
            pltpu.VMEM((S, D), F32),
            pltpu.VMEM((T, D), BF16),
            pltpu.VMEM((T, F), BF16),
            pltpu.VMEM((S, D), BF16),
            pltpu.SemaphoreType.DMA((NT,)),
            pltpu.SemaphoreType.DMA((NT,)),
            pltpu.SemaphoreType.DMA((NT,)),
            pltpu.SemaphoreType.DMA((NT,)),
            pltpu.SemaphoreType.DMA((3,)),
            pltpu.SemaphoreType.DMA((NT,)),
        ],
        compiler_params=pltpu.CompilerParams(vmem_limit_bytes=110 * 2**20),
    )(A_x.reshape(S, D), A_wqkv, A_wo, B_w_gate, B_w_up, B_w_down)
    return out.reshape(B, S, D)
```

```python
import jax
import jax.numpy as jnp
from jax import lax
import jax.experimental.pallas as pl
import jax.experimental.pallas.tpu as pltpu

HEAD_DIM = 32
WINDOW = 8
DILATION = 2
HALO = 16
LANES = 128
T = 256
H = T // 2
SB = 8
RB = 16
TN = 128
PLAIN = (1, 4)
GR = 256
PITCH = 33
NQ = 4
SCOPES = False
F32 = jnp.float32
BF16 = jnp.bfloat16
U32 = jnp.uint32


def _words(x):
    return pltpu.bitcast(x, U32)


def _halves(x):
    return pltpu.bitcast(x, BF16)


def _loop(name, n, body):
    def step(j, carry):
        if SCOPES:
            with jax.named_scope(name):
                body(j)
        else:
            body(j)
        return carry
    lax.fori_loop(0, n, step, 0)


def _emit(*stages):
    order = []
    for s, (lo, hi, steps) in enumerate(stages):
        order += [(lo + (hi - lo) * i / len(steps), s, i, f) for i, f in enumerate(steps)]
    for _, _, _, f in sorted(order, key=lambda t: t[:3]):
        f()


def _pipelined(pieces, depth):
    def step(t):
        for g in reversed(pieces[max(t - depth + 1, 0):t + 1]):
            next(g, None)
    return [lambda t=t: step(t) for t in range(len(pieces) + depth - 1)]


class _Pacer:
    def __init__(self, step=None):
        self.never = None if step is None else jnp.full((8, LANES), step, jnp.int32) < 0
        self.products = []
        self.due = []

    def _tie(self, x, others):
        regs = [[x[r:r + 8, c:c + LANES] for c in range(0, x.shape[1], LANES)]
                for r in range(0, x.shape[0], 8)]
        for k, other in enumerate(others):
            row, col = k % len(regs), k // len(regs) % len(regs[0])
            if other.dtype != x.dtype:
                other = pltpu.bitcast(other, x.dtype)
            regs[row][col] = jnp.where(self.never, other[:8, :LANES], regs[row][col])
        return jnp.concatenate([jnp.concatenate(row, axis=1) for row in regs], axis=0)

    def start(self, x, lag=1):
        if self.never is None or len(self.products) < lag:
            return x
        return self._tie(x, [self.products[-lag]] * (x.shape[0] // 8))

    def finish(self, x):
        if self.never is not None:
            self.due.append(x)

    def dot(self, lhs_words, rhs):
        if self.due:
            lhs_words = self._tie(lhs_words, self.due)
            self.due = []
        self.products.append(jnp.dot(_halves(lhs_words), rhs, preferred_element_type=F32))
        return self.products[-1]


def _gelu(x):
    c = 0.7978845608028654
    hx = 0.5 * x
    return hx + hx * jnp.tanh(x * (c + (c * 0.044715) * (x * x)))


def _lhs7(a11, a12, a21, a22):
    return [t.astype(BF16) for t in
            (a11 + a22, a21 + a22, a11, a22, a11 + a12, a21 - a11, a12 - a22)]


def _rhs7(b11, b12, b21, b22):
    f11, f12, f21, f22 = (b.astype(F32) for b in (b11, b12, b21, b22))
    return [t.astype(BF16) for t in
            (f11 + f22, b11, f12 - f22, f21 - f11, b22, f11 + f12, f21 + f22)]


def _strassen(pace, lhs, rhs, done):
    c = {}

    def m(i):
        return pace.dot(lhs(i), rhs(i))

    def s0():
        c["m1"] = m(0)

    def s1():
        c["m2"] = m(1)
        c[22] = c["m1"] - c["m2"]

    def s2():
        t = m(3)
        c[21] = c["m2"] + t
        c[11] = c["m1"] + t

    def s3():
        c["m5"] = m(4)
        c[11] = c[11] - c["m5"]

    def s4():
        t = m(2)
        c[12] = c["m5"] + t
        c[22] = c[22] + t

    def s5():
        c[11] = c[11] + m(6)

    def s6():
        done(c[11], c[12], c[21], c[22] + m(5))

    return [s0, s1, s2, s3, s4, s5, s6]


def _matmul(pace, lhs, rhs, width, done):
    steps = []
    for n in range(0, width, TN):
        steps += _strassen(pace, lhs, lambda i, n=n: rhs(i, n), lambda *c, n=n: done(n, *c))
    return steps


def _permute_cols(chunks):
    lane = lax.broadcasted_iota(jnp.int32, chunks[0].shape, 1)
    dl, blk, hl = lane // 32, lane // 4 % 8, lane % 4
    a = [pltpu.roll(chunks[c], 4 * c, 1) if c else chunks[c] for c in range(8)]
    yield
    e = [a[(-i) % 8] for i in range(8)]
    for s in (1, 2, 4):
        e = [jnp.where((blk & s) != 0, e[(i - s) % 8], e[i]) for i in range(8)]
    e = [jnp.take_along_axis(e[c], (hl * 32 + (blk + c) * 4 + dl) % LANES, axis=1)
         for c in range(8)]
    yield
    return e


def _kernel(x_hbm, wqkv_hbm, wo_hbm, wg_hbm, wu_hbm, wd_hbm, out_hbm,
            x_v, wq, wkv_raw, wo_raw, wo_f32, w_ops, ffn_w, a_ops, hn, attn, prob, act,
            q_raw, q_v, k_v, v_v, h_v, out_v,
            sem_x, sem_q, sem_kv, sem_o, sem_f, sem_out):
    S, D = x_v.shape
    DH = D // 2
    FH = wg_hbm.shape[2] // 2
    NT = S // T
    NI = NT // 2
    QR = GR // NQ
    KR = GR // NI
    FR = GR // NT
    PER = DH // GR
    WK, WV, WO = range(3)

    def ds(start, size):
        return pl.ds(start if isinstance(start, int) else pl.multiple_of(start, size), size)

    def x_copy(j):
        return pltpu.make_async_copy(x_hbm.at[ds(j * T, T)], x_v.at[ds(j * T, T)], sem_x.at[j])

    def block_copies(src, dst, rows, sem):
        _, per, _, half = dst.shape
        return [pltpu.make_async_copy(
            src.at[pl.ds(b // 2 * per, per), rows, pl.ds(b % 2 * half, half)],
            dst.at[1 + b, :, rows, :], sem) for b in range(4)]

    def wq_copies(j):
        return block_copies(wqkv_hbm, wq, ds(j * QR, QR), sem_q.at[j])

    def wkv_copy(j):
        return pltpu.make_async_copy(wqkv_hbm.at[:, ds(j * KR, KR), pl.ds(D, 2 * D)],
                                     wkv_raw.at[j], sem_kv.at[j])

    def wo_copies(j):
        return [pltpu.make_async_copy(wo_hbm.at[:, ds(s * DH + j * LANES, LANES)],
                                      wo_raw.at[j, s], sem_o.at[j]) for s in range(2)]

    def ffn_copies(j):
        return [c for src, dst in zip((wg_hbm, wu_hbm, wd_hbm), ffn_w)
                for c in block_copies(src, dst, ds(j * FR, FR), sem_f.at[j])]

    def out_copy(j):
        return pltpu.make_async_copy(out_v.at[ds(j * T, T)], out_hbm.at[ds(j * T, T)],
                                     sem_out.at[j])

    def store_weight(m, i, g, row, col, t):
        w_ops[m][i * PER + g, ds(row // 2, t.shape[0] // 2), col] = _words(t)

    def weight(m):
        return lambda i, n: _halves(
            w_ops[m][pl.ds(i * PER, PER), :, n:n + TN].reshape(DH // 2, TN))

    def norm_steps(pace, load_rows, store):
        def piece(r):
            def load():
                return jnp.concatenate([load_rows(s * H + r).astype(F32) for s in range(2)], axis=0)
            m = jnp.mean(pace.start(load()), axis=-1, keepdims=True)
            yield
            c = load() - m
            scale = lax.rsqrt(jnp.mean(c * c, axis=-1, keepdims=True) + 1e-5)
            yield
            y = (load() - m) * scale
            for i, t in enumerate(_lhs7(y[:RB, :DH], y[:RB, DH:], y[RB:, :DH], y[RB:, DH:])):
                store(i, pl.ds(r // 2, RB // 2), _words(t))
                for c in range(0, DH, LANES):
                    pace.finish(_words(t)[:, c:c + LANES])
        return _pipelined([piece(r) for r in range(0, H, RB)], 3)

    def xn_steps(pace, j, *copies):
        def store(i, rows, t):
            a_ops[7 * j + i, rows, :] = t
            for c in copies:
                c[i, rows, :] = t
        return norm_steps(pace, lambda r: x_v[ds(j * T + r, RB), :], store)

    def hn_steps(pace, slot):
        def store(i, rows, t):
            hn[i, rows, :] = t
        return norm_steps(pace, lambda r: h_v[slot, pl.ds(r, RB), :], store)

    def qkv_weight_steps(pace, raw, col, m, row0):
        def piece(g, r):
            u = [jnp.concatenate(
                [_words(raw[kh * PER + g, pl.ds(r, RB), pl.ds(col + c * LANES, LANES)])
                 for kh in range(2)], axis=0) for c in range(8)]
            u = yield from _permute_cols([pace.start(u[0])] + u[1:])
            for c in range(4):
                b = [_halves(u[nh * 4 + c][kh * RB // 2:(kh + 1) * RB // 2])
                     for kh in range(2) for nh in range(2)]
                for i, t in enumerate(_rhs7(*b)):
                    store_weight(m, i, g, row0 + r, pl.ds(c * LANES, LANES), t)
                    if i not in PLAIN:
                        pace.finish(_words(t))
        return _pipelined([piece(g, r) for r in range(0, raw.shape[1], RB)
                           for g in range(PER)], 3)

    def in_place_steps(pace, mats, row0, nrows):
        def step(w, g, r, n):
            idx = (g, ds(row0 + r, FR), pl.ds(n, 2 * LANES))
            blocks = [w[(1 + b,) + idx] for b in range(4)]
            pace.finish(blocks[0].astype(F32))
            for i, t in enumerate(_rhs7(*blocks)):
                if i not in PLAIN:
                    w[(i,) + idx] = t
        steps = [[lambda w=w, g=g, r=r, n=n: step(w, g, r, n) for g in range(w.shape[1])
                  for r in range(0, nrows, FR) for n in range(0, w.shape[3], 2 * LANES)]
                 for w in mats]
        return [f for group in zip(*steps) for f in group]

    def in_place_weight(w):
        return lambda i, n: w[i, :, :, n:n + TN].reshape(w.shape[1] * GR, TN)

    def permute_q_steps(pace, j):
        def piece(r):
            q = [q_raw[j, c, pl.ds(r, 2 * RB), :] for c in range(8)]
            q = yield from _permute_cols(q[:1] + [pace.start(q[1])] + q[2:])
            for c in range(8):
                q_v[j, c, pl.ds(r, 2 * RB), :] = q[c]
            pace.finish(q[7][2 * RB - 8:])
        return _pipelined([piece(r) for r in range(0, T, 2 * RB)], 3)

    def project(pace, j, lhs, rhs, dst, halo):
        def done(n, *c):
            for b, t in enumerate(c):
                chunk = (b % 2 * DH + n) // LANES
                dst[j, chunk, pl.ds(halo + b // 2 * H, H), :] = t
                if halo and b // 2:
                    dst[j + 1, chunk, pl.ds(0, halo), :] = t[H - halo:]
        return _matmul(pace, lhs or (lambda i: a_ops[7 * j + i]), rhs, DH, done)

    def softmax_steps(pace, q, k, out, rows, first=None):
        def piece(r):
            logits = [None] * WINDOW
            for c in range(8):
                qc = q[c, pl.ds(r, SB), :]
                if c == 0:
                    qc = pace.start(qc)
                for w in range(WINDOW):
                    t = qc * k[c, pl.ds(HALO + r - DILATION * w, SB), :]
                    logits[w] = t if c == 0 else logits[w] + t
            rolled = [pltpu.roll(l, LANES // 2, 1) for l in logits]
            yield
            logits = [a + b for a, b in zip(logits, rolled)]
            rolled = [pltpu.roll(l, LANES // 4, 1) for l in logits]
            yield
            for w in range(WINDOW):
                l = (logits[w] + rolled[w]) * (HEAD_DIM ** -0.5)
                if first is not None and r < DILATION * w:
                    pos = first + r + lax.broadcasted_iota(jnp.int32, (SB, LANES), 0)
                    l = jnp.where(pos >= DILATION * w, l, -1e9)
                logits[w] = l
            m = logits[0]
            for w in range(1, WINDOW):
                m = jnp.maximum(m, logits[w])
            e = [jnp.exp(l - m) for l in logits]
            total = e[0]
            for w in range(1, WINDOW):
                total = total + e[w]
            inv = 1.0 / total
            for w in range(WINDOW):
                p = e[w] * inv
                out[w, pl.ds(r, SB), :] = p
                pace.finish(p)
        return _pipelined([piece(r) for r in rows], 3)

    def value_steps(pace, weights, v, out, rows):
        def step(r, c):
            blocks = []
            for row in (r, H + r):
                o = [None, None]
                for w in range(WINDOW):
                    p = weights[w, pl.ds(row, RB), :]
                    if w == 0:
                        p = pace.start(p, 5)
                    for s in range(2):
                        t = p * v[c + 4 * s, pl.ds(HALO + row - DILATION * w, RB), :]
                        o[s] = t if w == 0 else o[s] + t
                blocks += o
            for i, t in enumerate(_lhs7(*blocks)):
                out[i, pl.ds(r // 2, RB // 2), pl.ds(c * LANES, LANES)] = _words(t)
                pace.finish(_words(t))
        return [lambda r=r, c=c: step(r, c) for r in rows for c in range(4)]

    def output_steps(pace, j, slot):
        def done(n, *c):
            for b, t in enumerate(c):
                cols = pl.ds(b % 2 * DH + n, TN)
                h_v[slot, pl.ds(b // 2 * H, H), cols] = (
                    x_v[ds(j * T + b // 2 * H, H), cols].astype(F32) + t)
        return _matmul(pace, lambda i: attn[i], weight(WO), DH, done)

    x_copy(0).start()
    for j in range(NQ):
        for c in wq_copies(j):
            c.start()
    x_copy(0).wait()
    _emit((0, 1, xn_steps(_Pacer(), 0, hn)))

    def prepare_q(j):
        for c in wq_copies(j):
            c.wait()
        _emit((0, 1, in_place_steps(_Pacer(), [wq], j * QR, QR)))
    _loop("prepare_q", NQ, prepare_q)
    for j in range(NI):
        for t in range(2 * j + 1, min(2 * j + 3, NT)):
            x_copy(t).start()
        wkv_copy(j).start()
        for c in wo_copies(j):
            c.start()

    def phase_q(j):
        x_copy(2 * j + 1).wait()

        @pl.when(j + 1 < NI)
        def _():
            x_copy(2 * j + 2).wait()
        wkv_copy(j).wait()
        for c in wo_copies(j):
            c.wait()

        @pl.when(j >= NI - 2)
        def _():
            for c in ffn_copies(j - (NI - 2)):
                c.start()

        pace = _Pacer(j)

        def wo_widen(s, r):
            wo_f32[s, pl.ds(r * PITCH, HEAD_DIM), :] = (
                wo_raw[j, s, pl.ds(r * HEAD_DIM, HEAD_DIM), :].astype(F32))

        def wo_step(d):
            b = [wo_f32[s, pl.ds(kh * HEAD_DIM // 2 + d, D // HEAD_DIM, stride=PITCH), :]
                 for kh in range(2) for s in range(2)]
            r = d * (D // HEAD_DIM)
            for i, t in enumerate(_rhs7(*b)):
                store_weight(WO, i, r // GR, r % GR, ds(j * LANES, LANES), t)
                pace.finish(_words(t))
                pace.finish(_words(t)[8:])

        _emit(
            (0, 1, project(pace, 2 * j, lambda i: hn[i], in_place_weight(wq), q_raw, 0)),
            (1, 2, project(pace, 2 * j + 1, lambda i: attn[i], in_place_weight(wq), q_raw, 0)),
            (0.05, 0.97, xn_steps(pace, 2 * j + 1, attn)),
            (0.95, 1.95, xn_steps(pace, jnp.minimum(2 * j + 2, NT - 1), hn)),
            (0.1, 1, qkv_weight_steps(pace, wkv_raw.at[j], 0, WK, j * KR)),
            (0.95, 1.95, qkv_weight_steps(pace, wkv_raw.at[j], D, WV, j * KR)),
            (0, 0.1, [lambda s=s, r=r: wo_widen(s, r) for s in range(2)
                      for r in range(D // HEAD_DIM)]),
            (0.3, 1.95, [lambda d=d: wo_step(d) for d in range(HEAD_DIM // 2)]),
        )
    _loop("phase_q", NI, phase_q)

    prob[:, pl.ds(0, H + RB), :] = jnp.zeros((WINDOW, H + RB, LANES), F32)
    v_v[0, :, pl.ds(0, HALO + H + RB), :] = jnp.zeros((8, HALO + H + RB, LANES), F32)
    k_v[0, :, pl.ds(0, HALO), :] = jnp.zeros((8, HALO, LANES), F32)

    def first_values(pace, g):
        for c in range(8):
            v_v[0, c, pl.ds(0, HALO), :] = jnp.broadcast_to(
                v_v[0, c, pl.ds(HALO, 1), :], (HALO, LANES))
        row = pl.multiple_of(g * RB, RB)
        return value_steps(pace, prob.at[:, pl.ds(row, H + RB)],
                           v_v.at[0, :, pl.ds(row, HALO + H + RB)],
                           attn.at[:, ds(g * RB // 2, RB // 2)], [0])

    def phase_kv(j):
        for c in ffn_copies(j):
            c.wait()

        @pl.when(j + 2 < NT)
        def _():
            for c in ffn_copies(j + 2):
                c.start()
        pace = _Pacer(j)
        row = pl.multiple_of(j * RB, RB)
        _emit(
            (0, 1, project(pace, j, None, weight(WK), k_v, HALO)),
            (1, 2, project(pace, j, None, weight(WV), v_v, HALO)),
            (0, 1.85, in_place_steps(pace, ffn_w, j * FR, FR)),
            (0, 1.1, permute_q_steps(pace, j)),
            (0.25, 1, first_values(pace, jnp.maximum(j - 1, 0))),
            (1.15, 1.9, softmax_steps(
                pace, q_v.at[0, :, pl.ds(row, H + RB)], k_v.at[0, :, pl.ds(row, HALO + H + RB)],
                prob.at[:, pl.ds(row, H + RB)],
                [s * H + r for s in range(2) for r in range(0, RB, SB)], row)),
        )
    _loop("phase_kv", NT, phase_kv)

    def first_output(_):
        pace = _Pacer()
        _emit((0, 1, first_values(pace, jnp.int32(NT - 1)) + output_steps(pace, 0, 0)
               + hn_steps(pace, 0)))
    _loop("first_output", 1, first_output)

    def phase_ffn(j):
        nxt = jnp.minimum(j + 1, NT - 1)
        slot = j % 2
        pace = _Pacer(j)
        gate = {}

        def gate_done(n, *c):
            gate[n] = [_gelu(t) for t in c]

        def up_done(n, *c):
            for i, t in enumerate(_lhs7(*[g * u for g, u in zip(gate.pop(n), c)])):
                act[i, :, n:n + TN] = _words(t)

        def down_done(n, *c):
            for b, t in enumerate(c):
                cols = pl.ds(b % 2 * DH + n, TN)
                out_v[ds(j * T + b // 2 * H, H), cols] = (
                    h_v[slot, pl.ds(b // 2 * H, H), cols] + t).astype(BF16)

        g = _matmul(pace, lambda i: hn[i], in_place_weight(ffn_w[0]), FH, gate_done)
        u = _matmul(pace, lambda i: hn[i], in_place_weight(ffn_w[1]), FH, up_done)
        gu = [f for n in range(0, len(g), 7) for f in g[n:n + 7] + u[n:n + 7]]
        _emit(
            (0, 1, gu),
            (1, 2, output_steps(pace, nxt, 1 - slot)),
            (2, 3, _matmul(pace, lambda i: act[i], in_place_weight(ffn_w[2]), DH, down_done)),
            (0.01, 0.58, softmax_steps(pace, q_v.at[nxt], k_v.at[nxt], prob, range(0, T, SB))),
            (0.58, 0.99, value_steps(pace, prob, v_v.at[nxt], attn, range(0, H, RB))),
            (2.05, 2.9, hn_steps(pace, 1 - slot)),
        )
        out_copy(j).start()
    _loop("phase_ffn", NT, phase_ffn)
    for j in range(NT):
        out_copy(j).wait()


@jax.jit
def pallas_sequential_preLN__sliding_local_dilated__glu_gated_geglu__prompt_kernel(
    A_x: jax.Array,
    A_wqkv: jax.Array,
    A_wo: jax.Array,
    B_x: jax.Array,
    B_w_gate: jax.Array,
    B_w_up: jax.Array,
    B_w_down: jax.Array,
):
    del B_x
    B, S, D = A_x.shape
    F = B_w_gate.shape[1]
    DH, FH = D // 2, F // 2
    NT = S // T
    NI = NT // 2
    assert B == 1 and D == 8 * LANES and NI * LANES == DH and FH % GR == 0 and 2 * GR == DH
    any_spec = pl.BlockSpec(memory_space=pl.ANY)
    out = pl.pallas_call(
        _kernel,
        in_specs=[any_spec] * 6,
        out_specs=any_spec,
        out_shape=jax.ShapeDtypeStruct((S, D), A_x.dtype),
        scratch_shapes=[
            pltpu.VMEM((S, D), BF16),
            pltpu.VMEM((7, DH // GR, GR, DH), BF16),
            pltpu.VMEM((NI, D // GR, GR // NI, 2 * D), BF16),
            pltpu.VMEM((NI, 2, D, LANES), BF16),
            pltpu.VMEM((2, HEAD_DIM * PITCH, LANES), F32),
            [pltpu.VMEM((7 * DH // GR, GR // 2, DH), U32)] * 3,
            [pltpu.VMEM((7, DH // GR, GR, FH), BF16)] * 2
            + [pltpu.VMEM((7, FH // GR, GR, DH), BF16)],
            pltpu.VMEM((7 * NT, H // 2, DH), U32),
            pltpu.VMEM((7, H // 2, DH), U32),
            pltpu.VMEM((7, H // 2, DH), U32),
            pltpu.VMEM((WINDOW, T, LANES), F32),
            pltpu.VMEM((7, H // 2, FH), U32),
            pltpu.VMEM((NT, 8, T, LANES), F32),
            pltpu.VMEM((NT, 8, T, LANES), F32),
            pltpu.VMEM((NT + 1, 8, HALO + T, LANES), F32),
            pltpu.VMEM((NT + 1, 8, HALO + T, LANES), F32),
            pltpu.VMEM((2, T, D), F32),
            pltpu.VMEM((S, D), BF16),
            pltpu.SemaphoreType.DMA((NT,)),
            pltpu.SemaphoreType.DMA((NQ,)),
            pltpu.SemaphoreType.DMA((NI,)),
            pltpu.SemaphoreType.DMA((NI,)),
            pltpu.SemaphoreType.DMA((NT,)),
            pltpu.SemaphoreType.DMA((NT,)),
        ],
        compiler_params=pltpu.CompilerParams(vmem_limit_bytes=124 * 2**20),
    )(A_x.reshape(S, D), A_wqkv.reshape(D // GR, GR, 3 * D), A_wo,
      B_w_gate.reshape(D // GR, GR, F), B_w_up.reshape(D // GR, GR, F),
      B_w_down.reshape(F // GR, GR, D))
    return out.reshape(B, S, D)
```

```python
import jax
import jax.numpy as jnp
from jax import lax
import jax.experimental.pallas as pl
import jax.experimental.pallas.tpu as pltpu

HEAD_DIM = 32
WINDOW = 8
DILATION = 2
HALO = 16
LANES = 128
T = 256
H = T // 2
SB = 8
RB = 16
TN = 128
PLAIN = (1, 4)
GR = 256
NQ = 4
SCOPES = False
F32 = jnp.float32
BF16 = jnp.bfloat16
U32 = jnp.uint32


def _words(x):
    return pltpu.bitcast(x, U32)


def _halves(x):
    return pltpu.bitcast(x, BF16)


def _loop(name, n, body):
    def step(j, carry):
        if SCOPES:
            with jax.named_scope(name):
                body(j)
        else:
            body(j)
        return carry
    lax.fori_loop(0, n, step, 0)


def _emit(*stages):
    order = []
    for s, (lo, hi, steps) in enumerate(stages):
        order += [(lo + (hi - lo) * i / len(steps), s, i, f) for i, f in enumerate(steps)]
    for _, _, _, f in sorted(order, key=lambda t: t[:3]):
        f()


def _pipelined(pieces, depth):
    def step(t):
        for g in reversed(pieces[max(t - depth + 1, 0):t + 1]):
            next(g, None)
    return [lambda t=t: step(t) for t in range(len(pieces) + depth - 1)]


class _Pacer:
    def __init__(self, step=None):
        self.never = None if step is None else jnp.full((8, LANES), step, jnp.int32) < 0
        self.products = []
        self.due = []

    def _tie(self, x, others):
        regs = [[x[r:r + 8, c:c + LANES] for c in range(0, x.shape[1], LANES)]
                for r in range(0, x.shape[0], 8)]
        for k, other in enumerate(others):
            row, col = k % len(regs), k // len(regs) % len(regs[0])
            if other.dtype != x.dtype:
                other = pltpu.bitcast(other, x.dtype)
            regs[row][col] = jnp.where(self.never, other[:8, :LANES], regs[row][col])
        return jnp.concatenate([jnp.concatenate(row, axis=1) for row in regs], axis=0)

    def start(self, x, lag=3):
        if self.never is None or len(self.products) < lag:
            return x
        return self._tie(x, [self.products[-lag]] * (x.shape[0] // 8))

    def finish(self, x):
        if self.never is not None:
            self.due.append(x)

    def dot(self, lhs_words, rhs):
        if self.due:
            lhs_words = self._tie(lhs_words, self.due)
            self.due = []
        self.products.append(jnp.dot(_halves(lhs_words), rhs, preferred_element_type=F32))
        return self.products[-1]


def _gelu(x):
    c = 0.7978845608028654
    hx = 0.5 * x
    return hx + hx * jnp.tanh(x * (c + (c * 0.044715) * (x * x)))


def _lhs7(a11, a12, a21, a22):
    return [t.astype(BF16) for t in
            (a11 + a22, a21 + a22, a11, a22, a11 + a12, a21 - a11, a12 - a22)]


def _rhs7(b11, b12, b21, b22):
    f11, f12, f21, f22 = (b.astype(F32) for b in (b11, b12, b21, b22))
    return [t.astype(BF16) for t in
            (f11 + f22, b11, f12 - f22, f21 - f11, b22, f11 + f12, f21 + f22)]


def _strassen(pace, lhs, rhs, done):
    c = {}

    def m(i):
        return pace.dot(lhs(i), rhs(i))

    def s0():
        c["m1"] = m(0)

    def s1():
        c["m2"] = m(1)
        c[22] = c["m1"] - c["m2"]

    def s2():
        t = m(3)
        c[21] = c["m2"] + t
        c[11] = c["m1"] + t

    def s3():
        c["m5"] = m(4)
        c[11] = c[11] - c["m5"]

    def s4():
        t = m(2)
        c[12] = c["m5"] + t
        c[22] = c[22] + t

    def s5():
        c[11] = c[11] + m(6)

    def s6():
        done(c[11], c[12], c[21], c[22] + m(5))

    return [s0, s1, s2, s3, s4, s5, s6]


def _matmul(pace, lhs, rhs, width, done):
    steps = []
    for n in range(0, width, TN):
        steps += _strassen(pace, lhs, lambda i, n=n: rhs(i, n), lambda *c, n=n: done(n, *c))
    return steps


def _permute_cols(chunks):
    blk = lax.broadcasted_iota(jnp.int32, chunks[0].shape, 1) // 4
    a = [pltpu.roll(chunks[c], 4 * c, 1) if c else chunks[c] for c in range(8)]
    yield
    e = [a[(-i) % 8] for i in range(8)]
    for s in (1, 2, 4):
        e = [jnp.where((blk & s) != 0, e[(i - s) % 8], e[i]) for i in range(8)]
    e = [pltpu.roll(e[c], LANES - 4 * c, 1) if c else e[c] for c in range(8)]
    yield
    return e


def _permuted_rows(ref, c, hl, cols):
    parts = []
    for cp in range(8):
        r = c * 4
        u = _words(ref[pl.ds(pl.multiple_of(cp * LANES + hl * 32 + r // 16 * 16, 16), 16), cols])
        parts.append(u[r % 16 // 2:r % 16 // 2 + 2, :])
    return _halves(jnp.concatenate(parts, axis=0))


def _kernel(x_hbm, wqkv_hbm, wo_hbm, wg_hbm, wu_hbm, wd_hbm, out_hbm,
            x_v, wq_raw, wkv_raw, wo_raw, centred, w_ops, ffn_w, a_ops, hn, attn, prob, act,
            q_raw, q_v, k_v, v_v, h_v, out_v,
            sem_x, sem_q, sem_kv, sem_o, sem_f, sem_out):
    S, D = x_hbm.shape
    DH = D // 2
    FH = wg_hbm.shape[2] // 2
    NT = S // T
    NI = NT // 2
    QR = GR // NQ
    KR = GR // NI
    FR = GR // NT
    PER = DH // GR
    WQ, WKV, WO = range(3)

    def ds(start, size):
        return pl.ds(start if isinstance(start, int) else pl.multiple_of(start, size), size)

    def last(j):
        return min(j, NT - 1) if isinstance(j, int) else jnp.minimum(j, NT - 1)

    def x_copy(j):
        return pltpu.make_async_copy(x_hbm.at[ds(last(j) * T, T)], x_v.at[ds(j * T, T)],
                                     sem_x.at[j])

    def wq_copy(j):
        return pltpu.make_async_copy(wqkv_hbm.at[:, ds(j * QR, QR), pl.ds(0, D)],
                                     wq_raw.at[j], sem_q.at[j])

    def wkv_copy(j):
        return pltpu.make_async_copy(
            wqkv_hbm.at[:, ds(j % NI * KR, KR), ds((1 + j // NI) * D, D)],
            wkv_raw.at[j], sem_kv.at[j])

    wo_copy = pltpu.make_async_copy(wo_hbm, wo_raw, sem_o)

    def ffn_copies(j):
        rows = ds(j * FR, FR)
        return [pltpu.make_async_copy(src.at[:, rows], dst.at[:, rows], sem_f.at[j])
                for src, (dst, _) in zip((wg_hbm, wu_hbm, wd_hbm), ffn_w)]

    def out_copy(j):
        return pltpu.make_async_copy(out_v.at[ds(j * T, T)], out_hbm.at[ds(j * T, T)],
                                     sem_out.at[j])

    def store_weight(m, i, g, row, col, t):
        w_ops[m][i * PER + g, ds(row // 2, t.shape[0] // 2), col] = _words(t)

    def weight(m, first=0):
        return lambda i, n: _halves(
            w_ops[m][pl.ds(first + i * PER, PER), :, n:n + TN].reshape(DH // 2, TN))

    def norm_steps(pace, load_rows, store):
        def piece(r):
            def load():
                return jnp.concatenate([load_rows(s * H + r).astype(F32) for s in range(2)], axis=0)
            m = jnp.mean(pace.start(load()), axis=-1, keepdims=True)
            yield
            c = load() - m
            centred[pl.ds(2 * r, 2 * RB), :] = c
            scale = lax.rsqrt(jnp.mean(c * c, axis=-1, keepdims=True) + 1e-5)
            yield
            y = centred[pl.ds(2 * r, 2 * RB), :] * scale
            for i, t in enumerate(_lhs7(y[:RB, :DH], y[:RB, DH:], y[RB:, :DH], y[RB:, DH:])):
                store(i, pl.ds(r // 2, RB // 2), _words(t))
                pace.finish(_words(t)[:, i % 4 * LANES:(i % 4 + 1) * LANES])
        return _pipelined([piece(r) for r in range(0, H, RB)], 3)

    def xn_steps(pace, j, *copies):
        def store(i, rows, t):
            a_ops[7 * j + i, rows, :] = t
            for c in copies:
                c[i, rows, :] = t
        return norm_steps(pace, lambda r: x_v[ds(j * T + r, RB), :], store)

    def hn_steps(pace, slot):
        def store(i, rows, t):
            hn[i, rows, :] = t
        return norm_steps(pace, lambda r: h_v[slot, pl.ds(r, RB), :], store)

    def kv_weight_steps(pace, raw, first, row0):
        def piece(g, r):
            u = [jnp.concatenate(
                [_words(raw[kh * PER + g, pl.ds(r, RB), pl.ds(c * LANES, LANES)])
                 for kh in range(2)], axis=0) for c in range(8)]
            u = yield from _permute_cols(u[:1] + [pace.start(u[1])] + u[2:])
            for c in range(4):
                b = [_halves(u[nh * 4 + c][kh * RB // 2:(kh + 1) * RB // 2])
                     for kh in range(2) for nh in range(2)]
                for i, t in enumerate(_rhs7(*b)):
                    store_weight(WKV, i, first + g, row0 + r, pl.ds(c * LANES, LANES), t)
                    if i >= 5:
                        pace.finish(_words(t))
        return _pipelined([piece(g, r) for r in range(0, raw.shape[1], RB)
                           for g in range(PER)], 3)

    def ffn_index(w, i, g, rows, n, width):
        blocks, extra = w
        _, per, _, half = extra.shape
        if 1 <= i <= 4:
            g = pl.ds((i - 1) // 2 * per, per) if g is None else (i - 1) // 2 * per + g
            return blocks, (g, rows, pl.ds((i - 1) % 2 * half + n, width))
        return extra, (i % 4, slice(None) if g is None else g, rows, pl.ds(n, width))

    def ffn_weight_steps(pace, j):
        def step(w, g, n):
            where = [ffn_index(w, i, g, ds(j * FR, FR), n, 2 * LANES) for i in range(7)]
            blocks = [ref[idx] for ref, idx in where[1:5]]
            blocks[0] = pace.start(blocks[0].astype(F32), 3)
            pace.finish(blocks[0])
            for i, t in enumerate(_rhs7(*blocks)):
                if i not in PLAIN:
                    ref, idx = where[i]
                    ref[idx] = t
        steps = [[lambda w=w, g=g, n=n: step(w, g, n) for g in range(w[1].shape[1])
                  for n in range(0, w[1].shape[3], 2 * LANES)] for w in ffn_w]
        return [f for group in zip(*steps) for f in group]

    def ffn_weight(w):
        def load(i, n):
            ref, idx = ffn_index(w, i, None, slice(None), n, TN)
            return ref[idx].reshape(w[1].shape[1] * GR, TN)
        return load

    def permute_q_steps(pace, j):
        def piece(r):
            q = [q_raw[j, c, pl.ds(r, 2 * RB), :] for c in range(8)]
            q = yield from _permute_cols(q[:1] + [pace.start(q[1])] + q[2:])
            for c in range(8):
                q_v[j, c, pl.ds(r, 2 * RB), :] = q[c]
                pace.finish(q[c][c % 4 * 8:])
        return _pipelined([piece(r) for r in range(0, T, 2 * RB)], 3)

    def project(pace, j, lhs, rhs, dst, halo):
        def done(n, *c):
            for b, t in enumerate(c):
                chunk = (b % 2 * DH + n) // LANES
                dst[j, chunk, pl.ds(halo + b // 2 * H, H), :] = t
                if halo and b // 2:
                    dst[j + 1, chunk, pl.ds(0, halo), :] = t[H - halo:]
        return _matmul(pace, lhs or (lambda i: a_ops[7 * j + i]), rhs, DH, done)

    def softmax_steps(pace, q, k, out, rows, first=None):
        def piece(r):
            logits = [None] * WINDOW
            for c in range(8):
                qc = q[c, pl.ds(r, SB), :]
                if c == 0:
                    qc = pace.start(qc)
                for w in range(WINDOW):
                    t = qc * k[c, pl.ds(HALO + r - DILATION * w, SB), :]
                    logits[w] = t if c == 0 else logits[w] + t
            lane = lax.broadcasted_iota(jnp.int32, (SB, LANES), 1)
            for s in (1, 2):
                rolled = [(pltpu.roll(l, s, 1), pltpu.roll(l, LANES - s, 1)) for l in logits]
                yield
                logits = [l + jnp.where((lane & s) != 0, a, b)
                          for l, (a, b) in zip(logits, rolled)]
            for w in range(WINDOW):
                l = logits[w] * (HEAD_DIM ** -0.5)
                if first is not None and r < DILATION * w:
                    pos = first + r + lax.broadcasted_iota(jnp.int32, (SB, LANES), 0)
                    l = jnp.where(pos >= DILATION * w, l, -1e9)
                logits[w] = l
            m = logits[0]
            for w in range(1, WINDOW):
                m = jnp.maximum(m, logits[w])
            e = [jnp.exp(l - m) for l in logits]
            total = e[0]
            for w in range(1, WINDOW):
                total = total + e[w]
            inv = 1.0 / total
            for w in range(WINDOW):
                p = e[w] * inv
                out[w, pl.ds(r, SB), :] = p
                pace.finish(p)
        return _pipelined([piece(r) for r in rows], 3)

    def value_steps(pace, weights, v, out, rows):
        def step(r, c):
            blocks = []
            for row in (r, H + r):
                o = [None, None]
                for w in range(WINDOW):
                    p = weights[w, pl.ds(row, RB), :]
                    if w == 0:
                        p = pace.start(p, 5)
                    for s in range(2):
                        t = p * v[c + 4 * s, pl.ds(HALO + row - DILATION * w, RB), :]
                        o[s] = t if w == 0 else o[s] + t
                blocks += o
            for i, t in enumerate(_lhs7(*blocks)):
                out[i, pl.ds(r // 2, RB // 2), pl.ds(c * LANES, LANES)] = _words(t)
                pace.finish(_words(t))
        return [lambda r=r, c=c: step(r, c) for r in rows for c in range(4)]

    def output_steps(pace, j, slot):
        def done(n, *c):
            for b, t in enumerate(c):
                cols = pl.ds(b % 2 * DH + n, TN)
                h_v[slot, pl.ds(b // 2 * H, H), cols] = (
                    x_v[ds(j * T + b // 2 * H, H), cols].astype(F32) + t)
        return _matmul(pace, lambda i: attn[i], weight(WO), DH, done)

    x_copy(0).start()
    wq_copy(0).start()
    wq_copy(1).start()
    prob[:, pl.ds(0, H + RB), :] = jnp.zeros((WINDOW, H + RB, LANES), F32)
    v_v[0, :, pl.ds(0, HALO + H + RB), :] = jnp.zeros((8, HALO + H + RB, LANES), F32)
    k_v[0, :, pl.ds(0, HALO), :] = jnp.zeros((8, HALO, LANES), F32)
    x_copy(0).wait()
    for j in range(2, NQ):
        wq_copy(j).start()
    _emit((0, 1, xn_steps(_Pacer(), 0, hn)))
    x_copy(1).start()
    wkv_copy(0).start()
    x_copy(2).start()
    wkv_copy(1).start()

    def prepare_q(j):
        wq_copy(j).wait()
        for g in range(PER):
            for r in range(0, QR, RB):
                for n in range(0, DH, 2 * LANES):
                    b = [wq_raw[j, kh * PER + g, pl.ds(r, RB), pl.ds(nh * DH + n, 2 * LANES)]
                         for kh in range(2) for nh in range(2)]
                    for i, t in enumerate(_rhs7(*b)):
                        store_weight(WQ, i, g, j * QR + r, pl.ds(n, 2 * LANES), t)
    _loop("prepare_q", NQ, prepare_q)
    for t in range(2, NT):
        x_copy(t + 1).start()
        wkv_copy(t).start()
    for c in [wo_copy] + ffn_copies(0) + ffn_copies(1):
        c.start()

    def phase_q(j):
        for t, (cur, nxt) in ((2 * j, (hn, attn)), (2 * j + 1, (attn, hn))):
            x_copy(t + 1).wait()
            wkv_copy(t).wait()
            pace = _Pacer(j)
            _emit(
                (0, 1, project(pace, t, lambda i: cur[i], weight(WQ), q_raw, 0)),
                (-0.05, 0.93, xn_steps(pace, t + 1, nxt)),
                (0.0, 0.97, kv_weight_steps(pace, wkv_raw.at[t], t // NI * 7 * PER,
                                             t % NI * KR)),
            )
    _loop("phase_q", NI, phase_q)
    for t in range(2, NT):
        for c in ffn_copies(t):
            c.start()
    wo_copy.wait()

    def first_values(pace, g):
        for c in range(8):
            v_v[0, c, pl.ds(0, HALO), :] = jnp.broadcast_to(
                v_v[0, c, pl.ds(HALO, 1), :], (HALO, LANES))
        row = pl.multiple_of(g * RB, RB)
        return value_steps(pace, prob.at[:, pl.ds(row, H + RB)],
                           v_v.at[0, :, pl.ds(row, HALO + H + RB)],
                           attn.at[:, ds(g * RB // 2, RB // 2)], [0])

    def phase_kv(j):
        for c in ffn_copies(j):
            c.wait()

        def wo_step(c, hl):
            col = j % NI * LANES
            b = [_permuted_rows(wo_raw, kh * 4 + c, hl, ds(s * DH + col, LANES))
                 for kh in range(2) for s in range(2)]
            b[0] = pace.start(b[0].astype(F32))
            for i, t in enumerate(_rhs7(*b)):
                store_weight(WO, i, c * LANES // GR, c * LANES % GR + hl * 32, ds(col, LANES), t)
                pace.finish(_words(t)[i % 2 * 8:])

        pace = _Pacer(j)
        row = pl.multiple_of(j * RB, RB)
        _emit(
            (0, 1, project(pace, j, None, weight(WKV), k_v, HALO)),
            (1, 2, project(pace, j, None, weight(WKV, 7 * PER), v_v, HALO)),
            (0, 1.85, ffn_weight_steps(pace, j)),
            (0, 1.2, permute_q_steps(pace, j)),
            (0.2, 1.95, [lambda c=c, hl=hl: wo_step(c, j // NI * 2 + hl)
                         for c in range(4) for hl in range(2)]),
            (0.25, 1, first_values(pace, jnp.maximum(j - 1, 0))),
            (1.25, 1.93, softmax_steps(
                pace, q_v.at[0, :, pl.ds(row, H + RB)], k_v.at[0, :, pl.ds(row, HALO + H + RB)],
                prob.at[:, pl.ds(row, H + RB)],
                [s * H + r for s in range(2) for r in range(0, RB, SB)], row)),
        )
    _loop("phase_kv", NT, phase_kv)

    def first_output(_):
        pace = _Pacer()
        _emit((0, 1, first_values(pace, jnp.int32(NT - 1)) + output_steps(pace, 0, 0)
               + hn_steps(pace, 0)))
    _loop("first_output", 1, first_output)

    def phase_ffn(j):
        nxt = last(j + 1)
        slot = j % 2
        pace = _Pacer(j)
        gate = {}

        def gate_done(n, *c):
            gate[n] = [_gelu(t) for t in c]

        def up_done(n, *c):
            for i, t in enumerate(_lhs7(*[g * u for g, u in zip(gate.pop(n), c)])):
                act[i, :, n:n + TN] = _words(t)

        def down_done(n, *c):
            for b, t in enumerate(c):
                cols = pl.ds(b % 2 * DH + n, TN)
                out_v[ds(j * T + b // 2 * H, H), cols] = (
                    h_v[slot, pl.ds(b // 2 * H, H), cols] + t).astype(BF16)

        g = _matmul(pace, lambda i: hn[i], ffn_weight(ffn_w[0]), FH, gate_done)
        u = _matmul(pace, lambda i: hn[i], ffn_weight(ffn_w[1]), FH, up_done)
        gu = [f for n in range(0, len(g), 7) for f in g[n:n + 7] + u[n:n + 7]]
        _emit(
            (0, 1, gu),
            (1, 2, output_steps(pace, nxt, 1 - slot)),
            (2, 3, _matmul(pace, lambda i: act[i], ffn_weight(ffn_w[2]), DH, down_done)),
            (0.01, 0.58, softmax_steps(pace, q_v.at[nxt], k_v.at[nxt], prob, range(0, T, SB))),
            (0.58, 0.99, value_steps(pace, prob, v_v.at[nxt], attn, range(0, H, RB))),
            (2.05, 2.9, hn_steps(pace, 1 - slot)),
        )
        out_copy(j).start()
    _loop("phase_ffn", NT, phase_ffn)
    for j in range(NT):
        out_copy(j).wait()


@jax.jit
def pallas_sequential_preLN__sliding_local_dilated__glu_gated_geglu__prompt_kernel(
    A_x: jax.Array,
    A_wqkv: jax.Array,
    A_wo: jax.Array,
    B_x: jax.Array,
    B_w_gate: jax.Array,
    B_w_up: jax.Array,
    B_w_down: jax.Array,
):
    del B_x
    B, S, D = A_x.shape
    F = B_w_gate.shape[1]
    DH, FH = D // 2, F // 2
    NT = S // T
    NI = NT // 2
    assert B == 1 and D == 8 * LANES and NI * LANES == DH and FH % GR == 0 and 2 * GR == DH
    any_spec = pl.BlockSpec(memory_space=pl.ANY)
    out = pl.pallas_call(
        _kernel,
        in_specs=[any_spec] * 6,
        out_specs=any_spec,
        out_shape=jax.ShapeDtypeStruct((S, D), A_x.dtype),
        scratch_shapes=[
            pltpu.VMEM((S + T, D), BF16),
            pltpu.VMEM((NQ, D // GR, GR // NQ, D), BF16),
            pltpu.VMEM((NT, D // GR, GR // NI, D), BF16),
            pltpu.VMEM((D, D), BF16),
            pltpu.VMEM((T, D), F32),
            [pltpu.VMEM((n * 7 * DH // GR, GR // 2, DH), U32)
             for n in (1, 2, 1)],
            [(pltpu.VMEM((k // GR, GR, n), BF16),
              pltpu.VMEM((3, k // 2 // GR, GR, n // 2), BF16))
             for k, n in ((D, F), (D, F), (F, D))],
            pltpu.VMEM((7 * NT + 7, H // 2, DH), U32),
            pltpu.VMEM((7, H // 2, DH), U32),
            pltpu.VMEM((7, H // 2, DH), U32),
            pltpu.VMEM((WINDOW, T, LANES), F32),
            pltpu.VMEM((7, H // 2, FH), U32),
            pltpu.VMEM((NT, 8, T, LANES), F32),
            pltpu.VMEM((NT, 8, T, LANES), F32),
            pltpu.VMEM((NT + 1, 8, HALO + T, LANES), F32),
            pltpu.VMEM((NT + 1, 8, HALO + T, LANES), F32),
            pltpu.VMEM((2, T, D), F32),
            pltpu.VMEM((S, D), BF16),
            pltpu.SemaphoreType.DMA((NT + 1,)),
            pltpu.SemaphoreType.DMA((NQ,)),
            pltpu.SemaphoreType.DMA((2 * NI,)),
            pltpu.SemaphoreType.DMA(()),
            pltpu.SemaphoreType.DMA((NT,)),
            pltpu.SemaphoreType.DMA((NT,)),
        ],
        compiler_params=pltpu.CompilerParams(vmem_limit_bytes=124 * 2**20),
    )(A_x.reshape(S, D), A_wqkv.reshape(D // GR, GR, 3 * D), A_wo,
      B_w_gate.reshape(D // GR, GR, F), B_w_up.reshape(D // GR, GR, F),
      B_w_down.reshape(F // GR, GR, D))
    return out.reshape(B, S, D)
```

```python
import jax
import jax.numpy as jnp
from jax import lax
import jax.experimental.pallas as pl
import jax.experimental.pallas.tpu as pltpu

HEAD_DIM = 32
WINDOW = 8
DILATION = 2
HALO = 16
LANES = 128
T = 256
H = T // 2
SB = 8
RB = 16
TN = 128
PLAIN = (1, 4)
GR = 256
NQ = 4
SCOPES = False
F32 = jnp.float32
BF16 = jnp.bfloat16
U32 = jnp.uint32


def _words(x):
    return pltpu.bitcast(x, U32)


def _halves(x):
    return pltpu.bitcast(x, BF16)


def _loop(name, n, body):
    def step(j, carry):
        if SCOPES:
            with jax.named_scope(name):
                body(j)
        else:
            body(j)
        return carry
    lax.fori_loop(0, n, step, 0)


def _emit(*stages):
    order = []
    for s, (lo, hi, steps) in enumerate(stages):
        order += [(lo + (hi - lo) * i / len(steps), s, i, f) for i, f in enumerate(steps)]
    for _, _, _, f in sorted(order, key=lambda t: t[:3]):
        f()


def _pipelined(pieces, depth):
    def step(t):
        for g in reversed(pieces[max(t - depth + 1, 0):t + 1]):
            next(g, None)
    return [lambda t=t: step(t) for t in range(len(pieces) + depth - 1)]


class _Pacer:
    def __init__(self, step=None):
        self.never = None if step is None else jnp.full((8, LANES), step, jnp.int32) < 0
        self.products = []
        self.due = []

    def _tie(self, x, others):
        regs = [[x[r:r + 8, c:c + LANES] for c in range(0, x.shape[1], LANES)]
                for r in range(0, x.shape[0], 8)]
        for k, other in enumerate(others):
            row, col = k % len(regs), k // len(regs) % len(regs[0])
            if other.dtype != x.dtype:
                other = pltpu.bitcast(other, x.dtype)
            regs[row][col] = jnp.where(self.never, other[:8, :LANES], regs[row][col])
        return jnp.concatenate([jnp.concatenate(row, axis=1) for row in regs], axis=0)

    def start(self, x, lag=3):
        if self.never is None or len(self.products) < lag:
            return x
        return self._tie(x, [self.products[-lag]] * (x.shape[0] // 8))

    def finish(self, x):
        if self.never is not None:
            self.due.append(x)

    def dot(self, lhs_words, rhs):
        if self.due:
            lhs_words = self._tie(lhs_words, self.due)
            self.due = []
        self.products.append(jnp.dot(_halves(lhs_words), rhs, preferred_element_type=F32))
        return self.products[-1]


def _gelu(x):
    c = 0.7978845608028654
    hx = 0.5 * x
    return hx + hx * jnp.tanh(x * (c + (c * 0.044715) * (x * x)))


def _lhs7(a11, a12, a21, a22):
    return [t.astype(BF16) for t in
            (a11 + a22, a21 + a22, a11, a22, a11 + a12, a21 - a11, a12 - a22)]


def _rhs7(b11, b12, b21, b22):
    f11, f12, f21, f22 = (b.astype(F32) for b in (b11, b12, b21, b22))
    return [t.astype(BF16) for t in
            (f11 + f22, b11, f12 - f22, f21 - f11, b22, f11 + f12, f21 + f22)]


def _strassen(pace, lhs, rhs, done):
    c = {}

    def m(i):
        return pace.dot(lhs(i), rhs(i))

    def s0():
        c["m1"] = m(0)

    def s1():
        c["m2"] = m(1)
        c[22] = c["m1"] - c["m2"]

    def s2():
        t = m(3)
        c[21] = c["m2"] + t
        c[11] = c["m1"] + t

    def s3():
        c["m5"] = m(4)
        c[11] = c[11] - c["m5"]

    def s4():
        t = m(2)
        c[12] = c["m5"] + t
        c[22] = c[22] + t

    def s5():
        c[11] = c[11] + m(6)

    def s6():
        done(c[11], c[12], c[21], c[22] + m(5))

    return [s0, s1, s2, s3, s4, s5, s6]


def _matmul(pace, lhs, rhs, width, done):
    steps = []
    for n in range(0, width, TN):
        steps += _strassen(pace, lhs, lambda i, n=n: rhs(i, n), lambda *c, n=n: done(n, *c))
    return steps


def _permute_cols(chunks):
    blk = lax.broadcasted_iota(jnp.int32, chunks[0].shape, 1) // 4
    a = [pltpu.roll(chunks[c], 4 * c, 1) if c else chunks[c] for c in range(8)]
    yield
    e = [a[(-i) % 8] for i in range(8)]
    for s in (1, 2, 4):
        e = [jnp.where((blk & s) != 0, e[(i - s) % 8], e[i]) for i in range(8)]
    e = [pltpu.roll(e[c], LANES - 4 * c, 1) if c else e[c] for c in range(8)]
    yield
    return e


def _permuted_rows(ref, c, hl, cols):
    parts = []
    for cp in range(8):
        r = c * 4
        u = _words(ref[pl.ds(pl.multiple_of(cp * LANES + hl * 32 + r // 16 * 16, 16), 16), cols])
        parts.append(u[r % 16 // 2:r % 16 // 2 + 2, :])
    return _halves(jnp.concatenate(parts, axis=0))


def _kernel(x_hbm, wqkv_hbm, wo_hbm, wg_hbm, wu_hbm, wd_hbm, out_hbm,
            x_v, wq_raw, wkv_raw, wo_raw, centred, w_ops, ffn_w, a_ops, hn, attn, prob, act,
            q_raw, q_v, k_v, v_v, h_v, out_v,
            sem_x, sem_q, sem_kv, sem_o, sem_f, sem_out):
    S, D = x_hbm.shape
    DH = D // 2
    FH = wg_hbm.shape[2] // 2
    NT = S // T
    NI = NT // 2
    QR = GR // NQ
    KR = GR // NI
    FR = GR // NT
    GROUP = H // NI
    PER = DH // GR
    WQ, WKV, WO = range(3)

    def ds(start, size):
        return pl.ds(start if isinstance(start, int) else pl.multiple_of(start, size), size)

    def last(j):
        return min(j, NT - 1) if isinstance(j, int) else jnp.minimum(j, NT - 1)

    def x_copy(j):
        return pltpu.make_async_copy(x_hbm.at[ds(last(j) * T, T)], x_v.at[ds(j * T, T)],
                                     sem_x.at[j])

    def wq_copy(j):
        return pltpu.make_async_copy(wqkv_hbm.at[:, ds(j * QR, QR), pl.ds(0, D)],
                                     wq_raw.at[j], sem_q.at[j])

    def wkv_copy(j):
        return pltpu.make_async_copy(
            wqkv_hbm.at[:, ds(j % NI * KR, KR), ds((1 + j // NI) * D, D)],
            wkv_raw.at[j], sem_kv.at[j])

    wo_copy = pltpu.make_async_copy(wo_hbm, wo_raw, sem_o)

    def ffn_copies(j):
        rows = ds(j * FR, FR)
        return [pltpu.make_async_copy(src.at[:, rows], dst.at[:, rows], sem_f.at[j])
                for src, (dst, _) in zip((wg_hbm, wu_hbm, wd_hbm), ffn_w)]

    def out_copy(j):
        return pltpu.make_async_copy(out_v.at[ds(j * T, T)], out_hbm.at[ds(j * T, T)],
                                     sem_out.at[j])

    def store_weight(m, i, g, row, col, t):
        w_ops[m][i * PER + g, ds(row // 2, t.shape[0] // 2), col] = _words(t)

    def weight(m, first=0):
        return lambda i, n: _halves(
            w_ops[m][pl.ds(first + i * PER, PER), :, n:n + TN].reshape(DH // 2, TN))

    def norm_steps(pace, load_rows, store):
        def piece(r):
            def load():
                return jnp.concatenate([load_rows(s * H + r).astype(F32) for s in range(2)], axis=0)
            m = jnp.mean(pace.start(load()), axis=-1, keepdims=True)
            yield
            c = load() - m
            centred[pl.ds(2 * r, 2 * RB), :] = c
            scale = lax.rsqrt(jnp.mean(c * c, axis=-1, keepdims=True) + 1e-5)
            yield
            y = centred[pl.ds(2 * r, 2 * RB), :] * scale
            for i, t in enumerate(_lhs7(y[:RB, :DH], y[:RB, DH:], y[RB:, :DH], y[RB:, DH:])):
                store(i, pl.ds(r // 2, RB // 2), _words(t))
                pace.finish(_words(t)[:, i % 4 * LANES:(i % 4 + 1) * LANES])
        return _pipelined([piece(r) for r in range(0, H, RB)], 3)

    def xn_steps(pace, j, *copies):
        def store(i, rows, t):
            a_ops[7 * j + i, rows, :] = t
            for c in copies:
                c[i, rows, :] = t
        return norm_steps(pace, lambda r: x_v[ds(j * T + r, RB), :], store)

    def hn_steps(pace, slot):
        def store(i, rows, t):
            hn[i, rows, :] = t
        return norm_steps(pace, lambda r: h_v[slot, pl.ds(r, RB), :], store)

    def kv_weight_steps(pace, raw, first, row0):
        def piece(g, r):
            u = [jnp.concatenate(
                [_words(raw[kh * PER + g, pl.ds(r, RB), pl.ds(c * LANES, LANES)])
                 for kh in range(2)], axis=0) for c in range(8)]
            u = yield from _permute_cols(u[:1] + [pace.start(u[1])] + u[2:])
            for c in range(4):
                b = [_halves(u[nh * 4 + c][kh * RB // 2:(kh + 1) * RB // 2])
                     for kh in range(2) for nh in range(2)]
                for i, t in enumerate(_rhs7(*b)):
                    store_weight(WKV, i, first + g, row0 + r, pl.ds(c * LANES, LANES), t)
                    if i >= 5:
                        pace.finish(_words(t))
        return _pipelined([piece(g, r) for r in range(0, raw.shape[1], RB)
                           for g in range(PER)], 3)

    def ffn_index(w, i, g, rows, n, width):
        blocks, extra = w
        _, per, _, half = extra.shape
        if 1 <= i <= 4:
            g = pl.ds((i - 1) // 2 * per, per) if g is None else (i - 1) // 2 * per + g
            return blocks, (g, rows, pl.ds((i - 1) % 2 * half + n, width))
        return extra, (i % 4, slice(None) if g is None else g, rows, pl.ds(n, width))

    def ffn_weight_steps(pace, j):
        def step(w, g, n):
            where = [ffn_index(w, i, g, ds(j * FR, FR), n, 2 * LANES) for i in range(7)]
            blocks = [ref[idx] for ref, idx in where[1:5]]
            blocks[0] = pace.start(blocks[0].astype(F32), 3)
            pace.finish(blocks[0])
            for i, t in enumerate(_rhs7(*blocks)):
                if i not in PLAIN:
                    ref, idx = where[i]
                    ref[idx] = t
        steps = [[lambda w=w, g=g, n=n: step(w, g, n) for g in range(w[1].shape[1])
                  for n in range(0, w[1].shape[3], 2 * LANES)] for w in ffn_w]
        return [f for group in zip(*steps) for f in group]

    def ffn_weight(w):
        def load(i, n):
            ref, idx = ffn_index(w, i, None, slice(None), n, TN)
            return ref[idx].reshape(w[1].shape[1] * GR, TN)
        return load

    def permute_q_steps(pace, j):
        def piece(r):
            q = [q_raw[j, c, pl.ds(r, 2 * RB), :] for c in range(8)]
            q = yield from _permute_cols(q[:1] + [pace.start(q[1])] + q[2:])
            for c in range(8):
                q_v[j, c, pl.ds(r, 2 * RB), :] = q[c]
                pace.finish(q[c][c % 4 * 8:])
        return _pipelined([piece(r) for r in range(0, T, 2 * RB)], 3)

    def project(pace, j, lhs, rhs, dst, halo):
        def done(n, *c):
            for b, t in enumerate(c):
                chunk = (b % 2 * DH + n) // LANES
                dst[j, chunk, pl.ds(halo + b // 2 * H, H), :] = t
                if halo and b // 2:
                    dst[j + 1, chunk, pl.ds(0, halo), :] = t[H - halo:]
        return _matmul(pace, lhs or (lambda i: a_ops[7 * j + i]), rhs, DH, done)

    def softmax_steps(pace, q, k, out, rows, first=None):
        def piece(r):
            logits = [None] * WINDOW
            for c in range(8):
                qc = q[c, pl.ds(r, SB), :]
                if c == 0:
                    qc = pace.start(qc)
                for w in range(WINDOW):
                    t = qc * k[c, pl.ds(HALO + r - DILATION * w, SB), :]
                    logits[w] = t if c == 0 else logits[w] + t
            lane = lax.broadcasted_iota(jnp.int32, (SB, LANES), 1)
            for s in (1, 2):
                rolled = [(pltpu.roll(l, s, 1), pltpu.roll(l, LANES - s, 1)) for l in logits]
                yield
                logits = [l + jnp.where((lane & s) != 0, a, b)
                          for l, (a, b) in zip(logits, rolled)]
            for w in range(WINDOW):
                l = logits[w] * (HEAD_DIM ** -0.5)
                if first is not None and r < DILATION * w:
                    pos = first + r + lax.broadcasted_iota(jnp.int32, (SB, LANES), 0)
                    l = jnp.where(pos >= DILATION * w, l, -1e9)
                logits[w] = l
            m = logits[0]
            for w in range(1, WINDOW):
                m = jnp.maximum(m, logits[w])
            e = [jnp.exp(l - m) for l in logits]
            total = e[0]
            for w in range(1, WINDOW):
                total = total + e[w]
            inv = 1.0 / total
            for w in range(WINDOW):
                p = e[w] * inv
                out[w, pl.ds(r, SB), :] = p
                pace.finish(p)
        return _pipelined([piece(r) for r in rows], 3)

    def value_steps(pace, weights, v, out, rows):
        def piece(r, c):
            blocks = []
            for row in (r, H + r):
                for chunk in (c, c + 4):
                    for w in range(WINDOW):
                        p = weights[w, pl.ds(row, RB), :]
                        t = (pace.start(p, 4) if w == 0 else p) * v[
                            chunk, pl.ds(HALO + row - DILATION * w, RB), :]
                        o = t if w == 0 else o + t
                    blocks.append(o)
                    pace.finish(o)
                    pace.finish(o[8:])
                    yield
            for i, t in enumerate(_lhs7(*blocks)):
                out[i, pl.ds(r // 2, RB // 2), pl.ds(c * LANES, LANES)] = _words(t)
                pace.finish(_words(t))
        pieces = [piece(r, c) for r in rows for c in range(4)]
        return [lambda g=g: next(g, None) for g in pieces for _ in range(5)]

    def output_steps(pace, j, slot):
        def done(n, *c):
            for b, t in enumerate(c):
                cols = pl.ds(b % 2 * DH + n, TN)
                h_v[slot, pl.ds(b // 2 * H, H), cols] = (
                    x_v[ds(j * T + b // 2 * H, H), cols].astype(F32) + t)
        return _matmul(pace, lambda i: attn[slot, i], weight(WO), DH, done)

    x_copy(0).start()
    wq_copy(0).start()
    wq_copy(1).start()
    prob[:, pl.ds(0, H + GROUP), :] = jnp.zeros((WINDOW, H + GROUP, LANES), F32)
    v_v[0, :, pl.ds(0, HALO + H + GROUP), :] = jnp.zeros((8, HALO + H + GROUP, LANES), F32)
    k_v[0, :, pl.ds(0, HALO), :] = jnp.zeros((8, HALO, LANES), F32)
    h_v[1] = jnp.zeros((T, D), F32)
    x_copy(0).wait()
    for j in range(2, NQ):
        wq_copy(j).start()
    _emit((0, 1, xn_steps(_Pacer(), 0, hn)))
    x_copy(1).start()
    wkv_copy(0).start()
    x_copy(2).start()
    wkv_copy(1).start()

    def prepare_q(j):
        wq_copy(j).wait()
        for g in range(PER):
            for r in range(0, QR, RB):
                for n in range(0, DH, 2 * LANES):
                    b = [wq_raw[j, kh * PER + g, pl.ds(r, RB), pl.ds(nh * DH + n, 2 * LANES)]
                         for kh in range(2) for nh in range(2)]
                    for i, t in enumerate(_rhs7(*b)):
                        store_weight(WQ, i, g, j * QR + r, pl.ds(n, 2 * LANES), t)
    _loop("prepare_q", NQ, prepare_q)
    for t in range(2, NT):
        x_copy(t + 1).start()
        wkv_copy(t).start()
    for c in [wo_copy] + ffn_copies(0) + ffn_copies(1):
        c.start()

    def phase_q(j):
        for t, (cur, nxt) in ((2 * j, (hn, attn.at[0])), (2 * j + 1, (attn.at[0], hn))):
            x_copy(t + 1).wait()
            wkv_copy(t).wait()
            pace = _Pacer(j)
            _emit(
                (0, 1, project(pace, t, lambda i: cur[i], weight(WQ), q_raw, 0)),
                (-0.05, 0.93, xn_steps(pace, t + 1, nxt)),
                (0.0, 0.97, kv_weight_steps(pace, wkv_raw.at[t], t // NI * 7 * PER,
                                             t % NI * KR)),
            )
    _loop("phase_q", NI, phase_q)
    for t in range(2, NT):
        for c in ffn_copies(t):
            c.start()
    wo_copy.wait()

    def first_values(pace, g):
        for c in range(8):
            v_v[0, c, pl.ds(0, HALO), :] = jnp.broadcast_to(
                v_v[0, c, pl.ds(HALO, 1), :], (HALO, LANES))
        tile, row = g // NI, pl.multiple_of(g % NI * GROUP, GROUP)
        return value_steps(pace, prob.at[:, pl.ds(row, H + GROUP)],
                           v_v.at[tile, :, pl.ds(row, HALO + H + GROUP)],
                           attn.at[tile, :, ds(row // 2, GROUP // 2)], range(0, GROUP, RB))

    def phase_kv(j):
        for c in ffn_copies(j):
            c.wait()

        def wo_step(c, hl):
            col = j % NI * LANES
            b = [_permuted_rows(wo_raw, kh * 4 + c, hl, ds(s * DH + col, LANES))
                 for kh in range(2) for s in range(2)]
            b[0] = pace.start(b[0].astype(F32))
            for i, t in enumerate(_rhs7(*b)):
                store_weight(WO, i, c * LANES // GR, c * LANES % GR + hl * 32, ds(col, LANES), t)
                pace.finish(_words(t)[i % 2 * 8:])

        pace = _Pacer(j)
        tile, row = j // NI, pl.multiple_of(j % NI * GROUP, GROUP)
        _emit(
            (0, 1, project(pace, j, None, weight(WKV), k_v, HALO)),
            (1, 2, project(pace, j, None, weight(WKV, 7 * PER), v_v, HALO)),
            (0, 1.85, ffn_weight_steps(pace, j)),
            (0, 1.05, permute_q_steps(pace, j)),
            (0.2, 1.95, [lambda c=c, hl=hl: wo_step(c, j // NI * 2 + hl)
                         for c in range(4) for hl in range(2)]),
            (0.25, 1, first_values(pace, jnp.maximum(j - 1, 0))),
            (1.1, 1.95, softmax_steps(
                pace, q_v.at[tile, :, pl.ds(row, H + GROUP)],
                k_v.at[tile, :, pl.ds(row, HALO + H + GROUP)], prob.at[:, pl.ds(row, H + GROUP)],
                [s * H + r for s in range(2) for r in range(0, GROUP, SB)], tile * T + row)),
        )
    _loop("phase_kv", NT, phase_kv)
    _emit((0, 1, first_values(_Pacer(), jnp.int32(NT - 1))))

    def ffn(j):
        nxt = last(j + 2)
        slot = j % 2
        pace = _Pacer(j)
        gate = {}

        def gate_done(n, *c):
            gate[n] = [_gelu(t) for t in c]

        def up_done(n, *c):
            for i, t in enumerate(_lhs7(*[g * u for g, u in zip(gate.pop(n), c)])):
                act[i, :, n:n + TN] = _words(t)

        def down_done(n, *c):
            for b, t in enumerate(c):
                cols = pl.ds(b % 2 * DH + n, TN)
                out_v[ds(j * T + b // 2 * H, H), cols] = (
                    h_v[slot, pl.ds(b // 2 * H, H), cols] + t).astype(BF16)

        g = _matmul(pace, lambda i: hn[i], ffn_weight(ffn_w[0]), FH, gate_done)
        u = _matmul(pace, lambda i: hn[i], ffn_weight(ffn_w[1]), FH, up_done)
        gu = [f for n in range(0, len(g), 7) for f in g[n:n + 7] + u[n:n + 7]]
        _emit(
            (0, 1, gu),
            (1, 1.5, _matmul(pace, lambda i: act[i], ffn_weight(ffn_w[2]), DH, down_done)),
            (0.01, 0.58, softmax_steps(pace, q_v.at[nxt], k_v.at[nxt], prob, range(0, T, SB))),
            (0.58, 0.99, value_steps(pace, prob, v_v.at[nxt], attn.at[slot], range(0, H, RB))),
        )
        out_copy(j).start()

    def phase_ffn(t):
        @pl.when(t < NT)
        def _():
            pace = _Pacer(t)
            _emit((0, 1, output_steps(pace, t, t % 2)),
                  (0, 0.95, hn_steps(pace, 1 - t % 2)))

        @pl.when(t == NT)
        def _():
            _emit((0, 1, hn_steps(_Pacer(), (NT - 1) % 2)))

        pl.when(t > 0)(lambda: ffn(t - 1))
    _loop("phase_ffn", NT + 1, phase_ffn)
    for j in range(NT):
        out_copy(j).wait()


@jax.jit
def pallas_sequential_preLN__sliding_local_dilated__glu_gated_geglu__prompt_kernel(
    A_x: jax.Array,
    A_wqkv: jax.Array,
    A_wo: jax.Array,
    B_x: jax.Array,
    B_w_gate: jax.Array,
    B_w_up: jax.Array,
    B_w_down: jax.Array,
):
    del B_x
    B, S, D = A_x.shape
    F = B_w_gate.shape[1]
    DH, FH = D // 2, F // 2
    NT = S // T
    NI = NT // 2
    assert B == 1 and D == 8 * LANES and NI * LANES == DH and FH % GR == 0 and 2 * GR == DH
    any_spec = pl.BlockSpec(memory_space=pl.ANY)
    out = pl.pallas_call(
        _kernel,
        in_specs=[any_spec] * 6,
        out_specs=any_spec,
        out_shape=jax.ShapeDtypeStruct((S, D), A_x.dtype),
        scratch_shapes=[
            pltpu.VMEM((S + T, D), BF16),
            pltpu.VMEM((NQ, D // GR, GR // NQ, D), BF16),
            pltpu.VMEM((NT, D // GR, GR // NI, D), BF16),
            pltpu.VMEM((D, D), BF16),
            pltpu.VMEM((T, D), F32),
            [pltpu.VMEM((n * 7 * DH // GR, GR // 2, DH), U32)
             for n in (1, 2, 1)],
            [(pltpu.VMEM((k // GR, GR, n), BF16),
              pltpu.VMEM((3, k // 2 // GR, GR, n // 2), BF16))
             for k, n in ((D, F), (D, F), (F, D))],
            pltpu.VMEM((7 * NT + 7, H // 2, DH), U32),
            pltpu.VMEM((7, H // 2, DH), U32),
            pltpu.VMEM((2, 7, H // 2, DH), U32),
            pltpu.VMEM((WINDOW, T, LANES), F32),
            pltpu.VMEM((7, H // 2, FH), U32),
            pltpu.VMEM((NT, 8, T, LANES), F32),
            pltpu.VMEM((NT, 8, T, LANES), F32),
            pltpu.VMEM((NT + 1, 8, HALO + T, LANES), F32),
            pltpu.VMEM((NT + 1, 8, HALO + T, LANES), F32),
            pltpu.VMEM((2, T, D), F32),
            pltpu.VMEM((S, D), BF16),
            pltpu.SemaphoreType.DMA((NT + 1,)),
            pltpu.SemaphoreType.DMA((NQ,)),
            pltpu.SemaphoreType.DMA((2 * NI,)),
            pltpu.SemaphoreType.DMA(()),
            pltpu.SemaphoreType.DMA((NT,)),
            pltpu.SemaphoreType.DMA((NT,)),
        ],
        compiler_params=pltpu.CompilerParams(vmem_limit_bytes=124 * 2**20),
    )(A_x.reshape(S, D), A_wqkv.reshape(D // GR, GR, 3 * D), A_wo,
      B_w_gate.reshape(D // GR, GR, F), B_w_up.reshape(D // GR, GR, F),
      B_w_down.reshape(F // GR, GR, D))
    return out.reshape(B, S, D)
```

```python
import jax
import jax.numpy as jnp
from jax import lax
import jax.experimental.pallas as pl
import jax.experimental.pallas.tpu as pltpu

HEAD_DIM = 32
WINDOW = 8
DILATION = 2
HALO = 16
LANES = 128
T = 256
H = T // 2
SB = 8
RB = 16
TN = 128
PLAIN = (1, 4)
GR = 256
SCOPES = False
F32 = jnp.float32
BF16 = jnp.bfloat16
U32 = jnp.uint32


def _words(x):
    return pltpu.bitcast(x, U32)


def _halves(x):
    return pltpu.bitcast(x, BF16)


def _loop(name, n, body):
    def step(j, carry):
        if SCOPES:
            with jax.named_scope(name):
                body(j)
        else:
            body(j)
        return carry
    lax.fori_loop(0, n, step, 0)


def _emit(*stages):
    order = []
    for s, (lo, hi, steps) in enumerate(stages):
        order += [(lo + (hi - lo) * i / len(steps), s, i, f) for i, f in enumerate(steps)]
    for _, _, _, f in sorted(order, key=lambda t: t[:3]):
        f()


def _pipelined(pieces, depth):
    def step(t):
        for g in reversed(pieces[max(t - depth + 1, 0):t + 1]):
            next(g, None)
    return [lambda t=t: step(t) for t in range(len(pieces) + depth - 1)]


class _Pacer:
    def __init__(self, step=None):
        self.never = None if step is None else jnp.full((8, LANES), step, jnp.int32) < 0
        self.products = []
        self.due = []

    def _tie(self, x, others):
        regs = [[x[r:r + 8, c:c + LANES] for c in range(0, x.shape[1], LANES)]
                for r in range(0, x.shape[0], 8)]
        for k, other in enumerate(others):
            row, col = k % len(regs), k // len(regs) % len(regs[0])
            if other.dtype != x.dtype:
                other = pltpu.bitcast(other, x.dtype)
            regs[row][col] = jnp.where(self.never, other[:8, :LANES], regs[row][col])
        return jnp.concatenate([jnp.concatenate(row, axis=1) for row in regs], axis=0)

    def start(self, x, lag=3):
        if self.never is None or len(self.products) < lag:
            return x
        return self._tie(x, [self.products[-lag]] * (x.shape[0] // 8))

    def finish(self, x):
        if self.never is not None:
            self.due.append(x)

    def dot(self, lhs_words, rhs):
        if self.due:
            lhs_words = self._tie(lhs_words, self.due)
            self.due = []
        self.products.append(jnp.dot(_halves(lhs_words), rhs, preferred_element_type=F32))
        return self.products[-1]


def _gelu(x):
    c = 0.7978845608028654
    hx = 0.5 * x
    return hx + hx * jnp.tanh(x * (c + (c * 0.044715) * (x * x)))


def _lhs7(a11, a12, a21, a22):
    return [t.astype(BF16) for t in
            (a11 + a22, a21 + a22, a11, a22, a11 + a12, a21 - a11, a12 - a22)]


def _rhs7(b11, b12, b21, b22):
    f11, f12, f21, f22 = (b.astype(F32) for b in (b11, b12, b21, b22))
    return [t.astype(BF16) for t in
            (f11 + f22, b11, f12 - f22, f21 - f11, b22, f11 + f12, f21 + f22)]


def _strassen(pace, lhs, rhs, done):
    c = {}

    def m(i):
        return pace.dot(lhs(i), rhs(i))

    def s0():
        c["m1"] = m(0)

    def s1():
        c["m2"] = m(1)
        c[22] = c["m1"] - c["m2"]

    def s2():
        t = m(3)
        c[21] = c["m2"] + t
        c[11] = c["m1"] + t

    def s3():
        c["m5"] = m(4)
        c[11] = c[11] - c["m5"]

    def s4():
        t = m(2)
        c[12] = c["m5"] + t
        c[22] = c[22] + t

    def s5():
        c[11] = c[11] + m(6)

    def s6():
        done(c[11], c[12], c[21], c[22] + m(5))

    return [s0, s1, s2, s3, s4, s5, s6]


def _matmul(pace, lhs, rhs, width, done):
    steps = []
    for n in range(0, width, TN):
        steps += _strassen(pace, lhs, lambda i, n=n: rhs(i, n), lambda *c, n=n: done(n, *c))
    return steps


def _permute_cols(chunks):
    blk = lax.broadcasted_iota(jnp.int32, chunks[0].shape, 1) // 4
    a = [pltpu.roll(chunks[c], 4 * c, 1) if c else chunks[c] for c in range(8)]
    yield
    e = [a[(-i) % 8] for i in range(8)]
    for s in (1, 2, 4):
        e = [jnp.where((blk & s) != 0, e[(i - s) % 8], e[i]) for i in range(8)]
    e = [pltpu.roll(e[c], LANES - 4 * c, 1) if c else e[c] for c in range(8)]
    yield
    return e


def _permuted_rows(ref, c, hl, cols):
    parts = []
    for cp in range(8):
        r = c * 4
        u = _words(ref[pl.ds(pl.multiple_of(cp * LANES + hl * 32 + r // 16 * 16, 16), 16), cols])
        parts.append(u[r % 16 // 2:r % 16 // 2 + 2, :])
    return _halves(jnp.concatenate(parts, axis=0))


def _kernel(x_hbm, wqkv_hbm, wo_hbm, wg_hbm, wu_hbm, wd_hbm, out_hbm,
            x_v, wq_raw, wkv_raw, wo_raw, centred, w_ops, ffn_w, a_ops, hn, attn, prob, act,
            q_raw, q_v, k_v, v_v, h_v, out_v,
            sem_x, sem_p, sem_q, sem_kv, sem_o, sem_f, sem_out):
    S, D = x_hbm.shape
    DH = D // 2
    FH = wg_hbm.shape[2] // 2
    NT = S // T
    NI = NT // 2
    FR = GR // NT
    NG = 2 * GR // RB
    KG = -(-NG // (NI - 1))
    GROUP = H // NI
    PER = DH // GR
    WQ, WKV, WO = range(3)

    def ds(start, size):
        return pl.ds(start if isinstance(start, int) else pl.multiple_of(start, size), size)

    def last(j):
        return min(j, NT - 1) if isinstance(j, int) else jnp.minimum(j, NT - 1)

    def x_copy(j):
        return pltpu.make_async_copy(x_hbm.at[ds(last(j) * T, T)], x_v.at[ds(j * T, T)],
                                     sem_x.at[j])

    def x_part_copy(n):
        return [pltpu.make_async_copy(x_hbm.at[ds(2 * T + s * H + n * GROUP, GROUP)],
                                      x_v.at[ds(2 * T + s * H + n * GROUP, GROUP)],
                                      sem_p.at[n]) for s in range(2)]

    def wq_copy(n):
        return pltpu.make_async_copy(wqkv_hbm.at[:, :, ds(n * 2 * TN, 2 * TN)],
                                     wq_raw.at[n], sem_q.at[n])

    def wkv_copies(j):
        copies = []
        for m in range(2):
            lo = max(j * KG * RB - m * GR, 0)
            hi = min((j + 1) * KG * RB - m * GR, GR)
            if lo < hi:
                copies.append(pltpu.make_async_copy(
                    wqkv_hbm.at[:, pl.ds(lo, hi - lo), pl.ds((1 + m) * D, D)],
                    wkv_raw.at[m, :, pl.ds(lo, hi - lo)], sem_kv.at[j]))
        return copies

    wo_copy = pltpu.make_async_copy(wo_hbm, wo_raw, sem_o)

    def ffn_copies(j):
        rows = ds(j * FR, FR)
        return [pltpu.make_async_copy(src.at[:, rows], dst.at[:, rows], sem_f.at[j])
                for src, (dst, _) in zip((wg_hbm, wu_hbm, wd_hbm), ffn_w)]

    def out_copy(j):
        return pltpu.make_async_copy(out_v.at[ds(j * T, T)], out_hbm.at[ds(j * T, T)],
                                     sem_out.at[j])

    def store_weight(m, i, g, row, col, t):
        w_ops[m][i * PER + g, ds(row // 2, t.shape[0] // 2), col] = _words(t)

    def weight(m, first=0):
        return lambda i, n: _halves(
            w_ops[m][pl.ds(first + i * PER, PER), :, ds(n, TN)].reshape(DH // 2, TN))

    def norm_steps(pace, load_rows, store, rows=range(0, H, RB)):
        def piece(r):
            def load():
                return jnp.concatenate([load_rows(s * H + r).astype(F32) for s in range(2)], axis=0)
            m = jnp.mean(pace.start(load()), axis=-1, keepdims=True)
            yield
            c = load() - m
            centred[ds(2 * r, 2 * RB), :] = c
            scale = lax.rsqrt(jnp.mean(c * c, axis=-1, keepdims=True) + 1e-5)
            yield
            y = centred[ds(2 * r, 2 * RB), :] * scale
            for i, t in enumerate(_lhs7(y[:RB, :DH], y[:RB, DH:], y[RB:, :DH], y[RB:, DH:])):
                store(i, ds(r // 2, RB // 2), _words(t))
                pace.finish(_words(t)[:, i % 4 * LANES:(i % 4 + 1) * LANES])
        return _pipelined([piece(r) for r in rows], 3)

    def xn_steps(pace, j, copy, *rows):
        def store(i, where, t):
            a_ops[7 * j + i, where, :] = t
            copy[i, where, :] = t
        return norm_steps(pace, lambda r: x_v[ds(j * T + r, RB), :], store, *rows)

    def hn_steps(pace, slot):
        def store(i, rows, t):
            hn[i, rows, :] = t
        return norm_steps(pace, lambda r: h_v[slot, pl.ds(r, RB), :], store)

    def q_weight_steps(pace, n):
        def step(g, r):
            top, bot = (wq_raw[n, kh * PER + g, pl.ds(r, 2 * RB), :] for kh in range(2))
            b11 = pace.start(top[:, :TN].astype(F32))
            for i, t in enumerate(_rhs7(b11, top[:, TN:], bot[:, :TN], bot[:, TN:])):
                store_weight(WQ, i, g, r, ds(n * TN, TN), t)
        return [lambda g=g, r=r: step(g, r) for g in range(PER) for r in range(0, GR, 2 * RB)]

    def kv_weight_steps(pace, j):
        def piece(g, group):
            m, row = group // (NG // 2), group % (NG // 2) * RB
            u = [jnp.concatenate(
                [_words(wkv_raw[m, kh * PER + g, ds(row, RB), pl.ds(c * LANES, LANES)])
                 for kh in range(2)], axis=0) for c in range(8)]
            u = yield from _permute_cols(u[:1] + [pace.start(u[1])] + u[2:])
            for c in range(4):
                b = [_halves(u[nh * 4 + c][kh * RB // 2:(kh + 1) * RB // 2])
                     for kh in range(2) for nh in range(2)]
                for i, t in enumerate(_rhs7(*b)):
                    store_weight(WKV, i, m * 7 * PER + g, row, pl.ds(c * LANES, LANES), t)
                    if i >= 5:
                        pace.finish(_words(t))
        return _pipelined([piece(g, jnp.minimum(j * KG + r, NG - 1)) for r in range(KG)
                           for g in range(PER)], 3)

    def ffn_index(w, i, g, rows, n, width):
        blocks, extra = w
        _, per, _, half = extra.shape
        if 1 <= i <= 4:
            g = pl.ds((i - 1) // 2 * per, per) if g is None else (i - 1) // 2 * per + g
            return blocks, (g, rows, pl.ds((i - 1) % 2 * half + n, width))
        return extra, (i % 4, slice(None) if g is None else g, rows, pl.ds(n, width))

    def ffn_weight_steps(pace, j):
        def step(w, g, n):
            where = [ffn_index(w, i, g, ds(j * FR, FR), n, 2 * LANES) for i in range(7)]
            blocks = [ref[idx] for ref, idx in where[1:5]]
            blocks[0] = pace.start(blocks[0].astype(F32), 3)
            pace.finish(blocks[0])
            for i, t in enumerate(_rhs7(*blocks)):
                if i not in PLAIN:
                    ref, idx = where[i]
                    ref[idx] = t
        steps = [[lambda w=w, g=g, n=n: step(w, g, n) for g in range(w[1].shape[1])
                  for n in range(0, w[1].shape[3], 2 * LANES)] for w in ffn_w]
        return [f for group in zip(*steps) for f in group]

    def ffn_weight(w):
        def load(i, n):
            ref, idx = ffn_index(w, i, None, slice(None), n, TN)
            return ref[idx].reshape(w[1].shape[1] * GR, TN)
        return load

    def permute_q_steps(pace, j):
        def piece(r):
            q = [q_raw[j, c, pl.ds(r, 2 * RB), :] for c in range(8)]
            q = yield from _permute_cols(q[:1] + [pace.start(q[1])] + q[2:])
            for c in range(8):
                q_v[j, c, pl.ds(r, 2 * RB), :] = q[c]
                pace.finish(q[c][c % 4 * 8:])
        return _pipelined([piece(r) for r in range(0, T, 2 * RB)], 3)

    def q_step(pace, j, lhs, n):
        def done(*c):
            for b, t in enumerate(c):
                q_raw[j, 2 * n + b % 2, pl.ds(b // 2 * H, H), :] = t
        return _strassen(pace, lambda i: lhs[i], lambda i: weight(WQ)(i, n * TN), done)

    def project(pace, j, rhs, dst):
        def done(n, *c):
            for b, t in enumerate(c):
                chunk = (b % 2 * DH + n) // LANES
                dst[j, chunk, pl.ds(HALO + b // 2 * H, H), :] = t
                if b // 2:
                    dst[j + 1, chunk, pl.ds(0, HALO), :] = t[H - HALO:]
        return _matmul(pace, lambda i: a_ops[7 * j + i], rhs, DH, done)

    def softmax_steps(pace, q, k, out, rows, first=None):
        def piece(r):
            logits = [None] * WINDOW
            for c in range(8):
                qc = q[c, pl.ds(r, SB), :]
                if c == 0:
                    qc = pace.start(qc)
                for w in range(WINDOW):
                    t = qc * k[c, pl.ds(HALO + r - DILATION * w, SB), :]
                    logits[w] = t if c == 0 else logits[w] + t
            lane = lax.broadcasted_iota(jnp.int32, (SB, LANES), 1)
            for s in (1, 2):
                rolled = [(pltpu.roll(l, s, 1), pltpu.roll(l, LANES - s, 1)) for l in logits]
                yield
                logits = [l + jnp.where((lane & s) != 0, a, b)
                          for l, (a, b) in zip(logits, rolled)]
            for w in range(WINDOW):
                l = logits[w] * (HEAD_DIM ** -0.5)
                if first is not None and r < DILATION * w:
                    pos = first + r + lax.broadcasted_iota(jnp.int32, (SB, LANES), 0)
                    l = jnp.where(pos >= DILATION * w, l, -1e9)
                logits[w] = l
            m = logits[0]
            for w in range(1, WINDOW):
                m = jnp.maximum(m, logits[w])
            e = [jnp.exp(l - m) for l in logits]
            total = e[0]
            for w in range(1, WINDOW):
                total = total + e[w]
            inv = 1.0 / total
            for w in range(WINDOW):
                p = e[w] * inv
                out[w, pl.ds(r, SB), :] = p
                pace.finish(p)
        return _pipelined([piece(r) for r in rows], 3)

    def value_steps(pace, weights, v, out, rows):
        def piece(r, c):
            blocks = []
            for row in (r, H + r):
                for chunk in (c, c + 4):
                    for w in range(WINDOW):
                        p = weights[w, pl.ds(row, RB), :]
                        t = (pace.start(p, 4) if w == 0 else p) * v[
                            chunk, pl.ds(HALO + row - DILATION * w, RB), :]
                        o = t if w == 0 else o + t
                    blocks.append(o)
                    pace.finish(o)
                    pace.finish(o[8:])
                    yield
            for i, t in enumerate(_lhs7(*blocks)):
                out[i, pl.ds(r // 2, RB // 2), pl.ds(c * LANES, LANES)] = _words(t)
                pace.finish(_words(t))
        pieces = [piece(r, c) for r in rows for c in range(4)]
        return [lambda g=g: next(g, None) for g in pieces for _ in range(5)]

    def output_steps(pace, j, slot):
        def done(n, *c):
            for b, t in enumerate(c):
                cols = pl.ds(b % 2 * DH + n, TN)
                h_v[slot, pl.ds(b // 2 * H, H), cols] = (
                    x_v[ds(j * T + b // 2 * H, H), cols].astype(F32) + t)
        return _matmul(pace, lambda i: attn[slot, i], weight(WO), DH, done)

    first = [x_copy(0), x_copy(1), wq_copy(0)]
    for c in first:
        c.start()
    for n in range(NI):
        for c in ([wq_copy(n + 1)] if n + 1 < NI else []) + x_part_copy(n):
            c.start()
    prob[:, pl.ds(0, H + GROUP), :] = jnp.zeros((WINDOW, H + GROUP, LANES), F32)
    v_v[0, :, pl.ds(0, HALO + H + GROUP), :] = jnp.zeros((8, HALO + H + GROUP, LANES), F32)
    k_v[0, :, pl.ds(0, HALO), :] = jnp.zeros((8, HALO, LANES), F32)
    h_v[1] = jnp.zeros((T, D), F32)
    for c, steps in zip(first, (xn_steps(_Pacer(), 0, hn), xn_steps(_Pacer(), 1, attn.at[0]),
                                q_weight_steps(_Pacer(), 0))):
        c.wait()
        _emit((0, 1, steps))
    for j in range(NI - 1):
        for c in [x_copy(2 * j + 3), x_copy(2 * j + 4)] + wkv_copies(j):
            c.start()

    def first_q(n):
        pl.when(n + 1 < NI)(lambda: wq_copy(n + 1).wait())
        for c in x_part_copy(n):
            c.wait()
        pace = _Pacer(n)
        _emit(
            (0, 1, q_step(pace, 0, hn, n) + q_step(pace, 1, attn.at[0], n)),
            (0, 0.9, q_weight_steps(pace, jnp.minimum(n + 1, NI - 1))),
            (0, 0.9, xn_steps(pace, 2, attn.at[1],
                              [n * GROUP + r for r in range(0, GROUP, RB)])),
        )
    _loop("first_q", NI, first_q)
    for c in [wo_copy] + ffn_copies(0) + ffn_copies(1):
        c.start()

    def phase_q(j):
        t = 2 * j + 2
        x_copy(t + 1).wait()
        x_copy(t + 2).wait()
        for k in range(NI - 1):
            @pl.when(j == k)
            def _():
                for c in wkv_copies(k):
                    c.wait()
        pace = _Pacer(j)
        _emit(
            (0, 1, [f for n in range(NI) for f in q_step(pace, t, attn.at[1], n)]),
            (1, 2, [f for n in range(NI) for f in q_step(pace, t + 1, hn, n)]),
            (-0.05, 0.97, xn_steps(pace, t + 1, hn)),
            (0.85, 1.93, xn_steps(pace, t + 2, attn.at[1])),
            (0, 1.97, kv_weight_steps(pace, j)),
        )
    _loop("phase_q", NI - 1, phase_q)
    for t in range(2, NT):
        for c in ffn_copies(t):
            c.start()
    wo_copy.wait()

    def first_values(pace, g):
        for c in range(8):
            v_v[0, c, pl.ds(0, HALO), :] = jnp.broadcast_to(
                v_v[0, c, pl.ds(HALO, 1), :], (HALO, LANES))
        tile, row = g // NI, pl.multiple_of(g % NI * GROUP, GROUP)
        return value_steps(pace, prob.at[:, pl.ds(row, H + GROUP)],
                           v_v.at[tile, :, pl.ds(row, HALO + H + GROUP)],
                           attn.at[tile, :, ds(row // 2, GROUP // 2)], range(0, GROUP, RB))

    def phase_kv(j):
        for c in ffn_copies(j):
            c.wait()

        def wo_step(c, hl):
            col = j % NI * LANES
            b = [_permuted_rows(wo_raw, kh * 4 + c, hl, ds(s * DH + col, LANES))
                 for kh in range(2) for s in range(2)]
            b[0] = pace.start(b[0].astype(F32))
            for i, t in enumerate(_rhs7(*b)):
                store_weight(WO, i, c * LANES // GR, c * LANES % GR + hl * 32, ds(col, LANES), t)
                pace.finish(_words(t)[i % 2 * 8:])

        pace = _Pacer(j)
        tile, row = j // NI, pl.multiple_of(j % NI * GROUP, GROUP)
        _emit(
            (0, 1, project(pace, j, weight(WKV), k_v)),
            (1, 2, project(pace, j, weight(WKV, 7 * PER), v_v)),
            (0, 1.85, ffn_weight_steps(pace, j)),
            (0, 1.05, permute_q_steps(pace, j)),
            (0.2, 1.95, [lambda c=c, hl=hl: wo_step(c, j // NI * 2 + hl)
                         for c in range(4) for hl in range(2)]),
            (0.25, 1, first_values(pace, jnp.maximum(j - 1, 0))),
            (1.1, 1.95, softmax_steps(
                pace, q_v.at[tile, :, pl.ds(row, H + GROUP)],
                k_v.at[tile, :, pl.ds(row, HALO + H + GROUP)], prob.at[:, pl.ds(row, H + GROUP)],
                [s * H + r for s in range(2) for r in range(0, GROUP, SB)], tile * T + row)),
        )
    _loop("phase_kv", NT, phase_kv)
    _emit((0, 1, first_values(_Pacer(), jnp.int32(NT - 1))))

    def ffn(j):
        nxt = last(j + 2)
        slot = j % 2
        pace = _Pacer(j)
        gate = {}

        def gate_done(n, *c):
            gate[n] = [_gelu(t) for t in c]

        def up_done(n, *c):
            for i, t in enumerate(_lhs7(*[g * u for g, u in zip(gate.pop(n), c)])):
                act[i, :, n:n + TN] = _words(t)

        def down_done(n, *c):
            for b, t in enumerate(c):
                cols = pl.ds(b % 2 * DH + n, TN)
                out_v[ds(j * T + b // 2 * H, H), cols] = (
                    h_v[slot, pl.ds(b // 2 * H, H), cols] + t).astype(BF16)

        g = _matmul(pace, lambda i: hn[i], ffn_weight(ffn_w[0]), FH, gate_done)
        u = _matmul(pace, lambda i: hn[i], ffn_weight(ffn_w[1]), FH, up_done)
        gu = [f for n in range(0, len(g), 7) for f in g[n:n + 7] + u[n:n + 7]]
        _emit(
            (0, 1, gu),
            (1, 1.5, _matmul(pace, lambda i: act[i], ffn_weight(ffn_w[2]), DH, down_done)),
            (0.01, 0.58, softmax_steps(pace, q_v.at[nxt], k_v.at[nxt], prob, range(0, T, SB))),
            (0.58, 0.99, value_steps(pace, prob, v_v.at[nxt], attn.at[slot], range(0, H, RB))),
        )
        out_copy(j).start()

    def phase_ffn(t):
        @pl.when(t < NT)
        def _():
            pace = _Pacer(t)
            _emit((0, 1, output_steps(pace, t, t % 2)),
                  (0, 0.95, hn_steps(pace, 1 - t % 2)))

        @pl.when(t == NT)
        def _():
            _emit((0, 1, hn_steps(_Pacer(), (NT - 1) % 2)))

        pl.when(t > 0)(lambda: ffn(t - 1))
    _loop("phase_ffn", NT + 1, phase_ffn)
    for j in range(NT):
        out_copy(j).wait()


@jax.jit
def pallas_sequential_preLN__sliding_local_dilated__glu_gated_geglu__prompt_kernel(
    A_x: jax.Array,
    A_wqkv: jax.Array,
    A_wo: jax.Array,
    B_x: jax.Array,
    B_w_gate: jax.Array,
    B_w_up: jax.Array,
    B_w_down: jax.Array,
):
    del B_x
    B, S, D = A_x.shape
    F = B_w_gate.shape[1]
    DH, FH = D // 2, F // 2
    NT = S // T
    NI = NT // 2
    assert B == 1 and D == 8 * LANES and NI * LANES == DH and FH % GR == 0 and 2 * GR == DH
    any_spec = pl.BlockSpec(memory_space=pl.ANY)
    out = pl.pallas_call(
        _kernel,
        in_specs=[any_spec] * 6,
        out_specs=any_spec,
        out_shape=jax.ShapeDtypeStruct((S, D), A_x.dtype),
        scratch_shapes=[
            pltpu.VMEM((S + T, D), BF16),
            pltpu.VMEM((NI, D // GR, GR, 2 * TN), BF16),
            pltpu.VMEM((2, D // GR, GR, D), BF16),
            pltpu.VMEM((D, D), BF16),
            pltpu.VMEM((T, D), F32),
            [pltpu.VMEM((n * 7 * DH // GR, GR // 2, DH), U32)
             for n in (1, 2, 1)],
            [(pltpu.VMEM((k // GR, GR, n), BF16),
              pltpu.VMEM((3, k // 2 // GR, GR, n // 2), BF16))
             for k, n in ((D, F), (D, F), (F, D))],
            pltpu.VMEM((7 * NT + 7, H // 2, DH), U32),
            pltpu.VMEM((7, H // 2, DH), U32),
            pltpu.VMEM((2, 7, H // 2, DH), U32),
            pltpu.VMEM((WINDOW, T, LANES), F32),
            pltpu.VMEM((7, H // 2, FH), U32),
            pltpu.VMEM((NT, 8, T, LANES), F32),
            pltpu.VMEM((NT, 8, T, LANES), F32),
            pltpu.VMEM((NT + 1, 8, HALO + T, LANES), F32),
            pltpu.VMEM((NT + 1, 8, HALO + T, LANES), F32),
            pltpu.VMEM((2, T, D), F32),
            pltpu.VMEM((S, D), BF16),
            pltpu.SemaphoreType.DMA((NT + 1,)),
            pltpu.SemaphoreType.DMA((NI,)),
            pltpu.SemaphoreType.DMA((NI,)),
            pltpu.SemaphoreType.DMA((NI - 1,)),
            pltpu.SemaphoreType.DMA(()),
            pltpu.SemaphoreType.DMA((NT,)),
            pltpu.SemaphoreType.DMA((NT,)),
        ],
        compiler_params=pltpu.CompilerParams(vmem_limit_bytes=124 * 2**20),
    )(A_x.reshape(S, D), A_wqkv.reshape(D // GR, GR, 3 * D), A_wo,
      B_w_gate.reshape(D // GR, GR, F), B_w_up.reshape(D // GR, GR, F),
      B_w_down.reshape(F // GR, GR, D))
    return out.reshape(B, S, D)
```

```python
import jax
import jax.numpy as jnp
from jax import lax
import jax.experimental.pallas as pl
import jax.experimental.pallas.tpu as pltpu

HEAD_DIM = 32
WINDOW = 8
DILATION = 2
HALO = 16
LANES = 128
T = 256
H = T // 2
SB = 8
RB = 16
TN = 128
PLAIN = (1, 4)
GR = 256
SCOPES = False
F32 = jnp.float32
BF16 = jnp.bfloat16
U32 = jnp.uint32


def _words(x):
    return pltpu.bitcast(x, U32)


def _halves(x):
    return pltpu.bitcast(x, BF16)


def _loop(name, n, body):
    def step(j, carry):
        if SCOPES:
            with jax.named_scope(name):
                body(j)
        else:
            body(j)
        return carry
    lax.fori_loop(0, n, step, 0)


def _emit(*stages):
    order = []
    for s, (lo, hi, steps) in enumerate(stages):
        order += [(lo + (hi - lo) * i / len(steps), s, i, f) for i, f in enumerate(steps)]
    for _, _, _, f in sorted(order, key=lambda t: t[:3]):
        f()


def _pipelined(pieces, depth):
    def step(t):
        for g in reversed(pieces[max(t - depth + 1, 0):t + 1]):
            next(g, None)
    return [lambda t=t: step(t) for t in range(len(pieces) + depth - 1)]


class _Pacer:
    def __init__(self, step=None):
        self.never = None if step is None else jnp.full((8, LANES), step, jnp.int32) < 0
        self.products = []
        self.due = []

    def _tie(self, x, others):
        regs = [[x[r:r + 8, c:c + LANES] for c in range(0, x.shape[1], LANES)]
                for r in range(0, x.shape[0], 8)]
        for k, other in enumerate(others):
            row, col = k % len(regs), k // len(regs) % len(regs[0])
            if other.dtype != x.dtype:
                other = pltpu.bitcast(other, x.dtype)
            regs[row][col] = jnp.where(self.never, other[:8, :LANES], regs[row][col])
        return jnp.concatenate([jnp.concatenate(row, axis=1) for row in regs], axis=0)

    def start(self, x, lag=3):
        if self.never is None or len(self.products) < lag:
            return x
        return self._tie(x, [self.products[-lag]] * (x.shape[0] // 8))

    def finish(self, x):
        if self.never is not None:
            self.due.append(x)

    def dot(self, lhs_words, rhs):
        if self.due:
            lhs_words = self._tie(lhs_words, self.due)
            self.due = []
        self.products.append(jnp.dot(_halves(lhs_words), rhs, preferred_element_type=F32))
        return self.products[-1]


def _gelu(x):
    c = 0.7978845608028654
    hx = 0.5 * x
    return hx + hx * jnp.tanh(x * (c + (c * 0.044715) * (x * x)))


def _lhs7(a11, a12, a21, a22):
    return [t.astype(BF16) for t in
            (a11 + a22, a21 + a22, a11, a22, a11 + a12, a21 - a11, a12 - a22)]


def _rhs7(b11, b12, b21, b22):
    f11, f12, f21, f22 = (b.astype(F32) for b in (b11, b12, b21, b22))
    return [t.astype(BF16) for t in
            (f11 + f22, b11, f12 - f22, f21 - f11, b22, f11 + f12, f21 + f22)]


def _strassen(pace, lhs, rhs, done):
    c = {}

    def m(i):
        return pace.dot(lhs(i), rhs(i))

    def s0():
        c["m1"] = m(0)

    def s1():
        c["m2"] = m(1)
        c[22] = c["m1"] - c["m2"]

    def s2():
        t = m(3)
        c[21] = c["m2"] + t
        c[11] = c["m1"] + t

    def s3():
        c["m5"] = m(4)
        c[11] = c[11] - c["m5"]

    def s4():
        t = m(2)
        c[12] = c["m5"] + t
        c[22] = c[22] + t

    def s5():
        c[11] = c[11] + m(6)

    def s6():
        done(c[11], c[12], c[21], c[22] + m(5))

    return [s0, s1, s2, s3, s4, s5, s6]


def _matmul(pace, lhs, rhs, width, done):
    steps = []
    for n in range(0, width, TN):
        steps += _strassen(pace, lhs, lambda i, n=n: rhs(i, n), lambda *c, n=n: done(n, *c))
    return steps


def _permute_cols(chunks):
    blk = lax.broadcasted_iota(jnp.int32, chunks[0].shape, 1) // 4
    a = [pltpu.roll(chunks[c], 4 * c, 1) if c else chunks[c] for c in range(8)]
    yield
    e = [a[(-i) % 8] for i in range(8)]
    for s in (1, 2, 4):
        e = [jnp.where((blk & s) != 0, e[(i - s) % 8], e[i]) for i in range(8)]
    e = [pltpu.roll(e[c], LANES - 4 * c, 1) if c else e[c] for c in range(8)]
    yield
    return e


def _permuted_rows(ref, c, hl, cols):
    parts = []
    for cp in range(8):
        r = c * 4
        u = _words(ref[pl.ds(pl.multiple_of(cp * LANES + hl * 32 + r // 16 * 16, 16), 16), cols])
        parts.append(u[r % 16 // 2:r % 16 // 2 + 2, :])
    return _halves(jnp.concatenate(parts, axis=0))


def _kernel(x_hbm, wqkv_hbm, wo_hbm, wg_hbm, wu_hbm, wd_hbm, out_hbm,
            x_v, wq_raw, wkv_raw, wo_raw, centred, w_ops, ffn_w, a_ops, hn, attn, prob, act,
            q_raw, q_v, k_v, v_v, h_v, out_v,
            sem_x, sem_p, sem_q, sem_kv, sem_o, sem_f, sem_out):
    S, D = x_hbm.shape
    DH = D // 2
    FH = wg_hbm.shape[2] // 2
    NT = S // T
    NI = NT // 2
    FR = GR // NT
    NG = 2 * GR // RB
    KG = -(-NG // (NI - 1))
    GROUP = H // NI
    PER = DH // GR
    WQ, WKV, WO = range(3)

    def ds(start, size):
        return pl.ds(start if isinstance(start, int) else pl.multiple_of(start, size), size)

    def last(j):
        return min(j, NT - 1) if isinstance(j, int) else jnp.minimum(j, NT - 1)

    def x_copy(j):
        return pltpu.make_async_copy(x_hbm.at[ds(last(j) * T, T)], x_v.at[ds(j * T, T)],
                                     sem_x.at[j])

    def x_part_copy(n):
        return [pltpu.make_async_copy(x_hbm.at[ds(2 * T + s * H + n * GROUP, GROUP)],
                                      x_v.at[ds(2 * T + s * H + n * GROUP, GROUP)],
                                      sem_p.at[n]) for s in range(2)]

    def wq_copy(n):
        return pltpu.make_async_copy(wqkv_hbm.at[:, :, ds(n * 2 * TN, 2 * TN)],
                                     wq_raw.at[n], sem_q.at[n])

    def wkv_copies(j):
        copies = []
        for m in range(2):
            lo = max(j * KG * RB - m * GR, 0)
            hi = min((j + 1) * KG * RB - m * GR, GR)
            if lo < hi:
                copies.append(pltpu.make_async_copy(
                    wqkv_hbm.at[:, pl.ds(lo, hi - lo), pl.ds((1 + m) * D, D)],
                    wkv_raw.at[m, :, pl.ds(lo, hi - lo)], sem_kv.at[j]))
        return copies

    wo_copy = pltpu.make_async_copy(wo_hbm, wo_raw, sem_o)

    def ffn_copies(j):
        rows = ds(j * FR, FR)
        return [pltpu.make_async_copy(src.at[:, rows], dst.at[:, rows], sem_f.at[j])
                for src, (dst, _) in zip((wg_hbm, wu_hbm, wd_hbm), ffn_w)]

    def out_copies(j, lo, hi):
        return [pltpu.make_async_copy(out_v.at[ds(j * T, T), pl.ds(s * DH + lo, hi - lo)],
                                      out_hbm.at[ds(j * T, T), pl.ds(s * DH + lo, hi - lo)],
                                      sem_out.at[j]) for s in range(2)]

    def store_weight(m, i, g, row, col, t):
        w_ops[m][i * PER + g, ds(row // 2, t.shape[0] // 2), col] = _words(t)

    def weight(m, first=0):
        return lambda i, n: _halves(
            w_ops[m][pl.ds(first + i * PER, PER), :, ds(n, TN)].reshape(DH // 2, TN))

    def norm_steps(pace, load_rows, store, rows=range(0, H, RB)):
        def piece(r):
            def load():
                return jnp.concatenate([load_rows(s * H + r).astype(F32) for s in range(2)], axis=0)
            m = jnp.mean(pace.start(load()), axis=-1, keepdims=True)
            yield
            c = load() - m
            centred[ds(2 * r, 2 * RB), :] = c
            scale = lax.rsqrt(jnp.mean(c * c, axis=-1, keepdims=True) + 1e-5)
            yield
            y = centred[ds(2 * r, 2 * RB), :] * scale
            for i, t in enumerate(_lhs7(y[:RB, :DH], y[:RB, DH:], y[RB:, :DH], y[RB:, DH:])):
                store(i, ds(r // 2, RB // 2), _words(t))
                pace.finish(_words(t)[:, i % 4 * LANES:(i % 4 + 1) * LANES])
        return _pipelined([piece(r) for r in rows], 3)

    def xn_steps(pace, j, copy, *rows):
        def store(i, where, t):
            a_ops[7 * j + i, where, :] = t
            copy[i, where, :] = t
        return norm_steps(pace, lambda r: x_v[ds(j * T + r, RB), :], store, *rows)

    def hn_steps(pace, slot, dest):
        def store(i, rows, t):
            hn[dest, i, rows, :] = t
        return norm_steps(pace, lambda r: h_v[slot, pl.ds(r, RB), :], store)

    def q_weight_steps(pace, n):
        def step(g, r):
            top, bot = (wq_raw[n, kh * PER + g, pl.ds(r, 2 * RB), :] for kh in range(2))
            b11 = pace.start(top[:, :TN].astype(F32))
            for i, t in enumerate(_rhs7(b11, top[:, TN:], bot[:, :TN], bot[:, TN:])):
                store_weight(WQ, i, g, r, ds(n * TN, TN), t)
        return [lambda g=g, r=r: step(g, r) for g in range(PER) for r in range(0, GR, 2 * RB)]

    def kv_weight_steps(pace, j):
        def piece(g, group):
            m, row = group // (NG // 2), group % (NG // 2) * RB
            u = [jnp.concatenate(
                [_words(wkv_raw[m, kh * PER + g, ds(row, RB), pl.ds(c * LANES, LANES)])
                 for kh in range(2)], axis=0) for c in range(8)]
            u = yield from _permute_cols(u[:1] + [pace.start(u[1])] + u[2:])
            for c in range(4):
                b = [_halves(u[nh * 4 + c][kh * RB // 2:(kh + 1) * RB // 2])
                     for kh in range(2) for nh in range(2)]
                for i, t in enumerate(_rhs7(*b)):
                    store_weight(WKV, i, m * 7 * PER + g, row, pl.ds(c * LANES, LANES), t)
                    if i >= 5:
                        pace.finish(_words(t))
        return _pipelined([piece(g, jnp.minimum(j * KG + r, NG - 1)) for r in range(KG)
                           for g in range(PER)], 3)

    def ffn_index(w, i, g, rows, n, width):
        blocks, extra = w
        _, per, _, half = extra.shape
        if 1 <= i <= 4:
            g = pl.ds((i - 1) // 2 * per, per) if g is None else (i - 1) // 2 * per + g
            return blocks, (g, rows, pl.ds((i - 1) % 2 * half + n, width))
        return extra, (i % 4, slice(None) if g is None else g, rows, pl.ds(n, width))

    def ffn_weight_steps(pace, j):
        def step(w, g, n):
            where = [ffn_index(w, i, g, ds(j * FR, FR), n, 2 * LANES) for i in range(7)]
            blocks = [ref[idx] for ref, idx in where[1:5]]
            blocks[0] = pace.start(blocks[0].astype(F32), 3)
            pace.finish(blocks[0])
            for i, t in enumerate(_rhs7(*blocks)):
                if i not in PLAIN:
                    ref, idx = where[i]
                    ref[idx] = t
        steps = [[lambda w=w, g=g, n=n: step(w, g, n) for g in range(w[1].shape[1])
                  for n in range(0, w[1].shape[3], 2 * LANES)] for w in ffn_w]
        return [f for group in zip(*steps) for f in group]

    def ffn_weight(w):
        def load(i, n):
            ref, idx = ffn_index(w, i, None, slice(None), n, TN)
            return ref[idx].reshape(w[1].shape[1] * GR, TN)
        return load

    def permute_q_steps(pace, j, rows):
        def piece(r):
            q = [q_raw[j, c, ds(r, GROUP), :] for c in range(8)]
            q = yield from _permute_cols(q[:1] + [pace.start(q[1])] + q[2:])
            for c in range(8):
                q_v[j % 2, c, ds(r, GROUP), :] = q[c]
                pace.finish(q[c][c * 8 % GROUP:])
        return _pipelined([piece(r) for r in rows], 3)

    def q_step(pace, j, lhs, n):
        def done(*c):
            for b, t in enumerate(c):
                q_raw[j, 2 * n + b % 2, pl.ds(b // 2 * H, H), :] = t
        return _strassen(pace, lambda i: lhs[i], lambda i: weight(WQ)(i, n * TN), done)

    def project(pace, j, rhs, dst):
        def done(n, *c):
            for b, t in enumerate(c):
                chunk = (b % 2 * DH + n) // LANES
                dst[j, chunk, pl.ds(HALO + b // 2 * H, H), :] = t
                if b // 2:
                    dst[j + 1, chunk, pl.ds(0, HALO), :] = t[H - HALO:]
        return _matmul(pace, lambda i: a_ops[7 * j + i], rhs, DH, done)

    def softmax_steps(pace, q, k, out, rows, first=None):
        def piece(r):
            logits = [None] * WINDOW
            for c in range(8):
                qc = q[c, pl.ds(r, SB), :]
                if c == 0:
                    qc = pace.start(qc)
                for w in range(WINDOW):
                    t = qc * k[c, pl.ds(HALO + r - DILATION * w, SB), :]
                    logits[w] = t if c == 0 else logits[w] + t
            lane = lax.broadcasted_iota(jnp.int32, (SB, LANES), 1)
            for s in (1, 2):
                rolled = [(pltpu.roll(l, s, 1), pltpu.roll(l, LANES - s, 1)) for l in logits]
                yield
                logits = [l + jnp.where((lane & s) != 0, a, b)
                          for l, (a, b) in zip(logits, rolled)]
            for w in range(WINDOW):
                l = logits[w] * (HEAD_DIM ** -0.5)
                if first is not None and r < DILATION * w:
                    pos = first + r + lax.broadcasted_iota(jnp.int32, (SB, LANES), 0)
                    l = jnp.where(pos >= DILATION * w, l, -1e9)
                logits[w] = l
            m = logits[0]
            for w in range(1, WINDOW):
                m = jnp.maximum(m, logits[w])
            e = [jnp.exp(l - m) for l in logits]
            total = e[0]
            for w in range(1, WINDOW):
                total = total + e[w]
            inv = 1.0 / total
            for w in range(WINDOW):
                p = e[w] * inv
                out[w, pl.ds(r, SB), :] = p
                pace.finish(p)
        return _pipelined([piece(r) for r in rows], 3)

    def value_steps(pace, weights, v, out, rows):
        def piece(r, c):
            blocks = []
            for row in (r, H + r):
                for chunk in (c, c + 4):
                    for w in range(WINDOW):
                        p = weights[w, pl.ds(row, RB), :]
                        t = (pace.start(p, 4) if w == 0 else p) * v[
                            chunk, pl.ds(HALO + row - DILATION * w, RB), :]
                        o = t if w == 0 else o + t
                    blocks.append(o)
                    pace.finish(o)
                    pace.finish(o[8:])
                    yield
            for i, t in enumerate(_lhs7(*blocks)):
                out[i, pl.ds(r // 2, RB // 2), pl.ds(c * LANES, LANES)] = _words(t)
                pace.finish(_words(t))
        pieces = [piece(r, c) for r in rows for c in range(4)]
        return [lambda g=g: next(g, None) for g in pieces for _ in range(5)]

    def output_steps(pace, j, slot):
        def done(n, *c):
            for b, t in enumerate(c):
                cols = pl.ds(b % 2 * DH + n, TN)
                h_v[slot, pl.ds(b // 2 * H, H), cols] = (
                    x_v[ds(j * T + b // 2 * H, H), cols].astype(F32) + t)
        return _matmul(pace, lambda i: attn[slot, i], weight(WO), DH, done)

    first = [x_copy(0), x_copy(1), wq_copy(0)]
    for c in first:
        c.start()
    for n in range(NI):
        for c in ([wq_copy(n + 1)] if n + 1 < NI else []) + x_part_copy(n):
            c.start()
    prob[:, pl.ds(0, H + GROUP), :] = jnp.zeros((WINDOW, H + GROUP, LANES), F32)
    v_v[0, :, pl.ds(0, HALO + H + GROUP), :] = jnp.zeros((8, HALO + H + GROUP, LANES), F32)
    k_v[0, :, pl.ds(0, HALO), :] = jnp.zeros((8, HALO, LANES), F32)
    h_v[0] = jnp.zeros((T, D), F32)
    for c, steps in zip(first, (xn_steps(_Pacer(), 0, hn.at[0]), xn_steps(_Pacer(), 1, attn.at[0]),
                                q_weight_steps(_Pacer(), 0))):
        c.wait()
        _emit((0, 1, steps))
    for j in range(NI - 1):
        for c in [x_copy(2 * j + 3), x_copy(2 * j + 4)] + wkv_copies(j):
            c.start()

    def first_q(n):
        pl.when(n + 1 < NI)(lambda: wq_copy(n + 1).wait())
        for c in x_part_copy(n):
            c.wait()
        pace = _Pacer(n)
        _emit(
            (0, 1, [f for fs in zip(q_step(pace, 0, hn.at[0], n), q_step(pace, 1, attn.at[0], n))
                    for f in fs]),
            (0.52, 0.97, q_weight_steps(pace, jnp.minimum(n + 1, NI - 1))),
            (-0.1, 0.7, xn_steps(pace, 2, attn.at[1],
                              [n * GROUP + r for r in range(0, GROUP, RB)])),
        )
    _loop("first_q", NI, first_q)
    for c in [wo_copy] + ffn_copies(0) + ffn_copies(1):
        c.start()

    def phase_q(j):
        t = 2 * j + 2
        x_copy(t + 1).wait()
        x_copy(t + 2).wait()
        for k in range(NI - 1):
            @pl.when(j == k)
            def _():
                for c in wkv_copies(k):
                    c.wait()
        pace = _Pacer(j)
        _emit(
            (0, 1, [f for n in range(NI) for f in q_step(pace, t, attn.at[1], n)]),
            (1, 2, [f for n in range(NI) for f in q_step(pace, t + 1, hn.at[0], n)]),
            (-0.05, 0.97, xn_steps(pace, t + 1, hn.at[0])),
            (0.85, 1.93, xn_steps(pace, t + 2, attn.at[1])),
            (0, 1.97, kv_weight_steps(pace, j)),
        )
    _loop("phase_q", NI - 1, phase_q)
    for t in range(2, NT):
        for c in ffn_copies(t):
            c.start()
    wo_copy.wait()

    def first_values(pace, g):
        for c in range(8):
            v_v[0, c, pl.ds(0, HALO), :] = jnp.broadcast_to(
                v_v[0, c, pl.ds(HALO, 1), :], (HALO, LANES))
        tile, row = g // NI, pl.multiple_of(g % NI * GROUP, GROUP)
        return value_steps(pace, prob.at[:, pl.ds(row, H + GROUP)],
                           v_v.at[tile, :, pl.ds(row, HALO + H + GROUP)],
                           attn.at[tile, :, ds(row // 2, GROUP // 2)], range(0, GROUP, RB))

    def phase_kv(j):
        for c in ffn_copies(j):
            c.wait()

        def wo_step(c, hl):
            col = j % NI * LANES
            b = [_permuted_rows(wo_raw, kh * 4 + c, hl, ds(s * DH + col, LANES))
                 for kh in range(2) for s in range(2)]
            b[0] = pace.start(b[0].astype(F32))
            for i, t in enumerate(_rhs7(*b)):
                store_weight(WO, i, c * LANES // GR, c * LANES % GR + hl * 32, ds(col, LANES), t)
                pace.finish(_words(t)[i % 2 * 8:])

        pace = _Pacer(j)
        tile, row = j // NI, pl.multiple_of(j % NI * GROUP, GROUP)
        _emit(
            (0, 1, project(pace, j, weight(WKV), k_v)),
            (1, 2, project(pace, j, weight(WKV, 7 * PER), v_v)),
            (0, 1.85, ffn_weight_steps(pace, j)),
            (0.3, 1, permute_q_steps(pace, tile, [row, H + row])),
            (0.2, 1.95, [lambda c=c, hl=hl: wo_step(c, j // NI * 2 + hl)
                         for c in range(4) for hl in range(2)]),
            (0.25, 1, first_values(pace, jnp.maximum(j - 1, 0))),
            (1.1, 1.95, softmax_steps(
                pace, q_v.at[tile, :, pl.ds(row, H + GROUP)],
                k_v.at[tile, :, pl.ds(row, HALO + H + GROUP)], prob.at[:, pl.ds(row, H + GROUP)],
                [s * H + r for s in range(2) for r in range(0, GROUP, SB)], tile * T + row)),
        )
    _loop("phase_kv", NT, phase_kv)
    _emit((0, 1, first_values(_Pacer(), jnp.int32(NT - 1))))

    def ffn(j):
        nxt = last(j + 2)
        slot = j % 2
        pace = _Pacer(j)
        gate = {}

        def gate_done(n, *c):
            gate[n] = [_gelu(t) for t in c]

        def up_done(n, *c):
            for i, t in enumerate(_lhs7(*[g * u for g, u in zip(gate.pop(n), c)])):
                act[i, :, n:n + TN] = _words(t)

        def down_done(n, *c):
            for b, t in enumerate(c):
                cols = pl.ds(b % 2 * DH + n, TN)
                out_v[ds(j * T + b // 2 * H, H), cols] = (
                    h_v[slot, pl.ds(b // 2 * H, H), cols] + t).astype(BF16)

        g = _matmul(pace, lambda i: hn[0, i], ffn_weight(ffn_w[0]), FH, gate_done)
        u = _matmul(pace, lambda i: hn[0, i], ffn_weight(ffn_w[1]), FH, up_done)
        gu = [f for n in range(0, len(g), 7) for f in g[n:n + 7] + u[n:n + 7]]
        _emit(
            (0, 1, gu),
            (1, 1.5, _matmul(pace, lambda i: act[i], ffn_weight(ffn_w[2]), DH, down_done)),
            (0.01, 0.58, softmax_steps(pace, q_v.at[nxt % 2], k_v.at[nxt], prob, range(0, T, SB))),
            (0.58, 0.99, value_steps(pace, prob, v_v.at[nxt], attn.at[slot], range(0, H, RB))),
            (1.02, 1.37, hn_steps(pace, 1 - slot, 0)),
            (1.39, 1.39, [c.start for c in out_copies(j, 0, DH - TN)]),
        )
        for c in out_copies(j, DH - TN, DH):
            c.start()

    def phase_ffn(t):
        @pl.when(t < NT)
        def _():
            pace = _Pacer(t)
            _emit((0, 1, output_steps(pace, t, t % 2)),
                  (-0.05, 0.92, hn_steps(pace, 0, jnp.where(t == 1, 0, 1))),
                  (0.0, 0.97, permute_q_steps(pace, last(t + 1), range(0, T, GROUP))))

        pl.when(t > 0)(lambda: ffn(t - 1))
    _loop("phase_ffn", NT + 1, phase_ffn)
    for j in range(NT):
        for c in out_copies(j, 0, DH - TN) + out_copies(j, DH - TN, DH):
            c.wait()


@jax.jit
def pallas_sequential_preLN__sliding_local_dilated__glu_gated_geglu__prompt_kernel(
    A_x: jax.Array,
    A_wqkv: jax.Array,
    A_wo: jax.Array,
    B_x: jax.Array,
    B_w_gate: jax.Array,
    B_w_up: jax.Array,
    B_w_down: jax.Array,
):
    del B_x
    B, S, D = A_x.shape
    F = B_w_gate.shape[1]
    DH, FH = D // 2, F // 2
    NT = S // T
    NI = NT // 2
    assert B == 1 and D == 8 * LANES and NI * LANES == DH and FH % GR == 0 and 2 * GR == DH
    any_spec = pl.BlockSpec(memory_space=pl.ANY)
    out = pl.pallas_call(
        _kernel,
        in_specs=[any_spec] * 6,
        out_specs=any_spec,
        out_shape=jax.ShapeDtypeStruct((S, D), A_x.dtype),
        scratch_shapes=[
            pltpu.VMEM((S + T, D), BF16),
            pltpu.VMEM((NI, D // GR, GR, 2 * TN), BF16),
            pltpu.VMEM((2, D // GR, GR, D), BF16),
            pltpu.VMEM((D, D), BF16),
            pltpu.VMEM((T, D), F32),
            [pltpu.VMEM((n * 7 * DH // GR, GR // 2, DH), U32)
             for n in (1, 2, 1)],
            [(pltpu.VMEM((k // GR, GR, n), BF16),
              pltpu.VMEM((3, k // 2 // GR, GR, n // 2), BF16))
             for k, n in ((D, F), (D, F), (F, D))],
            pltpu.VMEM((7 * NT + 7, H // 2, DH), U32),
            pltpu.VMEM((2, 7, H // 2, DH), U32),
            pltpu.VMEM((2, 7, H // 2, DH), U32),
            pltpu.VMEM((WINDOW, T, LANES), F32),
            pltpu.VMEM((7, H // 2, FH), U32),
            pltpu.VMEM((NT, 8, T, LANES), F32),
            pltpu.VMEM((2, 8, T, LANES), F32),
            pltpu.VMEM((NT + 1, 8, HALO + T, LANES), F32),
            pltpu.VMEM((NT + 1, 8, HALO + T, LANES), F32),
            pltpu.VMEM((2, T, D), F32),
            pltpu.VMEM((S, D), BF16),
            pltpu.SemaphoreType.DMA((NT + 1,)),
            pltpu.SemaphoreType.DMA((NI,)),
            pltpu.SemaphoreType.DMA((NI,)),
            pltpu.SemaphoreType.DMA((NI - 1,)),
            pltpu.SemaphoreType.DMA(()),
            pltpu.SemaphoreType.DMA((NT,)),
            pltpu.SemaphoreType.DMA((NT,)),
        ],
        compiler_params=pltpu.CompilerParams(vmem_limit_bytes=124 * 2**20),
    )(A_x.reshape(S, D), A_wqkv.reshape(D // GR, GR, 3 * D), A_wo,
      B_w_gate.reshape(D // GR, GR, F), B_w_up.reshape(D // GR, GR, F),
      B_w_down.reshape(F // GR, GR, D))
    return out.reshape(B, S, D)
```

```python
import jax
import jax.numpy as jnp
from jax import lax
import jax.experimental.pallas as pl
import jax.experimental.pallas.tpu as pltpu

HEAD_DIM = 32
WINDOW = 8
DILATION = 2
HALO = 16
LANES = 128
T = 256
H = T // 2
SB = 8
RB = 16
TN = 128
PLAIN = (1, 4)
GR = 256
SCOPES = False
F32 = jnp.float32
BF16 = jnp.bfloat16
U32 = jnp.uint32


def _words(x):
    return pltpu.bitcast(x, U32)


def _halves(x):
    return pltpu.bitcast(x, BF16)


def _loop(name, n, body):
    def step(j, carry):
        if SCOPES:
            with jax.named_scope(name):
                body(j)
        else:
            body(j)
        return carry
    lax.fori_loop(0, n, step, 0)


def _emit(*stages):
    order = []
    for s, (lo, hi, steps) in enumerate(stages):
        order += [(lo + (hi - lo) * i / len(steps), s, i, f) for i, f in enumerate(steps)]
    for _, _, _, f in sorted(order, key=lambda t: t[:3]):
        f()


def _pipelined(pieces, depth):
    def step(t):
        for g in reversed(pieces[max(t - depth + 1, 0):t + 1]):
            next(g, None)
    return [lambda t=t: step(t) for t in range(len(pieces) + depth - 1)]


class _Pacer:
    def __init__(self, step=None):
        self.never = None if step is None else jnp.full((8, LANES), step, jnp.int32) < 0
        self.products = []
        self.due = []

    def _tie(self, x, others):
        regs = [[x[r:r + 8, c:c + LANES] for c in range(0, x.shape[1], LANES)]
                for r in range(0, x.shape[0], 8)]
        for k, other in enumerate(others):
            row, col = k % len(regs), k // len(regs) % len(regs[0])
            if other.dtype != x.dtype:
                other = pltpu.bitcast(other, x.dtype)
            regs[row][col] = jnp.where(self.never, other[:8, :LANES], regs[row][col])
        return jnp.concatenate([jnp.concatenate(row, axis=1) for row in regs], axis=0)

    def start(self, x, lag=3):
        if self.never is None or len(self.products) < lag:
            return x
        return self._tie(x, [self.products[-lag]] * (x.shape[0] // 8))

    def finish(self, x):
        if self.never is not None:
            self.due.append(x)

    def dot(self, lhs_words, rhs):
        if self.due:
            lhs_words = self._tie(lhs_words, self.due)
            self.due = []
        self.products.append(jnp.dot(_halves(lhs_words), rhs, preferred_element_type=F32))
        return self.products[-1]


def _gelu(x):
    c = 0.7978845608028654
    hx = 0.5 * x
    return hx + hx * jnp.tanh(x * (c + (c * 0.044715) * (x * x)))


def _lhs7(a11, a12, a21, a22):
    return [t.astype(BF16) for t in
            (a11 + a22, a21 + a22, a11, a22, a11 + a12, a21 - a11, a12 - a22)]


def _rhs7(b11, b12, b21, b22):
    f11, f12, f21, f22 = (b.astype(F32) for b in (b11, b12, b21, b22))
    return [t.astype(BF16) for t in
            (f11 + f22, b11, f12 - f22, f21 - f11, b22, f11 + f12, f21 + f22)]


def _strassen(pace, lhs, rhs, done):
    c = {}

    def m(i):
        return pace.dot(lhs(i), rhs(i))

    def s0():
        c["m1"] = m(0)

    def s1():
        c["m2"] = m(1)
        c[22] = c["m1"] - c["m2"]

    def s2():
        t = m(3)
        c[21] = c["m2"] + t
        c[11] = c["m1"] + t

    def s3():
        c["m5"] = m(4)
        c[11] = c[11] - c["m5"]

    def s4():
        t = m(2)
        c[12] = c["m5"] + t
        c[22] = c[22] + t

    def s5():
        c[11] = c[11] + m(6)

    def s6():
        done(c[11], c[12], c[21], c[22] + m(5))

    return [s0, s1, s2, s3, s4, s5, s6]


def _matmul(pace, lhs, rhs, width, done):
    steps = []
    for n in range(0, width, TN):
        steps += _strassen(pace, lhs, lambda i, n=n: rhs(i, n), lambda *c, n=n: done(n, *c))
    return steps


def _permute_cols(chunks):
    blk = lax.broadcasted_iota(jnp.int32, chunks[0].shape, 1) // 4
    a = [pltpu.roll(chunks[c], 4 * c, 1) if c else chunks[c] for c in range(8)]
    yield
    e = [a[(-i) % 8] for i in range(8)]
    for s in (1, 2, 4):
        e = [jnp.where((blk & s) != 0, e[(i - s) % 8], e[i]) for i in range(8)]
    e = [pltpu.roll(e[c], LANES - 4 * c, 1) if c else e[c] for c in range(8)]
    yield
    return e


def _permuted_rows(ref, c, hl):
    parts = []
    for cp in range(8):
        r = c * 4
        u = _words(ref[pl.ds(cp * LANES + hl * 32 + r // 16 * 16, 16), :])
        parts.append(u[r % 16 // 2:r % 16 // 2 + 2, :])
    return _halves(jnp.concatenate(parts, axis=0))


def _kernel(x_hbm, wqkv_hbm, wo_hbm, wg_hbm, wu_hbm, wd_hbm, out_hbm,
            x_v, wq_raw, wkv_raw, wo_raw, centred, w_ops, ffn_w, a_ops, hn, attn, prob, act,
            q_raw, q_v, k_v, v_v, h_v, out_v,
            sem_x, sem_p, sem_q, sem_kv, sem_o, sem_f, sem_out):
    S, D = x_hbm.shape
    DH = D // 2
    FH = wg_hbm.shape[2] // 2
    NT = S // T
    NI = NT // 2
    FR = GR // NT
    NG = 2 * GR // RB
    KG = -(-NG // (NI - 1))
    GROUP = H // NI
    PER = DH // GR
    WQ, WKV, WO = range(3)

    def ds(start, size):
        return pl.ds(start if isinstance(start, int) else pl.multiple_of(start, size), size)

    def last(j):
        return min(j, NT - 1) if isinstance(j, int) else jnp.minimum(j, NT - 1)

    def x_copy(j):
        return pltpu.make_async_copy(x_hbm.at[ds(last(j) * T, T)], x_v.at[ds(j * T, T)],
                                     sem_x.at[j])

    def x_part_copy(n):
        return [pltpu.make_async_copy(x_hbm.at[ds(2 * T + s * H + n * GROUP, GROUP)],
                                      x_v.at[ds(2 * T + s * H + n * GROUP, GROUP)],
                                      sem_p.at[n]) for s in range(2)]

    def wq_copy(n):
        return pltpu.make_async_copy(wqkv_hbm.at[:, :, ds(n * 2 * TN, 2 * TN)],
                                     wq_raw.at[n], sem_q.at[n])

    def wkv_copies(j):
        copies = []
        for m in range(2):
            lo = max(j * KG * RB - m * GR, 0)
            hi = min((j + 1) * KG * RB - m * GR, GR)
            if lo < hi:
                copies.append(pltpu.make_async_copy(
                    wqkv_hbm.at[:, pl.ds(lo, hi - lo), pl.ds((1 + m) * D, D)],
                    wkv_raw.at[m, :, pl.ds(lo, hi - lo)], sem_kv.at[j]))
        return copies

    wo_copy = pltpu.make_async_copy(wo_hbm, wo_raw, sem_o)

    def ffn_copies(j):
        rows = ds(j * FR, FR)
        return [pltpu.make_async_copy(src.at[:, rows], dst.at[:, rows], sem_f.at[j])
                for src, (dst, _) in zip((wg_hbm, wu_hbm, wd_hbm), ffn_w)]

    def out_copies(j, lo, hi):
        return [pltpu.make_async_copy(out_v.at[ds(j * T, T), pl.ds(s * DH + lo, hi - lo)],
                                      out_hbm.at[ds(j * T, T), pl.ds(s * DH + lo, hi - lo)],
                                      sem_out.at[j]) for s in range(2)]

    def store_weight(m, i, g, row, col, t):
        w_ops[m][i * PER + g, ds(row // 2, t.shape[0] // 2), col] = _words(t)

    def weight(m, first=0):
        return lambda i, n: _halves(
            w_ops[m][pl.ds(first + i * PER, PER), :, ds(n, TN)].reshape(DH // 2, TN))

    def norm_steps(pace, load_rows, store, rows=range(0, H, RB)):
        def piece(r):
            def load():
                return jnp.concatenate([load_rows(s * H + r).astype(F32) for s in range(2)], axis=0)
            m = jnp.mean(pace.start(load()), axis=-1, keepdims=True)
            yield
            c = load() - m
            centred[ds(2 * r, 2 * RB), :] = c
            scale = lax.rsqrt(jnp.mean(c * c, axis=-1, keepdims=True) + 1e-5)
            yield
            y = centred[ds(2 * r, 2 * RB), :] * scale
            for i, t in enumerate(_lhs7(y[:RB, :DH], y[:RB, DH:], y[RB:, :DH], y[RB:, DH:])):
                store(i, ds(r // 2, RB // 2), _words(t))
                pace.finish(_words(t)[:, i % 4 * LANES:(i % 4 + 1) * LANES])
        return _pipelined([piece(r) for r in rows], 3)

    def xn_steps(pace, j, copy, *rows):
        def store(i, where, t):
            a_ops[7 * j + i, where, :] = t
            copy[i, where, :] = t
        return norm_steps(pace, lambda r: x_v[ds(j * T + r, RB), :], store, *rows)

    def hn_steps(pace, slot, dest):
        def store(i, rows, t):
            hn[dest, i, rows, :] = t
        return norm_steps(pace, lambda r: h_v[slot, pl.ds(r, RB), :], store)

    def q_weight_steps(pace, n):
        def step(g, r):
            top, bot = (wq_raw[n, kh * PER + g, pl.ds(r, 2 * RB), :] for kh in range(2))
            b11 = pace.start(top[:, :TN].astype(F32))
            for i, t in enumerate(_rhs7(b11, top[:, TN:], bot[:, :TN], bot[:, TN:])):
                store_weight(WQ, i, g, r, ds(n * TN, TN), t)
        return [lambda g=g, r=r: step(g, r) for g in range(PER) for r in range(0, GR, 2 * RB)]

    def kv_weight_steps(pace, j):
        def piece(g, group):
            m, row = group // (NG // 2), group % (NG // 2) * RB
            u = [jnp.concatenate(
                [_words(wkv_raw[m, kh * PER + g, ds(row, RB), pl.ds(c * LANES, LANES)])
                 for kh in range(2)], axis=0) for c in range(8)]
            u = yield from _permute_cols(u[:1] + [pace.start(u[1])] + u[2:])
            for c in range(4):
                b = [_halves(u[nh * 4 + c][kh * RB // 2:(kh + 1) * RB // 2])
                     for kh in range(2) for nh in range(2)]
                for i, t in enumerate(_rhs7(*b)):
                    store_weight(WKV, i, m * 7 * PER + g, row, pl.ds(c * LANES, LANES), t)
                    if i >= 5:
                        pace.finish(_words(t))
        return _pipelined([piece(g, jnp.minimum(j * KG + r, NG - 1)) for r in range(KG)
                           for g in range(PER)], 3)

    def ffn_index(w, i, g, rows, n, width):
        blocks, extra = w
        _, per, _, half = extra.shape
        if 1 <= i <= 4:
            g = pl.ds((i - 1) // 2 * per, per) if g is None else (i - 1) // 2 * per + g
            return blocks, (g, rows, pl.ds((i - 1) % 2 * half + n, width))
        return extra, (i % 4, slice(None) if g is None else g, rows, pl.ds(n, width))

    def ffn_weight_steps(pace, j):
        def step(w, g, n):
            where = [ffn_index(w, i, g, slice(None), n, 2 * LANES) for i in range(7)]
            blocks = [ref[idx] for ref, idx in where[1:5]]
            blocks[0] = pace.start(blocks[0].astype(F32), 3)
            pace.finish(blocks[0])
            for i, t in enumerate(_rhs7(*blocks)):
                if i not in PLAIN:
                    ref, idx = where[i]
                    ref[idx] = t
        chunk = [(blocks.at[:, ds(j * FR, FR)], extra.at[:, :, ds(j * FR, FR)])
                 for blocks, extra in ffn_w]
        steps = [[lambda w=w, g=g, n=n: step(w, g, n) for g in range(w[1].shape[1])
                  for n in range(0, w[1].shape[3], 2 * LANES)] for w in chunk]
        return [f for group in zip(*steps) for f in group]

    def ffn_weight(w):
        def load(i, n):
            ref, idx = ffn_index(w, i, None, slice(None), n, TN)
            return ref[idx].reshape(w[1].shape[1] * GR, TN)
        return load

    def permute_q_steps(pace, j, rows):
        def piece(r):
            q = [q_raw[j, c, ds(r, GROUP), :] for c in range(8)]
            q = yield from _permute_cols(q[:1] + [pace.start(q[1])] + q[2:])
            for c in range(8):
                q_v[j % 2, c, ds(r, GROUP), :] = q[c]
                pace.finish(q[c][c * 8 % GROUP:])
        return _pipelined([piece(r) for r in rows], 3)

    def q_step(pace, j, lhs, n):
        def done(*c):
            for b, t in enumerate(c):
                q_raw[j, 2 * n + b % 2, pl.ds(b // 2 * H, H), :] = t
        return _strassen(pace, lambda i: lhs[i], lambda i: weight(WQ)(i, n * TN), done)

    def project(pace, j, rhs, dst):
        lhs, dst = a_ops.at[pl.ds(7 * j, 7)], dst.at[pl.ds(j, 2)]

        def done(n, *c):
            for b, t in enumerate(c):
                chunk = (b % 2 * DH + n) // LANES
                dst[0, chunk, pl.ds(HALO + b // 2 * H, H), :] = t
                if b // 2:
                    dst[1, chunk, pl.ds(0, HALO), :] = t[H - HALO:]
        return _matmul(pace, lambda i: lhs[i], rhs, DH, done)

    def softmax_steps(pace, q, k, out, rows, first=None):
        def piece(r):
            logits = [None] * WINDOW
            for c in range(8):
                qc = q[c, pl.ds(r, SB), :]
                if c == 0:
                    qc = pace.start(qc)
                for w in range(WINDOW):
                    t = qc * k[c, pl.ds(HALO + r - DILATION * w, SB), :]
                    logits[w] = t if c == 0 else logits[w] + t
            lane = lax.broadcasted_iota(jnp.int32, (SB, LANES), 1)
            for s in (1, 2):
                rolled = [(pltpu.roll(l, s, 1), pltpu.roll(l, LANES - s, 1)) for l in logits]
                yield
                logits = [l + jnp.where((lane & s) != 0, a, b)
                          for l, (a, b) in zip(logits, rolled)]
            for w in range(WINDOW):
                l = logits[w] * (HEAD_DIM ** -0.5)
                if first is not None and r < DILATION * w:
                    pos = first + r + lax.broadcasted_iota(jnp.int32, (SB, LANES), 0)
                    l = jnp.where(pos >= DILATION * w, l, -1e9)
                logits[w] = l
            m = logits[0]
            for w in range(1, WINDOW):
                m = jnp.maximum(m, logits[w])
            e = [jnp.exp(l - m) for l in logits]
            total = e[0]
            for w in range(1, WINDOW):
                total = total + e[w]
            inv = 1.0 / total
            for w in range(WINDOW):
                p = e[w] * inv
                out[w, pl.ds(r, SB), :] = p
                pace.finish(p)
        return _pipelined([piece(r) for r in rows], 3)

    def value_steps(pace, weights, v, out, rows):
        def piece(r, c):
            blocks = []
            for row in (r, H + r):
                for chunk in (c, c + 4):
                    for w in range(WINDOW):
                        p = weights[w, pl.ds(row, RB), :]
                        t = (pace.start(p, 6) if w == 0 else p) * v[
                            chunk, pl.ds(HALO + row - DILATION * w, RB), :]
                        o = t if w == 0 else o + t
                    blocks.append(o)
                    pace.finish(o)
                    pace.finish(o[8:])
                    yield
            for i, t in enumerate(_lhs7(*blocks)):
                out[i, pl.ds(r // 2, RB // 2), pl.ds(c * LANES, LANES)] = _words(t)
                pace.finish(_words(t))
        pieces = [piece(r, c) for r in rows for c in range(4)]
        return [lambda g=g: next(g, None) for g in pieces for _ in range(5)]

    def output_steps(pace, j, slot):
        def done(n, *c):
            for b, t in enumerate(c):
                cols = pl.ds(b % 2 * DH + n, TN)
                h_v[slot, pl.ds(b // 2 * H, H), cols] = (
                    x_v[ds(j * T + b // 2 * H, H), cols].astype(F32) + t)
        return _matmul(pace, lambda i: attn[slot, i], weight(WO), DH, done)

    first = [x_copy(0), x_copy(1), wq_copy(0)]
    for c in first:
        c.start()
    later = [x_part_copy(n) + ([wq_copy(n + 1)] if n + 1 < NI else []) for n in range(NI)]
    for c in later[0]:
        c.start()
    prob[:, pl.ds(0, H + GROUP), :] = jnp.zeros((WINDOW, H + GROUP, LANES), F32)
    v_v[0, :, pl.ds(0, HALO + H + GROUP), :] = jnp.zeros((8, HALO + H + GROUP, LANES), F32)
    k_v[0, :, pl.ds(0, HALO), :] = jnp.zeros((8, HALO, LANES), F32)
    h_v[0] = jnp.zeros((T, D), F32)
    for c, steps in zip(first, (xn_steps(_Pacer(), 0, hn.at[0]), xn_steps(_Pacer(), 1, attn.at[0]),
                                q_weight_steps(_Pacer(), 0))):
        c.wait()
        _emit((0, 1, steps))
    for c in later[1]:
        c.start()
    batches = [sum(later[2:], [])] + [[x_copy(2 * j + 3), x_copy(2 * j + 4)] + wkv_copies(j)
                                      for j in range(NI - 1)]

    def first_q(n):
        pl.when(n + 1 < NI)(lambda: wq_copy(n + 1).wait())
        for c in x_part_copy(n):
            c.wait()
        for k, batch in enumerate(batches):
            @pl.when(n == k)
            def _():
                for c in batch:
                    c.start()
        pace = _Pacer(n)
        _emit(
            (0, 1, [f for fs in zip(q_step(pace, 0, hn.at[0], n), q_step(pace, 1, attn.at[0], n))
                    for f in fs]),
            (0.4, 0.99, q_weight_steps(pace, jnp.minimum(n + 1, NI - 1))),
            (-0.2, 0.6, xn_steps(pace, 2, attn.at[1],
                              [n * GROUP + r for r in range(0, GROUP, RB)])),
        )
    _loop("first_q", NI, first_q)
    for c in [wo_copy] + ffn_copies(0) + ffn_copies(1):
        c.start()

    def phase_q(j):
        t = 2 * j + 2
        x_copy(t + 1).wait()
        x_copy(t + 2).wait()
        for k in range(NI - 1):
            @pl.when(j == k)
            def _():
                for c in wkv_copies(k):
                    c.wait()
        pace = _Pacer(j)
        _emit(
            (0, 1, [f for n in range(NI) for f in q_step(pace, t, attn.at[1], n)]),
            (1, 2, [f for n in range(NI) for f in q_step(pace, t + 1, hn.at[0], n)]),
            (-0.05, 0.97, xn_steps(pace, t + 1, hn.at[0])),
            (0.85, 1.93, xn_steps(pace, t + 2, attn.at[1])),
            (0, 1.97, kv_weight_steps(pace, j)),
        )
    _loop("phase_q", NI - 1, phase_q)
    for t in range(2, NT):
        for c in ffn_copies(t):
            c.start()
    wo_copy.wait()

    def first_values(pace, g):
        for c in range(8):
            v_v[0, c, pl.ds(0, HALO), :] = jnp.broadcast_to(
                v_v[0, c, pl.ds(HALO, 1), :], (HALO, LANES))
        tile, row = g // NI, pl.multiple_of(g % NI * GROUP, GROUP)
        return value_steps(pace, prob.at[:, pl.ds(row, H + GROUP)],
                           v_v.at[tile, :, pl.ds(row, HALO + H + GROUP)],
                           attn.at[tile, :, ds(row // 2, GROUP // 2)], range(0, GROUP, RB))

    def phase_kv(j):
        for c in ffn_copies(j):
            c.wait()

        wo_src = [wo_raw.at[pl.ds(pl.multiple_of(j // NI * 64, 64), D - 64),
                            ds(s * DH + j % NI * LANES, LANES)] for s in range(2)]
        wo_dst = w_ops[WO].at[:, pl.ds(pl.multiple_of(j // NI * 32, 32), GR // 2 - 32),
                              ds(j % NI * LANES, LANES)]

        def wo_step(c, hl):
            b = [_permuted_rows(wo_src[s], kh * 4 + c, hl) for kh in range(2) for s in range(2)]
            b[0] = pace.start(b[0].astype(F32))
            for i, t in enumerate(_rhs7(*b)):
                wo_dst[i * PER + c * LANES // GR,
                       pl.ds((c * LANES % GR + hl * 32) // 2, 16), :] = _words(t)
                pace.finish(_words(t)[i % 2 * 8:])

        pace = _Pacer(j)
        tile, row = j // NI, pl.multiple_of(j % NI * GROUP, GROUP)
        _emit(
            (0, 1, project(pace, j, weight(WKV), k_v)),
            (1, 2, project(pace, j, weight(WKV, 7 * PER), v_v)),
            (0.05, 1.95, ffn_weight_steps(pace, j)),
            (0.5, 1.05, permute_q_steps(pace, tile, [row, H + row])),
            (0.1, 0.7, [lambda c=c, hl=hl: wo_step(c, hl)
                         for c in range(4) for hl in range(2)]),
            (0.15, 1, first_values(pace, jnp.maximum(j - 1, 0))),
            (1.08, 2.0, softmax_steps(
                pace, q_v.at[tile, :, pl.ds(row, H + GROUP)],
                k_v.at[tile, :, pl.ds(row, HALO + H + GROUP)], prob.at[:, pl.ds(row, H + GROUP)],
                [s * H + r for s in range(2) for r in range(0, GROUP, SB)], tile * T + row)),
        )
    _loop("phase_kv", NT, phase_kv)
    _emit((0, 1, first_values(_Pacer(), jnp.int32(NT - 1))))

    def ffn(j):
        nxt = last(j + 2)
        slot = j % 2
        pace = _Pacer(j)
        gate = {}

        def gate_done(n, *c):
            gate[n] = [_gelu(t) for t in c]

        def up_done(n, *c):
            for i, t in enumerate(_lhs7(*[g * u for g, u in zip(gate.pop(n), c)])):
                act[i, :, n:n + TN] = _words(t)

        def down_done(n, *c):
            for b, t in enumerate(c):
                cols = pl.ds(b % 2 * DH + n, TN)
                out_v[ds(j * T + b // 2 * H, H), cols] = (
                    h_v[slot, pl.ds(b // 2 * H, H), cols] + t).astype(BF16)

        g = _matmul(pace, lambda i: hn[0, i], ffn_weight(ffn_w[0]), FH, gate_done)
        u = _matmul(pace, lambda i: hn[0, i], ffn_weight(ffn_w[1]), FH, up_done)
        gu = [f for n in range(0, len(g), 7) for f in g[n:n + 7] + u[n:n + 7]]
        _emit(
            (0, 1, gu),
            (1, 1.5, _matmul(pace, lambda i: act[i], ffn_weight(ffn_w[2]), DH, down_done)),
            (0.01, 0.62, softmax_steps(pace, q_v.at[nxt % 2], k_v.at[nxt], prob, range(0, T, SB))),
            (0.62, 0.995, value_steps(pace, prob, v_v.at[nxt], attn.at[slot], range(0, H, RB))),
            (1.02, 1.37, hn_steps(pace, 1 - slot, 0)),
            (1.39, 1.39, [c.start for c in out_copies(j, 0, DH - TN)]),
        )
        for c in out_copies(j, DH - TN, DH):
            c.start()

    def phase_ffn(t):
        @pl.when(t < NT)
        def _():
            pace = _Pacer(t)
            _emit((0, 1, output_steps(pace, t, t % 2)),
                  (-0.05, 0.92, hn_steps(pace, 0, jnp.where(t == 1, 0, 1))),
                  (0.0, 0.97, permute_q_steps(pace, last(t + 1), range(0, T, GROUP))))

        pl.when(t > 0)(lambda: ffn(t - 1))
    _loop("phase_ffn", NT + 1, phase_ffn)
    for j in range(NT):
        for c in out_copies(j, 0, DH - TN) + out_copies(j, DH - TN, DH):
            c.wait()


@jax.jit
def pallas_sequential_preLN__sliding_local_dilated__glu_gated_geglu__prompt_kernel(
    A_x: jax.Array,
    A_wqkv: jax.Array,
    A_wo: jax.Array,
    B_x: jax.Array,
    B_w_gate: jax.Array,
    B_w_up: jax.Array,
    B_w_down: jax.Array,
):
    del B_x
    B, S, D = A_x.shape
    F = B_w_gate.shape[1]
    DH, FH = D // 2, F // 2
    NT = S // T
    NI = NT // 2
    assert B == 1 and D == 8 * LANES and NI * LANES == DH and FH % GR == 0 and 2 * GR == DH
    any_spec = pl.BlockSpec(memory_space=pl.ANY)
    out = pl.pallas_call(
        _kernel,
        in_specs=[any_spec] * 6,
        out_specs=any_spec,
        out_shape=jax.ShapeDtypeStruct((S, D), A_x.dtype),
        scratch_shapes=[
            pltpu.VMEM((S + T, D), BF16),
            pltpu.VMEM((NI, D // GR, GR, 2 * TN), BF16),
            pltpu.VMEM((2, D // GR, GR, D), BF16),
            pltpu.VMEM((D, D), BF16),
            pltpu.VMEM((T, D), F32),
            [pltpu.VMEM((n * 7 * DH // GR, GR // 2, DH), U32)
             for n in (1, 2, 1)],
            [(pltpu.VMEM((k // GR, GR, n), BF16),
              pltpu.VMEM((3, k // 2 // GR, GR, n // 2), BF16))
             for k, n in ((D, F), (D, F), (F, D))],
            pltpu.VMEM((7 * NT + 7, H // 2, DH), U32),
            pltpu.VMEM((2, 7, H // 2, DH), U32),
            pltpu.VMEM((2, 7, H // 2, DH), U32),
            pltpu.VMEM((WINDOW, T, LANES), F32),
            pltpu.VMEM((7, H // 2, FH), U32),
            pltpu.VMEM((NT, 8, T, LANES), F32),
            pltpu.VMEM((2, 8, T, LANES), F32),
            pltpu.VMEM((NT + 1, 8, HALO + T, LANES), F32),
            pltpu.VMEM((NT + 1, 8, HALO + T, LANES), F32),
            pltpu.VMEM((2, T, D), F32),
            pltpu.VMEM((S, D), BF16),
            pltpu.SemaphoreType.DMA((NT + 1,)),
            pltpu.SemaphoreType.DMA((NI,)),
            pltpu.SemaphoreType.DMA((NI,)),
            pltpu.SemaphoreType.DMA((NI - 1,)),
            pltpu.SemaphoreType.DMA(()),
            pltpu.SemaphoreType.DMA((NT,)),
            pltpu.SemaphoreType.DMA((NT,)),
        ],
        compiler_params=pltpu.CompilerParams(vmem_limit_bytes=124 * 2**20),
    )(A_x.reshape(S, D), A_wqkv.reshape(D // GR, GR, 3 * D), A_wo,
      B_w_gate.reshape(D // GR, GR, F), B_w_up.reshape(D // GR, GR, F),
      B_w_down.reshape(F // GR, GR, D))
    return out.reshape(B, S, D)
```

```python
import jax
import jax.numpy as jnp
from jax import lax
import jax.experimental.pallas as pl
import jax.experimental.pallas.tpu as pltpu

HEAD_DIM = 32
WINDOW = 8
DILATION = 2
HALO = 16
LANES = 128
T = 256
H = T // 2
SB = 8
RB = 16
TN = 128
PLAIN = (1, 4)
GR = 256
SCOPES = False
F32 = jnp.float32
BF16 = jnp.bfloat16
U32 = jnp.uint32


def _words(x):
    return pltpu.bitcast(x, U32)


def _halves(x):
    return pltpu.bitcast(x, BF16)


def _loop(name, n, body):
    def step(j, carry):
        if SCOPES:
            with jax.named_scope(name):
                body(j)
        else:
            body(j)
        return carry
    lax.fori_loop(0, n, step, 0)


def _emit(*stages):
    order = []
    for s, (lo, hi, steps) in enumerate(stages):
        order += [(lo + (hi - lo) * i / len(steps), s, i, f) for i, f in enumerate(steps)]
    for _, _, _, f in sorted(order, key=lambda t: t[:3]):
        f()


def _pipelined(pieces, depth):
    def step(t):
        for g in reversed(pieces[max(t - depth + 1, 0):t + 1]):
            next(g, None)
    return [lambda t=t: step(t) for t in range(len(pieces) + depth - 1)]


class _Pacer:
    def __init__(self, step=None):
        self.never = None if step is None else jnp.full((8, LANES), step, jnp.int32) < 0
        self.products = []
        self.due = []

    def _tie(self, x, others):
        regs = [[x[r:r + 8, c:c + LANES] for c in range(0, x.shape[1], LANES)]
                for r in range(0, x.shape[0], 8)]
        for k, other in enumerate(others):
            row, col = k % len(regs), k // len(regs) % len(regs[0])
            if other.dtype != x.dtype:
                other = pltpu.bitcast(other, x.dtype)
            regs[row][col] = jnp.where(self.never, other[:8, :LANES], regs[row][col])
        return jnp.concatenate([jnp.concatenate(row, axis=1) for row in regs], axis=0)

    def start(self, x, lag=3):
        if self.never is None or len(self.products) < lag:
            return x
        return self._tie(x, [self.products[-lag]] * (x.shape[0] // 8))

    def finish(self, x):
        if self.never is not None:
            self.due.append(x)

    def dot(self, lhs_words, rhs):
        if self.due:
            lhs_words = self._tie(lhs_words, self.due)
            self.due = []
        self.products.append(jnp.dot(_halves(lhs_words), rhs, preferred_element_type=F32))
        return self.products[-1]


def _gelu(x):
    c = 0.7978845608028654
    hx = 0.5 * x
    return hx + hx * jnp.tanh(x * (c + (c * 0.044715) * (x * x)))


def _lhs7(a11, a12, a21, a22):
    return [t.astype(BF16) for t in
            (a11 + a22, a21 + a22, a11, a22, a11 + a12, a21 - a11, a12 - a22)]


def _rhs7(b11, b12, b21, b22):
    f11, f12, f21, f22 = (b.astype(F32) for b in (b11, b12, b21, b22))
    return [t.astype(BF16) for t in
            (f11 + f22, b11, f12 - f22, f21 - f11, b22, f11 + f12, f21 + f22)]


def _strassen(pace, lhs, rhs, done):
    c = {}

    def m(i):
        return pace.dot(lhs(i), rhs(i))

    def s0():
        c["m1"] = m(0)

    def s1():
        c["m2"] = m(1)
        c[22] = c["m1"] - c["m2"]

    def s2():
        t = m(3)
        c[21] = c["m2"] + t
        c[11] = c["m1"] + t

    def s3():
        c["m5"] = m(4)
        c[11] = c[11] - c["m5"]

    def s4():
        t = m(2)
        c[12] = c["m5"] + t
        c[22] = c[22] + t

    def s5():
        c[11] = c[11] + m(6)

    def s6():
        done(c[11], c[12], c[21], c[22] + m(5))

    return [s0, s1, s2, s3, s4, s5, s6]


def _matmul(pace, lhs, rhs, width, done):
    steps = []
    for n in range(0, width, TN):
        steps += _strassen(pace, lhs, lambda i, n=n: rhs(i, n), lambda *c, n=n: done(n, *c))
    return steps


def _permute_cols(chunks):
    blk = lax.broadcasted_iota(jnp.int32, chunks[0].shape, 1) // 4
    a = [pltpu.roll(chunks[c], 4 * c, 1) if c else chunks[c] for c in range(8)]
    yield
    e = [a[(-i) % 8] for i in range(8)]
    for s in (1, 2, 4):
        e = [jnp.where((blk & s) != 0, e[(i - s) % 8], e[i]) for i in range(8)]
    e = [pltpu.roll(e[c], LANES - 4 * c, 1) if c else e[c] for c in range(8)]
    yield
    return e


def _permuted_rows(ref, c, hl):
    parts = []
    for cp in range(8):
        r = c * 4
        u = _words(ref[pl.ds(cp * LANES + hl * 32 + r // 16 * 16, 16), :])
        parts.append(u[r % 16 // 2:r % 16 // 2 + 2, :])
    return _halves(jnp.concatenate(parts, axis=0))


def _kernel(x_hbm, wqkv_hbm, wo_hbm, wg_hbm, wu_hbm, wd_hbm, out_hbm,
            x_v, wq_raw, wkv_raw, wo_raw, centred, w_ops, ffn_w, a_ops, hn, attn, prob, act,
            q_raw, q_v, k_v, v_v, h_v, out_v,
            sem_x, sem_p, sem_q, sem_kv, sem_o, sem_f, sem_out):
    S, D = x_hbm.shape
    DH = D // 2
    FH = wg_hbm.shape[2] // 2
    NT = S // T
    NI = NT // 2
    FR = GR // NT
    NG = 2 * GR // RB
    KG = -(-NG // (NI - 1))
    GROUP = H // NI
    PER = DH // GR
    WQ, WKV, WO = range(3)

    def ds(start, size):
        return pl.ds(start if isinstance(start, int) else pl.multiple_of(start, size), size)

    def last(j):
        return min(j, NT - 1) if isinstance(j, int) else jnp.minimum(j, NT - 1)

    def x_copy(j):
        return pltpu.make_async_copy(x_hbm.at[ds(last(j) * T, T)], x_v.at[ds(j * T, T)],
                                     sem_x.at[j])

    def x_part_copy(n):
        return [pltpu.make_async_copy(x_hbm.at[ds(2 * T + s * H + n * GROUP, GROUP)],
                                      x_v.at[ds(2 * T + s * H + n * GROUP, GROUP)],
                                      sem_p.at[n]) for s in range(2)]

    def wq_copy(n):
        return pltpu.make_async_copy(wqkv_hbm.at[:, :, ds(n * 2 * TN, 2 * TN)],
                                     wq_raw.at[n], sem_q.at[n])

    def wkv_copies(j):
        copies = []
        for m in range(2):
            lo = max(j * KG * RB - m * GR, 0)
            hi = min((j + 1) * KG * RB - m * GR, GR)
            if lo < hi:
                copies.append(pltpu.make_async_copy(
                    wqkv_hbm.at[:, pl.ds(lo, hi - lo), pl.ds((1 + m) * D, D)],
                    wkv_raw.at[m, :, pl.ds(lo, hi - lo)], sem_kv.at[j]))
        return copies

    wo_copy = pltpu.make_async_copy(wo_hbm, wo_raw, sem_o)

    def ffn_copies(j):
        rows = ds(j * FR, FR)
        return [pltpu.make_async_copy(src.at[:, rows], dst.at[:, rows], sem_f.at[j])
                for src, (dst, _) in zip((wg_hbm, wu_hbm, wd_hbm), ffn_w)]

    def out_copies(j, lo, hi):
        return [pltpu.make_async_copy(out_v.at[ds(j * T, T), pl.ds(s * DH + lo, hi - lo)],
                                      out_hbm.at[ds(j * T, T), pl.ds(s * DH + lo, hi - lo)],
                                      sem_out.at[j]) for s in range(2)]

    def store_weight(m, i, g, row, col, t):
        w_ops[m][i * PER + g, ds(row // 2, t.shape[0] // 2), col] = _words(t)

    def weight(m, first=0):
        return lambda i, n: _halves(
            w_ops[m][pl.ds(first + i * PER, PER), :, ds(n, TN)].reshape(DH // 2, TN))

    def norm_steps(pace, load_rows, store, rows=range(0, H, RB)):
        def piece(r):
            def load():
                return jnp.concatenate([load_rows(s * H + r).astype(F32) for s in range(2)], axis=0)
            m = jnp.mean(pace.start(load()), axis=-1, keepdims=True)
            yield
            c = load() - m
            centred[ds(2 * r, 2 * RB), :] = c
            scale = lax.rsqrt(jnp.mean(c * c, axis=-1, keepdims=True) + 1e-5)
            yield
            y = centred[ds(2 * r, 2 * RB), :] * scale
            for i, t in enumerate(_lhs7(y[:RB, :DH], y[:RB, DH:], y[RB:, :DH], y[RB:, DH:])):
                store(i, ds(r // 2, RB // 2), _words(t))
                pace.finish(_words(t)[:, i % 4 * LANES:(i % 4 + 1) * LANES])
        return _pipelined([piece(r) for r in rows], 3)

    def xn_steps(pace, j, copy, *rows):
        def store(i, where, t):
            a_ops[7 * j + i, where, :] = t
            copy[i, where, :] = t
        return norm_steps(pace, lambda r: x_v[ds(j * T + r, RB), :], store, *rows)

    def hn_steps(pace, slot, dest):
        def store(i, rows, t):
            hn[dest, i, rows, :] = t
        return norm_steps(pace, lambda r: h_v[slot, pl.ds(r, RB), :], store)

    def q_weight_steps(pace, n):
        def step(g, r):
            top, bot = (wq_raw[n, kh * PER + g, pl.ds(r, 2 * RB), :] for kh in range(2))
            b11 = pace.start(top[:, :TN].astype(F32))
            for i, t in enumerate(_rhs7(b11, top[:, TN:], bot[:, :TN], bot[:, TN:])):
                store_weight(WQ, i, g, r, ds(n * TN, TN), t)
        return [lambda g=g, r=r: step(g, r) for g in range(PER) for r in range(0, GR, 2 * RB)]

    def kv_weight_steps(pace, j):
        def piece(g, group):
            m, row = group // (NG // 2), group % (NG // 2) * RB
            u = [jnp.concatenate(
                [_words(wkv_raw[m, kh * PER + g, ds(row, RB), pl.ds(c * LANES, LANES)])
                 for kh in range(2)], axis=0) for c in range(8)]
            u = yield from _permute_cols(u[:1] + [pace.start(u[1])] + u[2:])
            for c in range(4):
                b = [_halves(u[nh * 4 + c][kh * RB // 2:(kh + 1) * RB // 2])
                     for kh in range(2) for nh in range(2)]
                for i, t in enumerate(_rhs7(*b)):
                    store_weight(WKV, i, m * 7 * PER + g, row, pl.ds(c * LANES, LANES), t)
                    if i >= 5:
                        pace.finish(_words(t))
        return _pipelined([piece(g, jnp.minimum(j * KG + r, NG - 1)) for r in range(KG)
                           for g in range(PER)], 3)

    def ffn_index(w, i, g, rows, n, width):
        blocks, extra = w
        _, per, _, half = extra.shape
        if 1 <= i <= 4:
            g = pl.ds((i - 1) // 2 * per, per) if g is None else (i - 1) // 2 * per + g
            return blocks, (g, rows, pl.ds((i - 1) % 2 * half + n, width))
        return extra, (i % 4, slice(None) if g is None else g, rows, pl.ds(n, width))

    def ffn_weight_steps(pace, j):
        def step(w, g, n):
            where = [ffn_index(w, i, g, slice(None), n, 2 * LANES) for i in range(7)]
            blocks = [ref[idx] for ref, idx in where[1:5]]
            blocks[0] = pace.start(blocks[0].astype(F32), 3)
            pace.finish(blocks[0])
            for i, t in enumerate(_rhs7(*blocks)):
                if i not in PLAIN:
                    ref, idx = where[i]
                    ref[idx] = t
        chunk = [(blocks.at[:, ds(j * FR, FR)], extra.at[:, :, ds(j * FR, FR)])
                 for blocks, extra in ffn_w]
        steps = [[lambda w=w, g=g, n=n: step(w, g, n) for g in range(w[1].shape[1])
                  for n in range(0, w[1].shape[3], 2 * LANES)] for w in chunk]
        return [f for group in zip(*steps) for f in group]

    def ffn_weight(w):
        def load(i, n):
            ref, idx = ffn_index(w, i, None, slice(None), n, TN)
            return ref[idx].reshape(w[1].shape[1] * GR, TN)
        return load

    def permute_q_steps(pace, j, rows):
        def piece(r):
            q = [q_raw[j, c, ds(r, GROUP), :] for c in range(8)]
            q = yield from _permute_cols(q[:1] + [pace.start(q[1])] + q[2:])
            for c in range(8):
                q_v[j % 2, c, ds(r, GROUP), :] = q[c]
                pace.finish(q[c][c * 8 % GROUP:])
        return _pipelined([piece(r) for r in rows], 3)

    def q_step(pace, j, lhs, n):
        def done(*c):
            for b, t in enumerate(c):
                q_raw[j, 2 * n + b % 2, pl.ds(b // 2 * H, H), :] = t
        return _strassen(pace, lambda i: lhs[i], lambda i: weight(WQ)(i, n * TN), done)

    def project(pace, j, rhs, dst):
        lhs, dst = a_ops.at[pl.ds(7 * j, 7)], dst.at[pl.ds(j, 2)]

        def done(n, *c):
            for b, t in enumerate(c):
                chunk = (b % 2 * DH + n) // LANES
                dst[0, chunk, pl.ds(HALO + b // 2 * H, H), :] = t
                if b // 2:
                    dst[1, chunk, pl.ds(0, HALO), :] = t[H - HALO:]
        return _matmul(pace, lambda i: lhs[i], rhs, DH, done)

    def softmax_steps(pace, q, k, out, rows, first=None):
        def piece(r):
            logits = [None] * WINDOW
            for c in range(8):
                qc = q[c, pl.ds(r, SB), :]
                if c == 0:
                    qc = pace.start(qc)
                for w in range(WINDOW):
                    t = qc * k[c, pl.ds(HALO + r - DILATION * w, SB), :]
                    logits[w] = t if c == 0 else logits[w] + t
            lane = lax.broadcasted_iota(jnp.int32, (SB, LANES), 1)
            for s in (1, 2):
                rolled = [(pltpu.roll(l, s, 1), pltpu.roll(l, LANES - s, 1)) for l in logits]
                yield
                logits = [l + jnp.where((lane & s) != 0, a, b)
                          for l, (a, b) in zip(logits, rolled)]
            for w in range(WINDOW):
                l = logits[w] * (HEAD_DIM ** -0.5)
                if first is not None and r < DILATION * w:
                    pos = first + r + lax.broadcasted_iota(jnp.int32, (SB, LANES), 0)
                    l = jnp.where(pos >= DILATION * w, l, -1e9)
                logits[w] = l
            m = logits[0]
            for w in range(1, WINDOW):
                m = jnp.maximum(m, logits[w])
            e = [jnp.exp(l - m) for l in logits]
            total = e[0]
            for w in range(1, WINDOW):
                total = total + e[w]
            inv = 1.0 / total
            for w in range(WINDOW):
                p = e[w] * inv
                out[w, pl.ds(r, SB), :] = p
                pace.finish(p)
        return _pipelined([piece(r) for r in rows], 3)

    def value_steps(pace, weights, v, out, rows):
        def piece(r, c):
            blocks = []
            for row in (r, H + r):
                for chunk in (c, c + 4):
                    for w in range(WINDOW):
                        p = weights[w, pl.ds(row, RB), :]
                        t = (pace.start(p, 6) if w == 0 else p) * v[
                            chunk, pl.ds(HALO + row - DILATION * w, RB), :]
                        o = t if w == 0 else o + t
                    blocks.append(o)
                    pace.finish(o)
                    pace.finish(o[8:])
                    yield
            for i, t in enumerate(_lhs7(*blocks)):
                out[i, pl.ds(r // 2, RB // 2), pl.ds(c * LANES, LANES)] = _words(t)
                pace.finish(_words(t))
        pieces = [piece(r, c) for r in rows for c in range(4)]
        return [lambda g=g: next(g, None) for g in pieces for _ in range(5)]

    def output_steps(pace, j, slot):
        def done(n, *c):
            for b, t in enumerate(c):
                cols = pl.ds(b % 2 * DH + n, TN)
                h_v[slot, pl.ds(b // 2 * H, H), cols] = (
                    x_v[ds(j * T + b // 2 * H, H), cols].astype(F32) + t)
        return _matmul(pace, lambda i: attn[slot, i], weight(WO), DH, done)

    first = [x_copy(0), x_copy(1), wq_copy(0)]
    for c in first:
        c.start()
    later = [x_part_copy(n) + ([wq_copy(n + 1)] if n + 1 < NI else []) for n in range(NI)]
    for c in later[0]:
        c.start()
    prob[:, pl.ds(0, H + GROUP), :] = jnp.zeros((WINDOW, H + GROUP, LANES), F32)
    v_v[0, :, pl.ds(0, HALO + H + GROUP), :] = jnp.zeros((8, HALO + H + GROUP, LANES), F32)
    k_v[0, :, pl.ds(0, HALO), :] = jnp.zeros((8, HALO, LANES), F32)
    h_v[0] = jnp.zeros((T, D), F32)
    for c, steps in zip(first, (xn_steps(_Pacer(), 0, hn.at[0]), xn_steps(_Pacer(), 1, attn.at[0]),
                                q_weight_steps(_Pacer(), 0))):
        c.wait()
        _emit((0, 1, steps))
    for c in later[1]:
        c.start()
    batches = [sum(later[2:], [])] + [[x_copy(2 * j + 3), x_copy(2 * j + 4)] + wkv_copies(j)
                                      for j in range(NI - 1)]

    def first_q(n):
        pl.when(n + 1 < NI)(lambda: wq_copy(n + 1).wait())
        for c in x_part_copy(n):
            c.wait()
        for k, batch in enumerate(batches):
            @pl.when(n == k)
            def _():
                for c in batch:
                    c.start()
        pace = _Pacer(n)
        _emit(
            (0, 1, [f for fs in zip(q_step(pace, 0, hn.at[0], n), q_step(pace, 1, attn.at[0], n))
                    for f in fs]),
            (0.4, 0.986, q_weight_steps(pace, jnp.minimum(n + 1, NI - 1))),
            (-0.201, 0.557, xn_steps(pace, 2, attn.at[1],
                              [n * GROUP + r for r in range(0, GROUP, RB)])),
        )
    _loop("first_q", NI, first_q)
    for c in [wo_copy] + ffn_copies(0) + ffn_copies(1):
        c.start()

    def phase_q(j):
        t = 2 * j + 2
        x_copy(t + 1).wait()
        x_copy(t + 2).wait()
        for k in range(NI - 1):
            @pl.when(j == k)
            def _():
                for c in wkv_copies(k):
                    c.wait()
        pace = _Pacer(j)
        _emit(
            (0, 1, [f for n in range(NI) for f in q_step(pace, t, attn.at[1], n)]),
            (1, 2, [f for n in range(NI) for f in q_step(pace, t + 1, hn.at[0], n)]),
            (-0.131, 0.969, xn_steps(pace, t + 1, hn.at[0])),
            (0.82, 1.964, xn_steps(pace, t + 2, attn.at[1])),
            (0, 1.995, kv_weight_steps(pace, j)),
        )
    _loop("phase_q", NI - 1, phase_q)
    for t in range(2, NT):
        for c in ffn_copies(t):
            c.start()
    wo_copy.wait()

    def first_values(pace, g):
        for c in range(8):
            v_v[0, c, pl.ds(0, HALO), :] = jnp.broadcast_to(
                v_v[0, c, pl.ds(HALO, 1), :], (HALO, LANES))
        tile, row = g // NI, pl.multiple_of(g % NI * GROUP, GROUP)
        return value_steps(pace, prob.at[:, pl.ds(row, H + GROUP)],
                           v_v.at[tile, :, pl.ds(row, HALO + H + GROUP)],
                           attn.at[tile, :, ds(row // 2, GROUP // 2)], range(0, GROUP, RB))

    def phase_kv(j):
        for c in ffn_copies(j):
            c.wait()

        wo_src = [wo_raw.at[pl.ds(pl.multiple_of(j // NI * 64, 64), D - 64),
                            ds(s * DH + j % NI * LANES, LANES)] for s in range(2)]
        wo_dst = w_ops[WO].at[:, pl.ds(pl.multiple_of(j // NI * 32, 32), GR // 2 - 32),
                              ds(j % NI * LANES, LANES)]

        def wo_step(c, hl):
            b = [_permuted_rows(wo_src[s], kh * 4 + c, hl) for kh in range(2) for s in range(2)]
            b[0] = pace.start(b[0].astype(F32))
            for i, t in enumerate(_rhs7(*b)):
                wo_dst[i * PER + c * LANES // GR,
                       pl.ds((c * LANES % GR + hl * 32) // 2, 16), :] = _words(t)
                pace.finish(_words(t)[i % 2 * 8:])

        pace = _Pacer(j)
        tile, row = j // NI, pl.multiple_of(j % NI * GROUP, GROUP)
        _emit(
            (0, 1, project(pace, j, weight(WKV), k_v)),
            (1, 2, project(pace, j, weight(WKV, 7 * PER), v_v)),
            (0.107, 1.883, ffn_weight_steps(pace, j)),
            (0.447, 1.05, permute_q_steps(pace, tile, [row, H + row])),
            (0.1, 0.6, [lambda c=c, hl=hl: wo_step(c, hl)
                         for c in range(4) for hl in range(2)]),
            (0.155, 1.035, first_values(pace, jnp.maximum(j - 1, 0))),
            (1.042, 2.043, softmax_steps(
                pace, q_v.at[tile, :, pl.ds(row, H + GROUP)],
                k_v.at[tile, :, pl.ds(row, HALO + H + GROUP)], prob.at[:, pl.ds(row, H + GROUP)],
                [s * H + r for s in range(2) for r in range(0, GROUP, SB)], tile * T + row)),
        )
    _loop("phase_kv", NT, phase_kv)
    _emit((0, 1, first_values(_Pacer(), jnp.int32(NT - 1))))

    def ffn(j):
        nxt = last(j + 2)
        slot = j % 2
        pace = _Pacer(j)
        gate = {}

        def gate_done(n, *c):
            gate[n] = [_gelu(t) for t in c]

        def up_done(n, *c):
            for i, t in enumerate(_lhs7(*[g * u for g, u in zip(gate.pop(n), c)])):
                act[i, :, n:n + TN] = _words(t)

        def down_done(n, *c):
            for b, t in enumerate(c):
                cols = pl.ds(b % 2 * DH + n, TN)
                out_v[ds(j * T + b // 2 * H, H), cols] = (
                    h_v[slot, pl.ds(b // 2 * H, H), cols] + t).astype(BF16)

        g = _matmul(pace, lambda i: hn[0, i], ffn_weight(ffn_w[0]), FH, gate_done)
        u = _matmul(pace, lambda i: hn[0, i], ffn_weight(ffn_w[1]), FH, up_done)
        gu = [f for n in range(0, len(g), 7) for f in g[n:n + 7] + u[n:n + 7]]
        _emit(
            (0, 1, gu),
            (1, 1.5, _matmul(pace, lambda i: act[i], ffn_weight(ffn_w[2]), DH, down_done)),
            (0.012, 0.62, softmax_steps(pace, q_v.at[nxt % 2], k_v.at[nxt], prob, range(0, T, SB))),
            (0.592, 0.99, value_steps(pace, prob, v_v.at[nxt], attn.at[slot], range(0, H, RB))),
            (1.004, 1.45, hn_steps(pace, 1 - slot, 0)),
            (1.39, 1.39, [c.start for c in out_copies(j, 0, DH - TN)]),
        )
        for c in out_copies(j, DH - TN, DH):
            c.start()

    def phase_ffn(t):
        @pl.when(t < NT)
        def _():
            pace = _Pacer(t)
            _emit((0, 1, output_steps(pace, t, t % 2)),
                  (-0.108, 1.03, hn_steps(pace, 0, jnp.where(t == 1, 0, 1))),
                  (0.036, 0.983, permute_q_steps(pace, last(t + 1), range(0, T, GROUP))))

        pl.when(t > 0)(lambda: ffn(t - 1))
    _loop("phase_ffn", NT + 1, phase_ffn)
    for j in range(NT):
        for c in out_copies(j, 0, DH - TN) + out_copies(j, DH - TN, DH):
            c.wait()


@jax.jit
def pallas_sequential_preLN__sliding_local_dilated__glu_gated_geglu__prompt_kernel(
    A_x: jax.Array,
    A_wqkv: jax.Array,
    A_wo: jax.Array,
    B_x: jax.Array,
    B_w_gate: jax.Array,
    B_w_up: jax.Array,
    B_w_down: jax.Array,
):
    del B_x
    B, S, D = A_x.shape
    F = B_w_gate.shape[1]
    DH, FH = D // 2, F // 2
    NT = S // T
    NI = NT // 2
    assert B == 1 and D == 8 * LANES and NI * LANES == DH and FH % GR == 0 and 2 * GR == DH
    any_spec = pl.BlockSpec(memory_space=pl.ANY)
    out = pl.pallas_call(
        _kernel,
        in_specs=[any_spec] * 6,
        out_specs=any_spec,
        out_shape=jax.ShapeDtypeStruct((S, D), A_x.dtype),
        scratch_shapes=[
            pltpu.VMEM((S + T, D), BF16),
            pltpu.VMEM((NI, D // GR, GR, 2 * TN), BF16),
            pltpu.VMEM((2, D // GR, GR, D), BF16),
            pltpu.VMEM((D, D), BF16),
            pltpu.VMEM((T, D), F32),
            [pltpu.VMEM((n * 7 * DH // GR, GR // 2, DH), U32)
             for n in (1, 2, 1)],
            [(pltpu.VMEM((k // GR, GR, n), BF16),
              pltpu.VMEM((3, k // 2 // GR, GR, n // 2), BF16))
             for k, n in ((D, F), (D, F), (F, D))],
            pltpu.VMEM((7 * NT + 7, H // 2, DH), U32),
            pltpu.VMEM((2, 7, H // 2, DH), U32),
            pltpu.VMEM((2, 7, H // 2, DH), U32),
            pltpu.VMEM((WINDOW, T, LANES), F32),
            pltpu.VMEM((7, H // 2, FH), U32),
            pltpu.VMEM((NT, 8, T, LANES), F32),
            pltpu.VMEM((2, 8, T, LANES), F32),
            pltpu.VMEM((NT + 1, 8, HALO + T, LANES), F32),
            pltpu.VMEM((NT + 1, 8, HALO + T, LANES), F32),
            pltpu.VMEM((2, T, D), F32),
            pltpu.VMEM((S, D), BF16),
            pltpu.SemaphoreType.DMA((NT + 1,)),
            pltpu.SemaphoreType.DMA((NI,)),
            pltpu.SemaphoreType.DMA((NI,)),
            pltpu.SemaphoreType.DMA((NI - 1,)),
            pltpu.SemaphoreType.DMA(()),
            pltpu.SemaphoreType.DMA((NT,)),
            pltpu.SemaphoreType.DMA((NT,)),
        ],
        compiler_params=pltpu.CompilerParams(vmem_limit_bytes=124 * 2**20),
    )(A_x.reshape(S, D), A_wqkv.reshape(D // GR, GR, 3 * D), A_wo,
      B_w_gate.reshape(D // GR, GR, F), B_w_up.reshape(D // GR, GR, F),
      B_w_down.reshape(F // GR, GR, D))
    return out.reshape(B, S, D)
```

```python
import jax
import jax.numpy as jnp
from jax import lax
import jax.experimental.pallas as pl
import jax.experimental.pallas.tpu as pltpu

HEAD_DIM = 32
WINDOW = 8
DILATION = 2
HALO = 16
LANES = 128
T = 256
H = T // 2
SB = 8
RB = 16
TN = 128
PLAIN = (1, 4)
GR = 256
SCOPES = False
F32 = jnp.float32
BF16 = jnp.bfloat16
U32 = jnp.uint32


def _words(x):
    return pltpu.bitcast(x, U32)


def _halves(x):
    return pltpu.bitcast(x, BF16)


def _loop(name, n, body):
    def step(j, carry):
        if SCOPES:
            with jax.named_scope(name):
                body(j)
        else:
            body(j)
        return carry
    lax.fori_loop(0, n, step, 0)


def _emit(*stages):
    order = []
    for s, (lo, hi, steps) in enumerate(stages):
        order += [(lo + (hi - lo) * i / len(steps), s, i, f) for i, f in enumerate(steps)]
    for _, _, _, f in sorted(order, key=lambda t: t[:3]):
        f()


def _pipelined(pieces, depth):
    def step(t):
        for g in reversed(pieces[max(t - depth + 1, 0):t + 1]):
            next(g, None)
    return [lambda t=t: step(t) for t in range(len(pieces) + depth - 1)]


class _Pacer:
    def __init__(self, value=None):
        if value is None:
            self.never = None
        else:
            value = jnp.broadcast_to(value, (8, LANES))
            self.never = (value > 1) & (value < -1)
        self.products = []
        self.due = []

    def _tie(self, x, others):
        regs = [[x[r:r + 8, c:c + LANES] for c in range(0, x.shape[1], LANES)]
                for r in range(0, x.shape[0], 8)]
        for k, other in enumerate(others):
            row, col = k % len(regs), k // len(regs) % len(regs[0])
            if other.dtype != x.dtype:
                other = pltpu.bitcast(other, x.dtype)
            regs[row][col] = jnp.where(self.never, other[:8, :LANES], regs[row][col])
        return jnp.concatenate([jnp.concatenate(row, axis=1) for row in regs], axis=0)

    def start(self, x, lag=3):
        if self.never is None or len(self.products) < lag:
            return x
        return self._tie(x, [self.products[-lag]] * (x.shape[0] // 8))

    def finish(self, x):
        if self.never is not None:
            self.due.append(x)

    def dot(self, lhs_words, rhs):
        if self.due:
            lhs_words = self._tie(lhs_words, self.due)
            self.due = []
        self.products.append(jnp.dot(_halves(lhs_words), rhs, preferred_element_type=F32))
        return self.products[-1]


def _gelu(x):
    c = 0.7978845608028654
    hx = 0.5 * x
    return hx + hx * jnp.tanh(x * (c + (c * 0.044715) * (x * x)))


def _lhs7(a11, a12, a21, a22):
    return [t.astype(BF16) for t in
            (a11 + a22, a21 + a22, a11, a22, a11 + a12, a21 - a11, a12 - a22)]


def _rhs7(b11, b12, b21, b22):
    f11, f12, f21, f22 = (b.astype(F32) for b in (b11, b12, b21, b22))
    return [t.astype(BF16) for t in
            (f11 + f22, b11, f12 - f22, f21 - f11, b22, f11 + f12, f21 + f22)]


def _strassen(pace, lhs, rhs, done):
    c = {}

    def m(i):
        return pace.dot(lhs(i), rhs(i))

    def s0():
        c["m1"] = m(0)

    def s1():
        c["m2"] = m(1)
        c[22] = c["m1"] - c["m2"]

    def s2():
        t = m(3)
        c[21] = c["m2"] + t
        c[11] = c["m1"] + t

    def s3():
        c["m5"] = m(4)
        c[11] = c[11] - c["m5"]

    def s4():
        t = m(2)
        c[12] = c["m5"] + t
        c[22] = c[22] + t

    def s5():
        c[11] = c[11] + m(6)

    def s6():
        done(c[11], c[12], c[21], c[22] + m(5))

    return [s0, s1, s2, s3, s4, s5, s6]


def _matmul(pace, lhs, rhs, width, done):
    steps = []
    for n in range(0, width, TN):
        steps += _strassen(pace, lhs, lambda i, n=n: rhs(i, n), lambda *c, n=n: done(n, *c))
    return steps


def _permute_cols(chunks):
    blk = lax.broadcasted_iota(jnp.int32, chunks[0].shape, 1) // 4
    a = [pltpu.roll(chunks[c], 4 * c, 1) if c else chunks[c] for c in range(8)]
    yield
    e = [a[(-i) % 8] for i in range(8)]
    for s in (1, 2, 4):
        e = [jnp.where((blk & s) != 0, e[(i - s) % 8], e[i]) for i in range(8)]
    e = [pltpu.roll(e[c], LANES - 4 * c, 1) if c else e[c] for c in range(8)]
    yield
    return e


def _permuted_rows(ref, c, hl):
    parts = []
    for cp in range(8):
        r = c * 4
        u = _words(ref[pl.ds(cp * LANES + hl * 32 + r // 16 * 16, 16), :])
        parts.append(u[r % 16 // 2:r % 16 // 2 + 2, :])
    return _halves(jnp.concatenate(parts, axis=0))


def _kernel(x_hbm, wqkv_hbm, wo_hbm, wg_hbm, wu_hbm, wd_hbm, out_hbm,
            x_v, wq_raw, wkv_raw, wo_raw, centred, w_ops, ffn_w, a_ops, hn, attn, prob, act,
            q_raw, q_v, k_v, v_v, h_v, out_v,
            sem_x, sem_q, sem_kv, sem_o, sem_f, sem_out):
    S, D = x_hbm.shape
    DH = D // 2
    FH = wg_hbm.shape[2] // 2
    NT = S // T
    NI = NT // 2
    FR = GR // NT
    NG = 2 * GR // RB
    KG = -(-NG // (NI - 1))
    SKIP = KG * (NI - 1) - NG
    GROUP = H // NI
    PER = DH // GR
    WQ, WKV, WO = range(3)

    def ds(start, size):
        return pl.ds(start if isinstance(start, int) else pl.multiple_of(start, size), size)

    def last(j):
        return min(j, NT - 1) if isinstance(j, int) else jnp.minimum(j, NT - 1)

    def x_copy(j):
        return pltpu.make_async_copy(x_hbm.at[ds(last(j) * T, T)], x_v.at[ds(j * T, T)],
                                     sem_x.at[j])

    def wq_copy(n):
        return pltpu.make_async_copy(wqkv_hbm.at[:, :, ds(n * 2 * TN, 2 * TN)],
                                     wq_raw.at[n], sem_q.at[n])

    def wkv_copies(j):
        copies = []
        for m in range(2):
            lo = max((j * KG - SKIP) * RB - m * GR, 0)
            hi = min(((j + 1) * KG - SKIP) * RB - m * GR, GR)
            if lo < hi:
                copies.append(pltpu.make_async_copy(
                    wqkv_hbm.at[:, pl.ds(lo, hi - lo), pl.ds((1 + m) * D, D)],
                    wkv_raw.at[m, :, pl.ds(lo, hi - lo)], sem_kv.at[j]))
        return copies

    wo_copy = pltpu.make_async_copy(wo_hbm, wo_raw, sem_o)

    def ffn_copies(j):
        rows = ds(j * FR, FR)
        return [pltpu.make_async_copy(src.at[:, rows], dst.at[:, rows], sem_f.at[j])
                for src, (dst, _) in zip((wg_hbm, wu_hbm, wd_hbm), ffn_w)]

    def out_copies(j, lo, hi):
        return [pltpu.make_async_copy(out_v.at[ds(j * T, T), pl.ds(s * DH + lo, hi - lo)],
                                      out_hbm.at[ds(j * T, T), pl.ds(s * DH + lo, hi - lo)],
                                      sem_out.at[j]) for s in range(2)]

    def store_weight(m, i, g, row, col, t):
        w_ops[m][i * PER + g, ds(row // 2, t.shape[0] // 2), col] = _words(t)

    def weight(m, first=0):
        return lambda i, n: _halves(
            w_ops[m][pl.ds(first + i * PER, PER), :, ds(n, TN)].reshape(DH // 2, TN))

    def norm_steps(pace, load_rows, store):
        def piece(r):
            def load():
                return jnp.concatenate([load_rows(s * H + r).astype(F32) for s in range(2)], axis=0)
            m = jnp.mean(pace.start(load()), axis=-1, keepdims=True)
            yield
            c = load() - m
            centred[ds(2 * r, 2 * RB), :] = c
            scale = lax.rsqrt(jnp.mean(c * c, axis=-1, keepdims=True) + 1e-5)
            yield
            y = centred[ds(2 * r, 2 * RB), :] * scale
            for i, t in enumerate(_lhs7(y[:RB, :DH], y[:RB, DH:], y[RB:, :DH], y[RB:, DH:])):
                store(i, ds(r // 2, RB // 2), _words(t))
                pace.finish(_words(t)[:, i % 4 * LANES:(i % 4 + 1) * LANES])
        return _pipelined([piece(r) for r in range(0, H, RB)], 3)

    def xn_steps(pace, j, copy):
        def store(i, where, t):
            a_ops[7 * j + i, where, :] = t
            copy[i, where, :] = t
        return norm_steps(pace, lambda r: x_v[ds(j * T + r, RB), :], store)

    def hn_steps(pace, slot, dest):
        def store(i, rows, t):
            hn[dest, i, rows, :] = t
        return norm_steps(pace, lambda r: h_v[slot, pl.ds(r, RB), :], store)

    def q_weight_steps(pace, n):
        def step(g, r):
            top, bot = (wq_raw[n, kh * PER + g, pl.ds(r, 2 * RB), :] for kh in range(2))
            b11 = pace.start(top[:, :TN].astype(F32))
            for i, t in enumerate(_rhs7(b11, top[:, TN:], bot[:, :TN], bot[:, TN:])):
                store_weight(WQ, i, g, r, ds(n * TN, TN), t)
                pace.finish(_words(t)[i % 2 * 8:])
        return [lambda g=g, r=r: step(g, r) for g in range(PER) for r in range(0, GR, 2 * RB)]

    def kv_weight_steps(pace, j):
        def piece(g, group):
            m, row = group // (NG // 2), group % (NG // 2) * RB
            u = [jnp.concatenate(
                [_words(wkv_raw[m, kh * PER + g, ds(row, RB), pl.ds(c * LANES, LANES)])
                 for kh in range(2)], axis=0) for c in range(8)]
            u = yield from _permute_cols(u[:1] + [pace.start(u[1])] + u[2:])
            for c in range(4):
                b = [_halves(u[nh * 4 + c][kh * RB // 2:(kh + 1) * RB // 2])
                     for kh in range(2) for nh in range(2)]
                for i, t in enumerate(_rhs7(*b)):
                    store_weight(WKV, i, m * 7 * PER + g, row, pl.ds(c * LANES, LANES), t)
                    if i >= 5:
                        pace.finish(_words(t))
        return _pipelined([piece(g, jnp.maximum(j * KG - SKIP + r, 0)) for r in range(KG)
                           for g in range(PER)], 3)

    def ffn_index(w, i, g, rows, n, width):
        blocks, extra = w
        _, per, _, half = extra.shape
        if 1 <= i <= 4:
            g = pl.ds((i - 1) // 2 * per, per) if g is None else (i - 1) // 2 * per + g
            return blocks, (g, rows, pl.ds((i - 1) % 2 * half + n, width))
        return extra, (i % 4, slice(None) if g is None else g, rows, pl.ds(n, width))

    def ffn_weight_steps(pace, j):
        def step(w, g, n):
            where = [ffn_index(w, i, g, slice(None), n, 2 * LANES) for i in range(7)]
            blocks = [ref[idx] for ref, idx in where[1:5]]
            blocks[0] = pace.start(blocks[0].astype(F32), 3)
            pace.finish(blocks[0])
            for i, t in enumerate(_rhs7(*blocks)):
                if i not in PLAIN:
                    ref, idx = where[i]
                    ref[idx] = t
        chunk = [(blocks.at[:, ds(j * FR, FR)], extra.at[:, :, ds(j * FR, FR)])
                 for blocks, extra in ffn_w]
        steps = [[lambda w=w, g=g, n=n: step(w, g, n) for g in range(w[1].shape[1])
                  for n in range(0, w[1].shape[3], 2 * LANES)] for w in chunk]
        return [f for group in zip(*steps) for f in group]

    def ffn_weight(w):
        def load(i, n):
            ref, idx = ffn_index(w, i, None, slice(None), n, TN)
            return ref[idx].reshape(w[1].shape[1] * GR, TN)
        return load

    def permute_q_steps(pace, j, rows):
        def piece(r):
            q = [q_raw[j, c, ds(r, GROUP), :] for c in range(8)]
            q = yield from _permute_cols(q[:1] + [pace.start(q[1])] + q[2:])
            for c in range(8):
                q_v[j % 2, c, ds(r, GROUP), :] = q[c]
                pace.finish(q[c][c * 8 % GROUP:])
        return _pipelined([piece(r) for r in rows], 3)

    def q_step(pace, j, lhs, n):
        def done(*c):
            for b, t in enumerate(c):
                q_raw[j, 2 * n + b % 2, pl.ds(b // 2 * H, H), :] = t
        return _strassen(pace, lambda i: lhs[i], lambda i: weight(WQ)(i, n * TN), done)

    def project(pace, j, rhs, dst):
        lhs, dst = a_ops.at[pl.ds(7 * j, 7)], dst.at[pl.ds(j, 2)]

        def done(n, *c):
            for b, t in enumerate(c):
                chunk = (b % 2 * DH + n) // LANES
                dst[0, chunk, pl.ds(HALO + b // 2 * H, H), :] = t
                if b // 2:
                    dst[1, chunk, pl.ds(0, HALO), :] = t[H - HALO:]
        return _matmul(pace, lambda i: lhs[i], rhs, DH, done)

    def softmax_steps(pace, q, k, out, rows, first=None):
        def piece(r):
            logits = [None] * WINDOW
            for c in range(8):
                qc = q[c, pl.ds(r, SB), :]
                if c == 0:
                    qc = pace.start(qc)
                for w in range(WINDOW):
                    t = qc * k[c, pl.ds(HALO + r - DILATION * w, SB), :]
                    logits[w] = t if c == 0 else logits[w] + t
            lane = lax.broadcasted_iota(jnp.int32, (SB, LANES), 1)
            for s in (1, 2):
                rolled = [(pltpu.roll(l, s, 1), pltpu.roll(l, LANES - s, 1)) for l in logits]
                yield
                logits = [l + jnp.where((lane & s) != 0, a, b)
                          for l, (a, b) in zip(logits, rolled)]
            for w in range(WINDOW):
                l = logits[w] * (HEAD_DIM ** -0.5)
                if first is not None and r < DILATION * w:
                    pos = first + r + lax.broadcasted_iota(jnp.int32, (SB, LANES), 0)
                    l = jnp.where(pos >= DILATION * w, l, -1e9)
                logits[w] = l
            m = logits[0]
            for w in range(1, WINDOW):
                m = jnp.maximum(m, logits[w])
            e = [jnp.exp(l - m) for l in logits]
            total = e[0]
            for w in range(1, WINDOW):
                total = total + e[w]
            inv = 1.0 / total
            for w in range(WINDOW):
                p = e[w] * inv
                out[w, pl.ds(r, SB), :] = p
                pace.finish(p)
        return _pipelined([piece(r) for r in rows], 3)

    def value_steps(pace, weights, v, out, rows):
        def piece(r, c):
            blocks = []
            for row in (r, H + r):
                for chunk in (c, c + 4):
                    for w in range(WINDOW):
                        p = weights[w, pl.ds(row, RB), :]
                        t = (pace.start(p, 6) if w == 0 else p) * v[
                            chunk, pl.ds(HALO + row - DILATION * w, RB), :]
                        o = t if w == 0 else o + t
                    blocks.append(o)
                    pace.finish(o)
                    pace.finish(o[8:])
                    yield
            for i, t in enumerate(_lhs7(*blocks)):
                out[i, pl.ds(r // 2, RB // 2), pl.ds(c * LANES, LANES)] = _words(t)
                pace.finish(_words(t))
        pieces = [piece(r, c) for r in rows for c in range(4)]
        return [lambda g=g: next(g, None) for g in pieces for _ in range(5)]

    def output_steps(pace, j, slot):
        def done(n, *c):
            for b, t in enumerate(c):
                cols = pl.ds(b % 2 * DH + n, TN)
                h_v[slot, pl.ds(b // 2 * H, H), cols] = (
                    x_v[ds(j * T + b // 2 * H, H), cols].astype(F32) + t)
        return _matmul(pace, lambda i: attn[slot, i], weight(WO), DH, done)

    def start(*copies):
        for c in copies:
            c.start()

    start(x_copy(0), wq_copy(0), x_copy(1))
    def clear(c):
        prob[c, pl.ds(0, H + GROUP), :] = jnp.zeros((H + GROUP, LANES), F32)
        v_v[0, c, pl.ds(0, HALO + H + GROUP), :] = jnp.zeros((HALO + H + GROUP, LANES), F32)
        k_v[0, c, pl.ds(0, HALO), :] = jnp.zeros((HALO, LANES), F32)
        h_v[0, ds(c * (T // 8), T // 8), :] = jnp.zeros((T // 8, D), F32)
    _loop("clear", 8, clear)
    x_copy(0).wait()
    start(wq_copy(1))
    _emit((0, 1, xn_steps(_Pacer(), 0, hn.at[0])))
    wq_copy(0).wait()
    start(wq_copy(2))
    _emit((0, 1, q_weight_steps(_Pacer(), 0)))

    def first_q(pace, n, tiles=(0, 1)):
        return [f for t in tiles for f in q_step(pace, t, (hn.at[0], attn.at[0])[t], n)]

    def wkv_batch(j):
        return [x_copy(2 * j + 3), x_copy(2 * j + 4)] + wkv_copies(j)

    x_copy(1).wait()
    start(wq_copy(3))
    pace = _Pacer(x_v[pl.ds(0, 8), pl.ds(0, LANES)].astype(F32))
    _emit((0, 1, first_q(pace, 0, [0])), (0, 1.2, xn_steps(pace, 1, attn.at[0])))
    start(x_copy(2))
    wq_copy(1).wait()
    pace = _Pacer(x_v[pl.ds(0, 8), pl.ds(0, LANES)].astype(F32))
    _emit((0, 1, first_q(pace, 0, [1])), (0.1, 0.9, q_weight_steps(pace, 1)))
    wq_copy(2).wait()
    start(*wkv_batch(0))
    pace = _Pacer(x_v[pl.ds(0, 8), pl.ds(0, LANES)].astype(F32))
    _emit((0, 1, first_q(pace, 1)), (0.05, 0.93, q_weight_steps(pace, 2)))
    wq_copy(3).wait()
    x_copy(2).wait()
    pace = _Pacer(x_v[pl.ds(0, 8), pl.ds(0, LANES)].astype(F32))
    _emit((0, 1, first_q(pace, 2)), (1, 2, first_q(pace, 3)),
          (0.05, 0.9, q_weight_steps(pace, 3)), (0.1, 1.95, xn_steps(pace, 2, attn.at[1])))
    following = [wkv_batch(1) + wkv_batch(2), [wo_copy] + ffn_copies(0), ffn_copies(1)]

    def phase_q(j):
        t = 2 * j + 2
        x_copy(t + 1).wait()
        x_copy(t + 2).wait()
        for k in range(NI - 1):
            @pl.when(j == k)
            def _():
                for c in wkv_copies(k):
                    c.wait()
                start(*following[k])
        pace = _Pacer(j)
        _emit(
            (0, 1, [f for n in range(NI) for f in q_step(pace, t, attn.at[1], n)]),
            (1, 2, [f for n in range(NI) for f in q_step(pace, t + 1, hn.at[0], n)]),
            (-0.131, 0.969, xn_steps(pace, t + 1, hn.at[0])),
            (0.82, 1.964, xn_steps(pace, t + 2, attn.at[1])),
            (0, 1.995, kv_weight_steps(pace, j)),
        )
    _loop("phase_q", NI - 1, phase_q)
    wo_copy.wait()

    def first_values(pace, g):
        for c in range(8):
            v_v[0, c, pl.ds(0, HALO), :] = jnp.broadcast_to(
                v_v[0, c, pl.ds(HALO, 1), :], (HALO, LANES))
        tile, row = g // NI, ds(g % NI * GROUP, GROUP).start
        return value_steps(pace, prob.at[:, pl.ds(row, H + GROUP)],
                           v_v.at[tile, :, pl.ds(row, HALO + H + GROUP)],
                           attn.at[tile, :, ds(row // 2, GROUP // 2)], range(0, GROUP, RB))

    def phase_kv(j):
        for c in ffn_copies(j):
            c.wait()
        pl.when(j + 2 < NT)(lambda: start(*ffn_copies(j + 2)))

        wo_src = [wo_raw.at[pl.ds(pl.multiple_of(j // NI * 64, 64), D - 64),
                            ds(s * DH + j % NI * LANES, LANES)] for s in range(2)]
        wo_dst = w_ops[WO].at[:, pl.ds(pl.multiple_of(j // NI * 32, 32), GR // 2 - 32),
                              ds(j % NI * LANES, LANES)]

        def wo_step(c, hl):
            b = [_permuted_rows(wo_src[s], kh * 4 + c, hl) for kh in range(2) for s in range(2)]
            b[0] = pace.start(b[0].astype(F32))
            for i, t in enumerate(_rhs7(*b)):
                wo_dst[i * PER + c * LANES // GR,
                       pl.ds((c * LANES % GR + hl * 32) // 2, 16), :] = _words(t)
                pace.finish(_words(t)[i % 2 * 8:])

        pace = _Pacer(j)
        tile, row = j // NI, pl.multiple_of(j % NI * GROUP, GROUP)
        _emit(
            (0, 1, project(pace, j, weight(WKV), k_v)),
            (1, 2, project(pace, j, weight(WKV, 7 * PER), v_v)),
            (0.107, 1.883, ffn_weight_steps(pace, j)),
            (0.447, 1.05, permute_q_steps(pace, tile, [row, H + row])),
            (0.1, 0.6, [lambda c=c, hl=hl: wo_step(c, hl)
                         for c in range(4) for hl in range(2)]),
            (0.155, 1.035, first_values(pace, jnp.maximum(j - 1, 0))),
            (1.042, 2.043, softmax_steps(
                pace, q_v.at[tile, :, pl.ds(row, H + GROUP)],
                k_v.at[tile, :, pl.ds(row, HALO + H + GROUP)], prob.at[:, pl.ds(row, H + GROUP)],
                [s * H + r for s in range(2) for r in range(0, GROUP, SB)], tile * T + row)),
        )
    _loop("phase_kv", NT, phase_kv)
    _emit((0, 1, first_values(_Pacer(), NT - 1)))

    def ffn(j):
        nxt = last(j + 2)
        slot = j % 2
        pace = _Pacer(j)
        gate = {}

        def gate_done(n, *c):
            gate[n] = [_gelu(t) for t in c]

        def up_done(n, *c):
            for i, t in enumerate(_lhs7(*[g * u for g, u in zip(gate.pop(n), c)])):
                act[i, :, n:n + TN] = _words(t)

        def down_done(n, *c):
            for b, t in enumerate(c):
                cols = pl.ds(b % 2 * DH + n, TN)
                out_v[ds(j * T + b // 2 * H, H), cols] = (
                    h_v[slot, pl.ds(b // 2 * H, H), cols] + t).astype(BF16)

        g = _matmul(pace, lambda i: hn[0, i], ffn_weight(ffn_w[0]), FH, gate_done)
        u = _matmul(pace, lambda i: hn[0, i], ffn_weight(ffn_w[1]), FH, up_done)
        gu = [f for n in range(0, len(g), 7) for f in g[n:n + 7] + u[n:n + 7]]
        _emit(
            (0, 1, gu),
            (1, 1.5, _matmul(pace, lambda i: act[i], ffn_weight(ffn_w[2]), DH, down_done)),
            (0.012, 0.62, softmax_steps(pace, q_v.at[nxt % 2], k_v.at[nxt], prob, range(0, T, SB))),
            (0.592, 0.99, value_steps(pace, prob, v_v.at[nxt], attn.at[slot], range(0, H, RB))),
            (1.004, 1.45, hn_steps(pace, 1 - slot, 0)),
            (1.39, 1.39, [c.start for c in out_copies(j, 0, DH - TN)]),
        )
        for c in out_copies(j, DH - TN, DH):
            c.start()

    def phase_ffn(t):
        @pl.when(t < NT)
        def _():
            pace = _Pacer(t)
            _emit((0, 1, output_steps(pace, t, t % 2)),
                  (-0.108, 1.03, hn_steps(pace, 0, jnp.where(t == 1, 0, 1))),
                  (0.036, 0.983, permute_q_steps(pace, last(t + 1), range(0, T, GROUP))))

        pl.when(t > 0)(lambda: ffn(t - 1))
    _loop("phase_ffn", NT + 1, phase_ffn)
    for j in range(NT):
        for c in out_copies(j, 0, DH - TN) + out_copies(j, DH - TN, DH):
            c.wait()


@jax.jit
def pallas_sequential_preLN__sliding_local_dilated__glu_gated_geglu__prompt_kernel(
    A_x: jax.Array,
    A_wqkv: jax.Array,
    A_wo: jax.Array,
    B_x: jax.Array,
    B_w_gate: jax.Array,
    B_w_up: jax.Array,
    B_w_down: jax.Array,
):
    del B_x
    B, S, D = A_x.shape
    F = B_w_gate.shape[1]
    DH, FH = D // 2, F // 2
    NT = S // T
    NI = NT // 2
    assert B == 1 and D == 8 * LANES and NI * LANES == DH and FH % GR == 0 and 2 * GR == DH
    any_spec = pl.BlockSpec(memory_space=pl.ANY)
    out = pl.pallas_call(
        _kernel,
        in_specs=[any_spec] * 6,
        out_specs=any_spec,
        out_shape=jax.ShapeDtypeStruct((S, D), A_x.dtype),
        scratch_shapes=[
            pltpu.VMEM((S + T, D), BF16),
            pltpu.VMEM((NI, D // GR, GR, 2 * TN), BF16),
            pltpu.VMEM((2, D // GR, GR, D), BF16),
            pltpu.VMEM((D, D), BF16),
            pltpu.VMEM((T, D), F32),
            [pltpu.VMEM((n * 7 * DH // GR, GR // 2, DH), U32)
             for n in (1, 2, 1)],
            [(pltpu.VMEM((k // GR, GR, n), BF16),
              pltpu.VMEM((3, k // 2 // GR, GR, n // 2), BF16))
             for k, n in ((D, F), (D, F), (F, D))],
            pltpu.VMEM((7 * NT + 7, H // 2, DH), U32),
            pltpu.VMEM((2, 7, H // 2, DH), U32),
            pltpu.VMEM((2, 7, H // 2, DH), U32),
            pltpu.VMEM((WINDOW, T, LANES), F32),
            pltpu.VMEM((7, H // 2, FH), U32),
            pltpu.VMEM((NT, 8, T, LANES), F32),
            pltpu.VMEM((2, 8, T, LANES), F32),
            pltpu.VMEM((NT + 1, 8, HALO + T, LANES), F32),
            pltpu.VMEM((NT + 1, 8, HALO + T, LANES), F32),
            pltpu.VMEM((2, T, D), F32),
            pltpu.VMEM((S, D), BF16),
            pltpu.SemaphoreType.DMA((NT + 1,)),
            pltpu.SemaphoreType.DMA((NI,)),
            pltpu.SemaphoreType.DMA((NI - 1,)),
            pltpu.SemaphoreType.DMA(()),
            pltpu.SemaphoreType.DMA((NT,)),
            pltpu.SemaphoreType.DMA((NT,)),
        ],
        compiler_params=pltpu.CompilerParams(vmem_limit_bytes=124 * 2**20),
    )(A_x.reshape(S, D), A_wqkv.reshape(D // GR, GR, 3 * D), A_wo,
      B_w_gate.reshape(D // GR, GR, F), B_w_up.reshape(D // GR, GR, F),
      B_w_down.reshape(F // GR, GR, D))
    return out.reshape(B, S, D)
```

```python
import jax
import jax.numpy as jnp
from jax import lax
import jax.experimental.pallas as pl
import jax.experimental.pallas.tpu as pltpu

HEAD_DIM = 32
WINDOW = 8
DILATION = 2
HALO = 16
LANES = 128
T = 256
H = T // 2
SB = 8
RB = 16
TN = 128
PLAIN = (1, 4)
GR = 256
SCOPES = False
F32 = jnp.float32
BF16 = jnp.bfloat16
U32 = jnp.uint32


def _words(x):
    return pltpu.bitcast(x, U32)


def _halves(x):
    return pltpu.bitcast(x, BF16)


def _loop(name, n, body):
    def step(j, carry):
        if SCOPES:
            with jax.named_scope(name):
                body(j)
        else:
            body(j)
        return carry
    lax.fori_loop(0, n, step, 0)


def _emit(*stages):
    order = []
    for s, (lo, hi, steps) in enumerate(stages):
        order += [(lo + (hi - lo) * i / len(steps), s, i, f) for i, f in enumerate(steps)]
    for _, _, _, f in sorted(order, key=lambda t: t[:3]):
        f()


def _pipelined(pieces, depth):
    def step(t):
        for g in reversed(pieces[max(t - depth + 1, 0):t + 1]):
            next(g, None)
    return [lambda t=t: step(t) for t in range(len(pieces) + depth - 1)]


class _Pacer:
    def __init__(self, value=None):
        if value is None:
            self.never = None
        else:
            value = jnp.broadcast_to(value, (8, LANES))
            self.never = (value > 1) & (value < -1)
        self.products = []
        self.due = []

    def _tie(self, x, others):
        regs = [[x[r:r + 8, c:c + LANES] for c in range(0, x.shape[1], LANES)]
                for r in range(0, x.shape[0], 8)]
        for k, other in enumerate(others):
            row, col = k % len(regs), k // len(regs) % len(regs[0])
            if other.dtype != x.dtype:
                other = pltpu.bitcast(other, x.dtype)
            regs[row][col] = jnp.where(self.never, other[:8, :LANES], regs[row][col])
        return jnp.concatenate([jnp.concatenate(row, axis=1) for row in regs], axis=0)

    def start(self, x, lag=3):
        if self.never is None or len(self.products) < lag:
            return x
        return self._tie(x, [self.products[-lag]] * (x.shape[0] // 8))

    def finish(self, x):
        if self.never is not None:
            self.due.append(x)

    def dot(self, lhs_words, rhs):
        if self.due:
            lhs_words = self._tie(lhs_words, self.due)
            self.due = []
        self.products.append(jnp.dot(_halves(lhs_words), rhs, preferred_element_type=F32))
        return self.products[-1]


def _gelu(x):
    c = 0.7978845608028654
    hx = 0.5 * x
    return hx + hx * jnp.tanh(x * (c + (c * 0.044715) * (x * x)))


def _lhs7(a11, a12, a21, a22):
    return [t.astype(BF16) for t in
            (a11 + a22, a21 + a22, a11, a22, a11 + a12, a21 - a11, a12 - a22)]


def _rhs7(b11, b12, b21, b22):
    f11, f12, f21, f22 = (b.astype(F32) for b in (b11, b12, b21, b22))
    return [t.astype(BF16) for t in
            (f11 + f22, b11, f12 - f22, f21 - f11, b22, f11 + f12, f21 + f22)]


def _strassen(pace, lhs, rhs, done):
    c = {}

    def m(i):
        return pace.dot(lhs(i), rhs(i))

    def s0():
        c["m1"] = m(0)

    def s1():
        c["m2"] = m(1)
        c[22] = c["m1"] - c["m2"]

    def s2():
        t = m(3)
        c[21] = c["m2"] + t
        c[11] = c["m1"] + t

    def s3():
        c["m5"] = m(4)
        c[11] = c[11] - c["m5"]

    def s4():
        t = m(2)
        c[12] = c["m5"] + t
        c[22] = c[22] + t

    def s5():
        c[11] = c[11] + m(6)

    def s6():
        done(c[11], c[12], c[21], c[22] + m(5))

    return [s0, s1, s2, s3, s4, s5, s6]


def _matmul(pace, lhs, rhs, width, done):
    steps = []
    for n in range(0, width, TN):
        steps += _strassen(pace, lhs, lambda i, n=n: rhs(i, n), lambda *c, n=n: done(n, *c))
    return steps


def _permute_cols(chunks):
    blk = lax.broadcasted_iota(jnp.int32, chunks[0].shape, 1) // 4
    a = [pltpu.roll(chunks[c], 4 * c, 1) if c else chunks[c] for c in range(8)]
    yield
    e = [a[(-i) % 8] for i in range(8)]
    for s in (1, 2, 4):
        e = [jnp.where((blk & s) != 0, e[(i - s) % 8], e[i]) for i in range(8)]
    e = [pltpu.roll(e[c], LANES - 4 * c, 1) if c else e[c] for c in range(8)]
    yield
    return e


def _permuted_rows(ref, c, hl):
    parts = []
    for cp in range(8):
        r = c * 4
        u = _words(ref[pl.ds(cp * LANES + hl * 32 + r // 16 * 16, 16), :])
        parts.append(u[r % 16 // 2:r % 16 // 2 + 2, :])
    return _halves(jnp.concatenate(parts, axis=0))


def _kernel(x_hbm, wqkv_hbm, wo_hbm, wg_hbm, wu_hbm, wd_hbm, out_hbm,
            x_v, wq_raw, wkv_raw, wo_raw, centred, w_ops, ffn_w, a_ops, hn, attn, prob, act,
            q_raw, q_v, k_v, v_v, h_v, out_v,
            sem_x, sem_q, sem_kv, sem_o, sem_f, sem_out):
    S, D = x_hbm.shape
    DH = D // 2
    FH = wg_hbm.shape[2] // 2
    NT = S // T
    NI = NT // 2
    FR = GR // NT
    NG = 2 * GR // RB
    KG = -(-NG // (NI - 1))
    SKIP = KG * (NI - 1) - NG
    GROUP = H // NI
    PER = DH // GR
    WQ, WKV, WO = range(3)

    def ds(start, size):
        return pl.ds(start if isinstance(start, int) else pl.multiple_of(start, size), size)

    def last(j):
        return min(j, NT - 1) if isinstance(j, int) else jnp.minimum(j, NT - 1)

    def x_copy(j):
        return pltpu.make_async_copy(x_hbm.at[ds(last(j) * T, T)], x_v.at[ds(j * T, T)],
                                     sem_x.at[j])

    def wq_copy(n):
        return pltpu.make_async_copy(wqkv_hbm.at[:, :, ds(n * 2 * TN, 2 * TN)],
                                     wq_raw.at[n], sem_q.at[n])

    def wkv_copies(j):
        copies = []
        for m in range(2):
            lo = max((j * KG - SKIP) * RB - m * GR, 0)
            hi = min(((j + 1) * KG - SKIP) * RB - m * GR, GR)
            if lo < hi:
                copies.append(pltpu.make_async_copy(
                    wqkv_hbm.at[:, pl.ds(lo, hi - lo), pl.ds((1 + m) * D, D)],
                    wkv_raw.at[m, :, pl.ds(lo, hi - lo)], sem_kv.at[j]))
        return copies

    wo_copy = pltpu.make_async_copy(wo_hbm, wo_raw, sem_o)

    def ffn_copies(j):
        rows = ds(j * FR, FR)
        return [pltpu.make_async_copy(src.at[:, rows], dst.at[:, rows], sem_f.at[j])
                for src, (dst, _) in zip((wg_hbm, wu_hbm, wd_hbm), ffn_w)]

    def out_copies(j, lo, hi):
        return [pltpu.make_async_copy(out_v.at[ds(j * T, T), pl.ds(s * DH + lo, hi - lo)],
                                      out_hbm.at[ds(j * T, T), pl.ds(s * DH + lo, hi - lo)],
                                      sem_out.at[j]) for s in range(2)]

    def store_weight(m, i, g, row, col, t):
        w_ops[m][i * PER + g, ds(row // 2, t.shape[0] // 2), col] = _words(t)

    def weight(m, first=0):
        return lambda i, n: _halves(
            w_ops[m][pl.ds(first + i * PER, PER), :, ds(n, TN)].reshape(DH // 2, TN))

    def norm_steps(pace, load_rows, store):
        def piece(r):
            def load():
                return jnp.concatenate([load_rows(s * H + r).astype(F32) for s in range(2)], axis=0)
            m = jnp.mean(pace.start(load()), axis=-1, keepdims=True)
            yield
            c = load() - m
            centred[ds(2 * r, 2 * RB), :] = c
            scale = lax.rsqrt(jnp.mean(c * c, axis=-1, keepdims=True) + 1e-5)
            yield
            y = centred[ds(2 * r, 2 * RB), :] * scale
            for i, t in enumerate(_lhs7(y[:RB, :DH], y[:RB, DH:], y[RB:, :DH], y[RB:, DH:])):
                store(i, ds(r // 2, RB // 2), _words(t))
                pace.finish(_words(t)[:, i % 4 * LANES:(i % 4 + 1) * LANES])
        return _pipelined([piece(r) for r in range(0, H, RB)], 3)

    def xn_steps(pace, j, copy):
        def store(i, where, t):
            a_ops[7 * j + i, where, :] = t
            copy[i, where, :] = t
        return norm_steps(pace, lambda r: x_v[ds(j * T + r, RB), :], store)

    def hn_steps(pace, slot, dest):
        def store(i, rows, t):
            hn[dest, i, rows, :] = t
        return norm_steps(pace, lambda r: h_v[slot, pl.ds(r, RB), :], store)

    def q_weight_steps(pace, n):
        def step(g, r):
            top, bot = (wq_raw[n, kh * PER + g, pl.ds(r, 2 * RB), :] for kh in range(2))
            b11 = pace.start(top[:, :TN].astype(F32))
            for i, t in enumerate(_rhs7(b11, top[:, TN:], bot[:, :TN], bot[:, TN:])):
                store_weight(WQ, i, g, r, ds(n * TN, TN), t)
                pace.finish(_words(t)[i % 2 * 8:])
        return [lambda g=g, r=r: step(g, r) for g in range(PER) for r in range(0, GR, 2 * RB)]

    def kv_weight_steps(pace, j):
        def piece(g, group):
            m, row = group // (NG // 2), group % (NG // 2) * RB
            u = [jnp.concatenate(
                [_words(wkv_raw[m, kh * PER + g, ds(row, RB), pl.ds(c * LANES, LANES)])
                 for kh in range(2)], axis=0) for c in range(8)]
            u = yield from _permute_cols(u[:1] + [pace.start(u[1])] + u[2:])
            for c in range(4):
                b = [_halves(u[nh * 4 + c][kh * RB // 2:(kh + 1) * RB // 2])
                     for kh in range(2) for nh in range(2)]
                for i, t in enumerate(_rhs7(*b)):
                    store_weight(WKV, i, m * 7 * PER + g, row, pl.ds(c * LANES, LANES), t)
                    if i >= 5:
                        pace.finish(_words(t))
        return _pipelined([piece(g, jnp.maximum(j * KG - SKIP + r, 0)) for r in range(KG)
                           for g in range(PER)], 3)

    def ffn_index(w, i, g, rows, n, width):
        blocks, extra = w
        _, per, _, half = extra.shape
        if 1 <= i <= 4:
            g = pl.ds((i - 1) // 2 * per, per) if g is None else (i - 1) // 2 * per + g
            return blocks, (g, rows, pl.ds((i - 1) % 2 * half + n, width))
        return extra, (i % 4, slice(None) if g is None else g, rows, pl.ds(n, width))

    def ffn_weight_steps(pace, j):
        def step(w, g, n):
            where = [ffn_index(w, i, g, slice(None), n, 2 * LANES) for i in range(7)]
            blocks = [ref[idx] for ref, idx in where[1:5]]
            blocks[0] = pace.start(blocks[0].astype(F32), 3)
            pace.finish(blocks[0])
            for i, t in enumerate(_rhs7(*blocks)):
                if i not in PLAIN:
                    ref, idx = where[i]
                    ref[idx] = t
        chunk = [(blocks.at[:, ds(j * FR, FR)], extra.at[:, :, ds(j * FR, FR)])
                 for blocks, extra in ffn_w]
        steps = [[lambda w=w, g=g, n=n: step(w, g, n) for g in range(w[1].shape[1])
                  for n in range(0, w[1].shape[3], 2 * LANES)] for w in chunk]
        return [f for group in zip(*steps) for f in group]

    def ffn_weight(w):
        def load(i, n):
            ref, idx = ffn_index(w, i, None, slice(None), n, TN)
            return ref[idx].reshape(w[1].shape[1] * GR, TN)
        return load

    def permute_q_steps(pace, j, rows):
        def piece(r):
            q = [q_raw[j, c, ds(r, GROUP), :] for c in range(8)]
            q = yield from _permute_cols(q[:1] + [pace.start(q[1])] + q[2:])
            for c in range(8):
                q_v[j % 2, c, ds(r, GROUP), :] = q[c]
                pace.finish(q[c][c * 8 % GROUP:])
        return _pipelined([piece(r) for r in rows], 3)

    def q_step(pace, j, lhs, n):
        def done(*c):
            for b, t in enumerate(c):
                q_raw[j, 2 * n + b % 2, pl.ds(b // 2 * H, H), :] = t
        return _strassen(pace, lambda i: lhs[i], lambda i: weight(WQ)(i, n * TN), done)

    def project(pace, j, rhs, dst):
        lhs, dst = a_ops.at[pl.ds(7 * j, 7)], dst.at[pl.ds(j, 2)]

        def done(n, *c):
            for b, t in enumerate(c):
                chunk = (b % 2 * DH + n) // LANES
                dst[0, chunk, pl.ds(HALO + b // 2 * H, H), :] = t
                if b // 2:
                    dst[1, chunk, pl.ds(0, HALO), :] = t[H - HALO:]
        return _matmul(pace, lambda i: lhs[i], rhs, DH, done)

    def softmax_steps(pace, q, k, out, rows, first=None):
        def piece(r):
            logits = [None] * WINDOW
            for c in range(8):
                qc = q[c, pl.ds(r, SB), :]
                if c == 0:
                    qc = pace.start(qc)
                for w in range(WINDOW):
                    t = qc * k[c, pl.ds(HALO + r - DILATION * w, SB), :]
                    logits[w] = t if c == 0 else logits[w] + t
            lane = lax.broadcasted_iota(jnp.int32, (SB, LANES), 1)
            for s in (1, 2):
                rolled = [(pltpu.roll(l, s, 1), pltpu.roll(l, LANES - s, 1)) for l in logits]
                yield
                logits = [l + jnp.where((lane & s) != 0, a, b)
                          for l, (a, b) in zip(logits, rolled)]
            for w in range(WINDOW):
                l = logits[w] * (HEAD_DIM ** -0.5)
                if first is not None and r < DILATION * w:
                    pos = first + r + lax.broadcasted_iota(jnp.int32, (SB, LANES), 0)
                    l = jnp.where(pos >= DILATION * w, l, -1e9)
                logits[w] = l
            m = logits[0]
            for w in range(1, WINDOW):
                m = jnp.maximum(m, logits[w])
            e = [jnp.exp(l - m) for l in logits]
            total = e[0]
            for w in range(1, WINDOW):
                total = total + e[w]
            inv = 1.0 / total
            for w in range(WINDOW):
                p = e[w] * inv
                out[w, pl.ds(r, SB), :] = p
                pace.finish(p)
        return _pipelined([piece(r) for r in rows], 3)

    def value_steps(pace, weights, v, out, rows):
        def piece(r, c):
            blocks = []
            for row in (r, H + r):
                for chunk in (c, c + 4):
                    for w in range(WINDOW):
                        p = weights[w, pl.ds(row, RB), :]
                        t = (pace.start(p, 6) if w == 0 else p) * v[
                            chunk, pl.ds(HALO + row - DILATION * w, RB), :]
                        o = t if w == 0 else o + t
                    blocks.append(o)
                    pace.finish(o)
                    pace.finish(o[8:])
                    yield
            for i, t in enumerate(_lhs7(*blocks)):
                out[i, pl.ds(r // 2, RB // 2), pl.ds(c * LANES, LANES)] = _words(t)
                pace.finish(_words(t))
        pieces = [piece(r, c) for r in rows for c in range(4)]
        return [lambda g=g: next(g, None) for g in pieces for _ in range(5)]

    def output_steps(pace, j, slot):
        def done(n, *c):
            for b, t in enumerate(c):
                cols = pl.ds(b % 2 * DH + n, TN)
                h_v[slot, pl.ds(b // 2 * H, H), cols] = (
                    x_v[ds(j * T + b // 2 * H, H), cols].astype(F32) + t)
        return _matmul(pace, lambda i: attn[slot, i], weight(WO), DH, done)

    def start(*copies):
        for c in copies:
            c.start()

    start(x_copy(0), wq_copy(0), x_copy(1))
    def clear(c):
        prob[c, pl.ds(0, H + GROUP), :] = jnp.zeros((H + GROUP, LANES), F32)
        v_v[0, c, pl.ds(0, HALO + H + GROUP), :] = jnp.zeros((HALO + H + GROUP, LANES), F32)
        k_v[0, c, pl.ds(0, HALO), :] = jnp.zeros((HALO, LANES), F32)
        h_v[0, ds(c * (T // 8), T // 8), :] = jnp.zeros((T // 8, D), F32)
    _loop("clear", 8, clear)
    x_copy(0).wait()
    start(wq_copy(1))
    _emit((0, 1, xn_steps(_Pacer(), 0, hn.at[0])))
    wq_copy(0).wait()
    start(wq_copy(2))
    _emit((0, 1, q_weight_steps(_Pacer(), 0)))

    def first_q(pace, n, tiles=(0, 1)):
        return [f for t in tiles for f in q_step(pace, t, (hn.at[0], attn.at[0])[t], n)]

    def wkv_batch(j):
        return [x_copy(2 * j + 3), x_copy(2 * j + 4)] + wkv_copies(j)

    x_copy(1).wait()
    start(wq_copy(3))
    pace = _Pacer(x_v[pl.ds(0, 8), pl.ds(0, LANES)].astype(F32))
    _emit((0, 1, first_q(pace, 0, [0])), (0, 1.2, xn_steps(pace, 1, attn.at[0])))
    start(x_copy(2))
    wq_copy(1).wait()
    start(*wkv_copies(0))
    pace = _Pacer(x_v[pl.ds(0, 8), pl.ds(0, LANES)].astype(F32))
    _emit((0, 1, first_q(pace, 0, [1])), (0.118, 0.9, q_weight_steps(pace, 1)))
    wq_copy(2).wait()
    start(x_copy(3), x_copy(4))
    pace = _Pacer(x_v[pl.ds(0, 8), pl.ds(0, LANES)].astype(F32))
    _emit((0, 1, first_q(pace, 1)), (0.05, 0.9, q_weight_steps(pace, 2)))
    wq_copy(3).wait()
    x_copy(2).wait()
    pace = _Pacer(x_v[pl.ds(0, 8), pl.ds(0, LANES)].astype(F32))
    _emit((0, 1, first_q(pace, 2)), (1, 2, first_q(pace, 3)),
          (0.05, 0.9, q_weight_steps(pace, 3)), (0.167, 1.943, xn_steps(pace, 2, attn.at[1])))
    following = [wkv_batch(1) + wkv_batch(2), [wo_copy] + ffn_copies(0), ffn_copies(1)]

    def phase_q(j):
        t = 2 * j + 2
        x_copy(t + 1).wait()
        x_copy(t + 2).wait()
        for k in range(NI - 1):
            @pl.when(j == k)
            def _():
                for c in wkv_copies(k):
                    c.wait()
                start(*following[k])
        pace = _Pacer(j)
        _emit(
            (0, 1, [f for n in range(NI) for f in q_step(pace, t, attn.at[1], n)]),
            (1, 2, [f for n in range(NI) for f in q_step(pace, t + 1, hn.at[0], n)]),
            (-0.131, 0.969, xn_steps(pace, t + 1, hn.at[0])),
            (0.82, 1.964, xn_steps(pace, t + 2, attn.at[1])),
            (0, 1.995, kv_weight_steps(pace, j)),
        )
    _loop("phase_q", NI - 1, phase_q)
    wo_copy.wait()

    def first_values(pace, g):
        for c in range(8):
            v_v[0, c, pl.ds(0, HALO), :] = jnp.broadcast_to(
                v_v[0, c, pl.ds(HALO, 1), :], (HALO, LANES))
        tile, row = g // NI, ds(g % NI * GROUP, GROUP).start
        return value_steps(pace, prob.at[:, pl.ds(row, H + GROUP)],
                           v_v.at[tile, :, pl.ds(row, HALO + H + GROUP)],
                           attn.at[tile, :, ds(row // 2, GROUP // 2)], range(0, GROUP, RB))

    def phase_kv(j):
        for c in ffn_copies(j):
            c.wait()
        pl.when(j + 2 < NT)(lambda: start(*ffn_copies(j + 2)))

        wo_src = [wo_raw.at[pl.ds(pl.multiple_of(j // NI * 64, 64), D - 64),
                            ds(s * DH + j % NI * LANES, LANES)] for s in range(2)]
        wo_dst = w_ops[WO].at[:, pl.ds(pl.multiple_of(j // NI * 32, 32), GR // 2 - 32),
                              ds(j % NI * LANES, LANES)]

        def wo_step(c, hl):
            b = [_permuted_rows(wo_src[s], kh * 4 + c, hl) for kh in range(2) for s in range(2)]
            b[0] = pace.start(b[0].astype(F32))
            for i, t in enumerate(_rhs7(*b)):
                wo_dst[i * PER + c * LANES // GR,
                       pl.ds((c * LANES % GR + hl * 32) // 2, 16), :] = _words(t)
                pace.finish(_words(t)[i % 2 * 8:])

        pace = _Pacer(j)
        tile, row = j // NI, pl.multiple_of(j % NI * GROUP, GROUP)
        _emit(
            (0, 1, project(pace, j, weight(WKV), k_v)),
            (1, 2, project(pace, j, weight(WKV, 7 * PER), v_v)),
            (0.107, 1.883, ffn_weight_steps(pace, j)),
            (0.447, 1.05, permute_q_steps(pace, tile, [row, H + row])),
            (0.1, 0.6, [lambda c=c, hl=hl: wo_step(c, hl)
                         for c in range(4) for hl in range(2)]),
            (0.155, 1.035, first_values(pace, jnp.maximum(j - 1, 0))),
            (1.042, 2.043, softmax_steps(
                pace, q_v.at[tile, :, pl.ds(row, H + GROUP)],
                k_v.at[tile, :, pl.ds(row, HALO + H + GROUP)], prob.at[:, pl.ds(row, H + GROUP)],
                [s * H + r for s in range(2) for r in range(0, GROUP, SB)], tile * T + row)),
        )
    _loop("phase_kv", NT, phase_kv)
    _emit((0, 1, first_values(_Pacer(), NT - 1)))

    def ffn(j):
        nxt = last(j + 2)
        slot = j % 2
        pace = _Pacer(j)
        gate = {}

        def gate_done(n, *c):
            gate[n] = [_gelu(t) for t in c]

        def up_done(n, *c):
            for i, t in enumerate(_lhs7(*[g * u for g, u in zip(gate.pop(n), c)])):
                act[i, :, n:n + TN] = _words(t)

        def down_done(n, *c):
            for b, t in enumerate(c):
                cols = pl.ds(b % 2 * DH + n, TN)
                out_v[ds(j * T + b // 2 * H, H), cols] = (
                    h_v[slot, pl.ds(b // 2 * H, H), cols] + t).astype(BF16)

        g = _matmul(pace, lambda i: hn[0, i], ffn_weight(ffn_w[0]), FH, gate_done)
        u = _matmul(pace, lambda i: hn[0, i], ffn_weight(ffn_w[1]), FH, up_done)
        gu = [f for n in range(0, len(g), 7) for f in g[n:n + 7] + u[n:n + 7]]
        _emit(
            (0, 1, gu),
            (1, 1.5, _matmul(pace, lambda i: act[i], ffn_weight(ffn_w[2]), DH, down_done)),
            (0.012, 0.62, softmax_steps(pace, q_v.at[nxt % 2], k_v.at[nxt], prob, range(0, T, SB))),
            (0.592, 0.99, value_steps(pace, prob, v_v.at[nxt], attn.at[slot], range(0, H, RB))),
            (1.014, 1.351, hn_steps(pace, 1 - slot, 0)),
            (1.39, 1.39, [c.start for c in out_copies(j, 0, DH - TN)]),
        )
        for c in out_copies(j, DH - TN, DH):
            c.start()

    def phase_ffn(t):
        @pl.when(t < NT)
        def _():
            pace = _Pacer(t)
            _emit((0, 1, output_steps(pace, t, t % 2)),
                  (-0.108, 1.029, hn_steps(pace, 0, jnp.where(t == 1, 0, 1))),
                  (0.045, 1.046, permute_q_steps(pace, last(t + 1), range(0, T, GROUP))))

        pl.when(t > 0)(lambda: ffn(t - 1))
    _loop("phase_ffn", NT + 1, phase_ffn)
    for j in range(NT):
        for c in out_copies(j, 0, DH - TN) + out_copies(j, DH - TN, DH):
            c.wait()


@jax.jit
def pallas_sequential_preLN__sliding_local_dilated__glu_gated_geglu__prompt_kernel(
    A_x: jax.Array,
    A_wqkv: jax.Array,
    A_wo: jax.Array,
    B_x: jax.Array,
    B_w_gate: jax.Array,
    B_w_up: jax.Array,
    B_w_down: jax.Array,
):
    del B_x
    B, S, D = A_x.shape
    F = B_w_gate.shape[1]
    DH, FH = D // 2, F // 2
    NT = S // T
    NI = NT // 2
    assert B == 1 and D == 8 * LANES and NI == 4 and NI * TN == DH and FH % GR == 0 and 2 * GR == DH
    any_spec = pl.BlockSpec(memory_space=pl.ANY)
    out = pl.pallas_call(
        _kernel,
        in_specs=[any_spec] * 6,
        out_specs=any_spec,
        out_shape=jax.ShapeDtypeStruct((S, D), A_x.dtype),
        scratch_shapes=[
            pltpu.VMEM((S + T, D), BF16),
            pltpu.VMEM((NI, D // GR, GR, 2 * TN), BF16),
            pltpu.VMEM((2, D // GR, GR, D), BF16),
            pltpu.VMEM((D, D), BF16),
            pltpu.VMEM((T, D), F32),
            [pltpu.VMEM((n * 7 * DH // GR, GR // 2, DH), U32)
             for n in (1, 2, 1)],
            [(pltpu.VMEM((k // GR, GR, n), BF16),
              pltpu.VMEM((3, k // 2 // GR, GR, n // 2), BF16))
             for k, n in ((D, F), (D, F), (F, D))],
            pltpu.VMEM((7 * NT + 7, H // 2, DH), U32),
            pltpu.VMEM((2, 7, H // 2, DH), U32),
            pltpu.VMEM((2, 7, H // 2, DH), U32),
            pltpu.VMEM((WINDOW, T, LANES), F32),
            pltpu.VMEM((7, H // 2, FH), U32),
            pltpu.VMEM((NT, 8, T, LANES), F32),
            pltpu.VMEM((2, 8, T, LANES), F32),
            pltpu.VMEM((NT + 1, 8, HALO + T, LANES), F32),
            pltpu.VMEM((NT + 1, 8, HALO + T, LANES), F32),
            pltpu.VMEM((2, T, D), F32),
            pltpu.VMEM((S, D), BF16),
            pltpu.SemaphoreType.DMA((NT + 1,)),
            pltpu.SemaphoreType.DMA((NI,)),
            pltpu.SemaphoreType.DMA((NI - 1,)),
            pltpu.SemaphoreType.DMA(()),
            pltpu.SemaphoreType.DMA((NT,)),
            pltpu.SemaphoreType.DMA((NT,)),
        ],
        compiler_params=pltpu.CompilerParams(vmem_limit_bytes=124 * 2**20),
    )(A_x.reshape(S, D), A_wqkv.reshape(D // GR, GR, 3 * D), A_wo,
      B_w_gate.reshape(D // GR, GR, F), B_w_up.reshape(D // GR, GR, F),
      B_w_down.reshape(F // GR, GR, D))
    return out.reshape(B, S, D)
```

```python
import jax
import jax.numpy as jnp
from jax import lax
import jax.experimental.pallas as pl
import jax.experimental.pallas.tpu as pltpu

HEAD_DIM = 32
WINDOW = 8
DILATION = 2
HALO = 16
LANES = 128
T = 256
H = T // 2
SB = 8
RB = 16
TN = 128
PLAIN = (1, 4)
GR = 256
SCOPES = False
F32 = jnp.float32
BF16 = jnp.bfloat16
U32 = jnp.uint32


def _words(x):
    return pltpu.bitcast(x, U32)


def _halves(x):
    return pltpu.bitcast(x, BF16)


def _loop(name, n, body):
    def step(j, carry):
        if SCOPES:
            with jax.named_scope(name):
                body(j)
        else:
            body(j)
        return carry
    lax.fori_loop(0, n, step, 0)


def _emit(*stages):
    order = []
    for s, (lo, hi, steps) in enumerate(stages):
        order += [(lo + (hi - lo) * i / len(steps), s, i, f) for i, f in enumerate(steps)]
    for _, _, _, f in sorted(order, key=lambda t: t[:3]):
        f()


def _pipelined(pieces, depth):
    def step(t):
        for g in reversed(pieces[max(t - depth + 1, 0):t + 1]):
            next(g, None)
    return [lambda t=t: step(t) for t in range(len(pieces) + depth - 1)]


class _Pacer:
    def __init__(self, value=None):
        if value is None:
            self.never = None
        else:
            value = jnp.broadcast_to(value, (8, LANES))
            self.never = (value > 1) & (value < -1)
        self.products = []
        self.due = []

    def _tie(self, x, others):
        regs = [[x[r:r + 8, c:c + LANES] for c in range(0, x.shape[1], LANES)]
                for r in range(0, x.shape[0], 8)]
        for k, other in enumerate(others):
            row, col = k % len(regs), k // len(regs) % len(regs[0])
            if other.dtype != x.dtype:
                other = pltpu.bitcast(other, x.dtype)
            regs[row][col] = jnp.where(self.never, other[:8, :LANES], regs[row][col])
        return jnp.concatenate([jnp.concatenate(row, axis=1) for row in regs], axis=0)

    def start(self, x, lag=3):
        if self.never is None or len(self.products) < lag:
            return x
        return self._tie(x, [self.products[-lag]] * (x.shape[0] // 8))

    def finish(self, x):
        if self.never is not None:
            self.due.append(x)

    def dot(self, lhs_words, rhs):
        if self.due:
            lhs_words = self._tie(lhs_words, self.due)
            self.due = []
        self.products.append(jnp.dot(_halves(lhs_words), rhs, preferred_element_type=F32))
        return self.products[-1]


def _gelu(x):
    c = 0.7978845608028654
    hx = 0.5 * x
    return hx + hx * jnp.tanh(x * (c + (c * 0.044715) * (x * x)))


def _lhs7(a11, a12, a21, a22):
    return [t.astype(BF16) for t in
            (a11 + a22, a21 + a22, a11, a22, a11 + a12, a21 - a11, a12 - a22)]


def _rhs7(b11, b12, b21, b22):
    f11, f12, f21, f22 = (b.astype(F32) for b in (b11, b12, b21, b22))
    return [t.astype(BF16) for t in
            (f11 + f22, b11, f12 - f22, f21 - f11, b22, f11 + f12, f21 + f22)]


def _strassen(pace, lhs, rhs, done):
    c = {}

    def m(i):
        return pace.dot(lhs(i), rhs(i))

    def s0():
        c["m1"] = m(0)

    def s1():
        c["m2"] = m(1)
        c[22] = c["m1"] - c["m2"]

    def s2():
        t = m(3)
        c[21] = c["m2"] + t
        c[11] = c["m1"] + t

    def s3():
        c["m5"] = m(4)
        c[11] = c[11] - c["m5"]

    def s4():
        t = m(2)
        c[12] = c["m5"] + t
        c[22] = c[22] + t

    def s5():
        c[11] = c[11] + m(6)

    def s6():
        done(c[11], c[12], c[21], c[22] + m(5))

    return [s0, s1, s2, s3, s4, s5, s6]


def _matmul(pace, lhs, rhs, width, done):
    steps = []
    for n in range(0, width, TN):
        steps += _strassen(pace, lhs, lambda i, n=n: rhs(i, n), lambda *c, n=n: done(n, *c))
    return steps


def _permute_cols(chunks):
    blk = lax.broadcasted_iota(jnp.int32, chunks[0].shape, 1) // 4
    a = [pltpu.roll(chunks[c], 4 * c, 1) if c else chunks[c] for c in range(8)]
    yield
    e = [a[(-i) % 8] for i in range(8)]
    for s in (1, 2, 4):
        e = [jnp.where((blk & s) != 0, e[(i - s) % 8], e[i]) for i in range(8)]
    e = [pltpu.roll(e[c], LANES - 4 * c, 1) if c else e[c] for c in range(8)]
    yield
    return e


def _transpose_row_groups(u):
    return [jnp.concatenate([t[2 * c:2 * c + 2] for t in u], axis=0) for c in range(4)]


def _kernel(x_hbm, wqkv_hbm, wo_hbm, wg_hbm, wu_hbm, wd_hbm, out_hbm,
            x_v, wq_raw, wkv_raw, wo_raw, centred, w_ops, ffn_w, a_ops, hn, attn, prob, act,
            q_raw, q_v, k_v, v_v, h_v, out_v,
            sem_x, sem_q, sem_kv, sem_o, sem_f, sem_out):
    S, D = x_hbm.shape
    DH = D // 2
    FH = wg_hbm.shape[2] // 2
    NT = S // T
    NI = NT // 2
    FR = GR // NT
    NG = 2 * GR // RB
    KG = -(-NG // (NI - 1))
    SKIP = KG * (NI - 1) - NG
    GROUP = H // NI
    PER = DH // GR
    WQ, WKV, WO = range(3)

    def ds(start, size):
        return pl.ds(start if isinstance(start, int) else pl.multiple_of(start, size), size)

    def last(j):
        return min(j, NT - 1) if isinstance(j, int) else jnp.minimum(j, NT - 1)

    def x_copy(j):
        return pltpu.make_async_copy(x_hbm.at[ds(last(j) * T, T)], x_v.at[ds(j * T, T)],
                                     sem_x.at[j])

    def wq_copy(n):
        return pltpu.make_async_copy(wqkv_hbm.at[:, :, ds(n * 2 * TN, 2 * TN)],
                                     wq_raw.at[n], sem_q.at[n])

    def wkv_copies(j):
        copies = []
        for m in range(2):
            lo = max((j * KG - SKIP) * RB - m * GR, 0)
            hi = min(((j + 1) * KG - SKIP) * RB - m * GR, GR)
            if lo < hi:
                copies.append(pltpu.make_async_copy(
                    wqkv_hbm.at[:, pl.ds(lo, hi - lo), pl.ds((1 + m) * D, D)],
                    wkv_raw.at[m, :, pl.ds(lo, hi - lo)], sem_kv.at[j]))
        return copies

    wo_copy = pltpu.make_async_copy(wo_hbm, wo_raw, sem_o)

    def ffn_copies(j):
        rows = ds(j * FR, FR)
        return [pltpu.make_async_copy(src.at[:, rows], dst.at[:, rows], sem_f.at[j])
                for src, (dst, _) in zip((wg_hbm, wu_hbm, wd_hbm), ffn_w)]

    def out_copies(j, lo, hi):
        return [pltpu.make_async_copy(out_v.at[ds(j * T, T), pl.ds(s * DH + lo, hi - lo)],
                                      out_hbm.at[ds(j * T, T), pl.ds(s * DH + lo, hi - lo)],
                                      sem_out.at[j]) for s in range(2)]

    def store_weight(m, i, g, row, col, t):
        w_ops[m][i * PER + g, ds(row // 2, t.shape[0] // 2), col] = _words(t)

    def weight(m, first=0):
        return lambda i, n: _halves(
            w_ops[m][pl.ds(first + i * PER, PER), :, ds(n, TN)].reshape(DH // 2, TN))

    def norm_steps(pace, load_rows, store):
        def piece(r):
            def load():
                return jnp.concatenate([load_rows(s * H + r).astype(F32) for s in range(2)], axis=0)
            m = jnp.mean(pace.start(load()), axis=-1, keepdims=True)
            yield
            c = load() - m
            centred[ds(2 * r, 2 * RB), :] = c
            scale = lax.rsqrt(jnp.mean(c * c, axis=-1, keepdims=True) + 1e-5)
            yield
            y = centred[ds(2 * r, 2 * RB), :] * scale
            for i, t in enumerate(_lhs7(y[:RB, :DH], y[:RB, DH:], y[RB:, :DH], y[RB:, DH:])):
                store(i, ds(r // 2, RB // 2), _words(t))
                pace.finish(_words(t)[:, i % 4 * LANES:(i % 4 + 1) * LANES])
        return _pipelined([piece(r) for r in range(0, H, RB)], 3)

    def xn_steps(pace, j, copy):
        def store(i, where, t):
            a_ops[7 * j + i, where, :] = t
            copy[i, where, :] = t
        return norm_steps(pace, lambda r: x_v[ds(j * T + r, RB), :], store)

    def hn_steps(pace, slot, dest):
        def store(i, rows, t):
            hn[dest, i, rows, :] = t
        return norm_steps(pace, lambda r: h_v[slot, pl.ds(r, RB), :], store)

    def q_weight_steps(pace, n):
        def step(g, r):
            top, bot = (wq_raw[n, kh * PER + g, pl.ds(r, 2 * RB), :] for kh in range(2))
            b11 = pace.start(top[:, :TN].astype(F32))
            for i, t in enumerate(_rhs7(b11, top[:, TN:], bot[:, :TN], bot[:, TN:])):
                store_weight(WQ, i, g, r, ds(n * TN, TN), t)
                pace.finish(_words(t)[i % 2 * 8:])
        return [lambda g=g, r=r: step(g, r) for g in range(PER) for r in range(0, GR, 2 * RB)]

    def kv_weight_steps(pace, j):
        def piece(g, group):
            m, row = group // (NG // 2), group % (NG // 2) * RB
            u = [jnp.concatenate(
                [_words(wkv_raw[m, kh * PER + g, ds(row, RB), pl.ds(c * LANES, LANES)])
                 for kh in range(2)], axis=0) for c in range(8)]
            u = yield from _permute_cols(u[:1] + [pace.start(u[1])] + u[2:])
            for c in range(4):
                b = [_halves(u[nh * 4 + c][kh * RB // 2:(kh + 1) * RB // 2])
                     for kh in range(2) for nh in range(2)]
                for i, t in enumerate(_rhs7(*b)):
                    store_weight(WKV, i, m * 7 * PER + g, row, pl.ds(c * LANES, LANES), t)
                    if i >= 5:
                        pace.finish(_words(t))
        return _pipelined([piece(g, jnp.maximum(j * KG - SKIP + r, 0)) for r in range(KG)
                           for g in range(PER)], 3)

    def ffn_index(w, i, g, rows, n, width):
        blocks, extra = w
        _, per, _, half = extra.shape
        if 1 <= i <= 4:
            g = pl.ds((i - 1) // 2 * per, per) if g is None else (i - 1) // 2 * per + g
            return blocks, (g, rows, pl.ds((i - 1) % 2 * half + n, width))
        return extra, (i % 4, slice(None) if g is None else g, rows, pl.ds(n, width))

    def ffn_weight_steps(pace, j):
        def step(w, g, n):
            where = [ffn_index(w, i, g, slice(None), n, 2 * LANES) for i in range(7)]
            blocks = [ref[idx] for ref, idx in where[1:5]]
            blocks[0] = pace.start(blocks[0].astype(F32), 3)
            pace.finish(blocks[0])
            for i, t in enumerate(_rhs7(*blocks)):
                if i not in PLAIN:
                    ref, idx = where[i]
                    ref[idx] = t
        chunk = [(blocks.at[:, ds(j * FR, FR)], extra.at[:, :, ds(j * FR, FR)])
                 for blocks, extra in ffn_w]
        steps = [[lambda w=w, g=g, n=n: step(w, g, n) for g in range(w[1].shape[1])
                  for n in range(0, w[1].shape[3], 2 * LANES)] for w in chunk]
        return [f for group in zip(*steps) for f in group]

    def ffn_weight(w):
        def load(i, n):
            ref, idx = ffn_index(w, i, None, slice(None), n, TN)
            return ref[idx].reshape(w[1].shape[1] * GR, TN)
        return load

    def permute_q_steps(pace, j, rows):
        def piece(r):
            q = [q_raw[j, c, ds(r, GROUP), :] for c in range(8)]
            q = yield from _permute_cols(q[:1] + [pace.start(q[1])] + q[2:])
            for c in range(8):
                q_v[j % 2, c, ds(r, GROUP), :] = q[c]
                pace.finish(q[c][c * 8 % GROUP:])
        return _pipelined([piece(r) for r in rows], 3)

    def q_step(pace, j, lhs, n):
        def done(*c):
            for b, t in enumerate(c):
                q_raw[j, 2 * n + b % 2, pl.ds(b // 2 * H, H), :] = t
        return _strassen(pace, lambda i: lhs[i], lambda i: weight(WQ)(i, n * TN), done)

    def project(pace, j, rhs, dst):
        lhs, dst = a_ops.at[pl.ds(7 * j, 7)], dst.at[pl.ds(j, 2)]

        def done(n, *c):
            for b, t in enumerate(c):
                chunk = (b % 2 * DH + n) // LANES
                dst[0, chunk, pl.ds(HALO + b // 2 * H, H), :] = t
                if b // 2:
                    dst[1, chunk, pl.ds(0, HALO), :] = t[H - HALO:]
        return _matmul(pace, lambda i: lhs[i], rhs, DH, done)

    def softmax_steps(pace, q, k, out, rows, first=None):
        def piece(r):
            logits = [None] * WINDOW
            for c in range(8):
                qc = q[c, pl.ds(r, SB), :]
                if c == 0:
                    qc = pace.start(qc)
                for w in range(WINDOW):
                    t = qc * k[c, pl.ds(HALO + r - DILATION * w, SB), :]
                    logits[w] = t if c == 0 else logits[w] + t
            lane = lax.broadcasted_iota(jnp.int32, (SB, LANES), 1)
            for s in (1, 2):
                rolled = [(pltpu.roll(l, s, 1), pltpu.roll(l, LANES - s, 1)) for l in logits]
                yield
                logits = [l + jnp.where((lane & s) != 0, a, b)
                          for l, (a, b) in zip(logits, rolled)]
            for w in range(WINDOW):
                l = logits[w] * (HEAD_DIM ** -0.5)
                if first is not None and r < DILATION * w:
                    pos = first + r + lax.broadcasted_iota(jnp.int32, (SB, LANES), 0)
                    l = jnp.where(pos >= DILATION * w, l, -1e9)
                logits[w] = l
            m = logits[0]
            for w in range(1, WINDOW):
                m = jnp.maximum(m, logits[w])
            e = [jnp.exp(l - m) for l in logits]
            total = e[0]
            for w in range(1, WINDOW):
                total = total + e[w]
            inv = 1.0 / total
            for w in range(WINDOW):
                p = e[w] * inv
                out[w, pl.ds(r, SB), :] = p
                pace.finish(p)
        return _pipelined([piece(r) for r in rows], 3)

    def value_steps(pace, weights, v, out, rows):
        def piece(r, c):
            blocks = []
            for row in (r, H + r):
                for chunk in (c, c + 4):
                    for w in range(WINDOW):
                        p = weights[w, pl.ds(row, RB), :]
                        t = (pace.start(p, 6) if w == 0 else p) * v[
                            chunk, pl.ds(HALO + row - DILATION * w, RB), :]
                        o = t if w == 0 else o + t
                    blocks.append(o)
                    pace.finish(o)
                    pace.finish(o[8:])
                    yield
            for i, t in enumerate(_lhs7(*blocks)):
                out[i, pl.ds(r // 2, RB // 2), pl.ds(c * LANES, LANES)] = _words(t)
                pace.finish(_words(t))
        pieces = [piece(r, c) for r in rows for c in range(4)]
        return [lambda g=g: next(g, None) for g in pieces for _ in range(5)]

    def output_steps(pace, j, slot):
        def done(n, *c):
            for b, t in enumerate(c):
                cols = pl.ds(b % 2 * DH + n, TN)
                h_v[slot, pl.ds(b // 2 * H, H), cols] = (
                    x_v[ds(j * T + b // 2 * H, H), cols].astype(F32) + t)
        return _matmul(pace, lambda i: attn[slot, i], weight(WO), DH, done)

    def start(*copies):
        for c in copies:
            c.start()

    start(x_copy(0), wq_copy(0), x_copy(1))
    def clear(c):
        prob[c, pl.ds(0, H + GROUP), :] = jnp.zeros((H + GROUP, LANES), F32)
        v_v[0, c, pl.ds(0, HALO + H + GROUP), :] = jnp.zeros((HALO + H + GROUP, LANES), F32)
        k_v[0, c, pl.ds(0, HALO), :] = jnp.zeros((HALO, LANES), F32)
        h_v[0, ds(c * (T // 8), T // 8), :] = jnp.zeros((T // 8, D), F32)
    _loop("clear", 8, clear)
    x_copy(0).wait()
    start(wq_copy(1))
    _emit((0, 1, xn_steps(_Pacer(), 0, hn.at[0])))
    wq_copy(0).wait()
    start(wq_copy(2))
    _emit((0, 1, q_weight_steps(_Pacer(), 0)))

    def first_q(pace, n, tiles=(0, 1)):
        return [f for t in tiles for f in q_step(pace, t, (hn.at[0], attn.at[0])[t], n)]

    def wkv_batch(j):
        return [x_copy(2 * j + 3), x_copy(2 * j + 4)] + wkv_copies(j)

    x_copy(1).wait()
    start(wq_copy(3))
    pace = _Pacer(x_v[pl.ds(0, 8), pl.ds(0, LANES)].astype(F32))
    _emit((0, 1, first_q(pace, 0, [0])), (0.063, 1.356, xn_steps(pace, 1, attn.at[0])))
    start(x_copy(2))
    wq_copy(1).wait()
    start(*wkv_copies(0))
    pace = _Pacer(x_v[pl.ds(0, 8), pl.ds(0, LANES)].astype(F32))
    _emit((0, 1, first_q(pace, 0, [1])), (0.118, 0.9, q_weight_steps(pace, 1)))
    wq_copy(2).wait()
    start(x_copy(3), x_copy(4))
    pace = _Pacer(x_v[pl.ds(0, 8), pl.ds(0, LANES)].astype(F32))
    _emit((0, 1, first_q(pace, 1)), (0.136, 0.855, q_weight_steps(pace, 2)))
    wq_copy(3).wait()
    x_copy(2).wait()
    pace = _Pacer(x_v[pl.ds(0, 8), pl.ds(0, LANES)].astype(F32))
    _emit((0, 1, first_q(pace, 2)), (1, 2, first_q(pace, 3)),
          (0.049, 0.918, q_weight_steps(pace, 3)), (0.167, 1.817, xn_steps(pace, 2, attn.at[1])))
    following = [wkv_batch(1) + wkv_batch(2), [wo_copy] + ffn_copies(0), ffn_copies(1)]

    def phase_q(j):
        t = 2 * j + 2
        x_copy(t + 1).wait()
        x_copy(t + 2).wait()
        for k in range(NI - 1):
            @pl.when(j == k)
            def _():
                for c in wkv_copies(k):
                    c.wait()
                start(*following[k])
        pace = _Pacer(j)
        _emit(
            (0, 1, [f for n in range(NI) for f in q_step(pace, t, attn.at[1], n)]),
            (1, 2, [f for n in range(NI) for f in q_step(pace, t + 1, hn.at[0], n)]),
            (-0.131, 0.969, xn_steps(pace, t + 1, hn.at[0])),
            (0.82, 1.898, xn_steps(pace, t + 2, attn.at[1])),
            (0.1, 2.03, kv_weight_steps(pace, j)),
        )
    _loop("phase_q", NI - 1, phase_q)
    wo_copy.wait()

    def first_values(pace, g):
        for c in range(8):
            v_v[0, c, pl.ds(0, HALO), :] = jnp.broadcast_to(
                v_v[0, c, pl.ds(HALO, 1), :], (HALO, LANES))
        tile, row = g // NI, ds(g % NI * GROUP, GROUP).start
        return value_steps(pace, prob.at[:, pl.ds(row, H + GROUP)],
                           v_v.at[tile, :, pl.ds(row, HALO + H + GROUP)],
                           attn.at[tile, :, ds(row // 2, GROUP // 2)], range(0, GROUP, RB))

    def phase_kv(j):
        for c in ffn_copies(j):
            c.wait()
        pl.when(j + 2 < NT)(lambda: start(*ffn_copies(j + 2)))

        wo_src = [wo_raw.at[pl.ds(pl.multiple_of(j // NI * 64, 64), D - 64),
                            ds(s * DH + j % NI * LANES, LANES)] for s in range(2)]
        wo_dst = w_ops[WO].at[:, pl.ds(pl.multiple_of(j // NI * 32, 32), GR // 2 - 32),
                              ds(j % NI * LANES, LANES)]

        def wo_piece(hl, half):
            b = []
            for kh in range(2):
                for s in range(2):
                    u = [_words(wo_src[s][pl.ds(cp * LANES + hl * 32 + kh * 16, 16), :])
                         for cp in range(4 * half, 4 * half + 4)]
                    b.append(_transpose_row_groups([pace.start(t) for t in u]))
            for c in range(4):
                for i, t in enumerate(_rhs7(*[_halves(t[c]) for t in b])):
                    wo_dst[i * PER + c * LANES // GR,
                           pl.ds((c * LANES % GR + hl * 32 + half * 16) // 2, 8), :] = _words(t)
                    pace.finish(_words(t))
                yield

        wo_pieces = [wo_piece(hl, half) for hl in range(2) for half in range(2)]
        pace = _Pacer(j)
        tile, row = j // NI, pl.multiple_of(j % NI * GROUP, GROUP)
        _emit(
            (0, 1, project(pace, j, weight(WKV), k_v)),
            (1, 2, project(pace, j, weight(WKV, 7 * PER), v_v)),
            (0.051, 1.97, ffn_weight_steps(pace, j)),
            (0.447, 0.898, permute_q_steps(pace, tile, [row, H + row])),
            (0.05, 1.114, [lambda g=g: next(g) for g in wo_pieces for _ in range(4)]),
            (0.072, 1.017, first_values(pace, jnp.maximum(j - 1, 0))),
            (1.042, 2.045, softmax_steps(
                pace, q_v.at[tile, :, pl.ds(row, H + GROUP)],
                k_v.at[tile, :, pl.ds(row, HALO + H + GROUP)], prob.at[:, pl.ds(row, H + GROUP)],
                [s * H + r for s in range(2) for r in range(0, GROUP, SB)], tile * T + row)),
        )
    _loop("phase_kv", NT, phase_kv)
    _emit((0, 1, first_values(_Pacer(), NT - 1)))

    def ffn(j):
        nxt = last(j + 2)
        slot = j % 2
        pace = _Pacer(j)
        gate = {}

        def gate_done(n, *c):
            gate[n] = [_gelu(t) for t in c]

        def up_done(n, *c):
            for i, t in enumerate(_lhs7(*[g * u for g, u in zip(gate.pop(n), c)])):
                act[i, :, n:n + TN] = _words(t)

        def down_done(n, *c):
            for b, t in enumerate(c):
                cols = pl.ds(b % 2 * DH + n, TN)
                out_v[ds(j * T + b // 2 * H, H), cols] = (
                    h_v[slot, pl.ds(b // 2 * H, H), cols] + t).astype(BF16)

        g = _matmul(pace, lambda i: hn[0, i], ffn_weight(ffn_w[0]), FH, gate_done)
        u = _matmul(pace, lambda i: hn[0, i], ffn_weight(ffn_w[1]), FH, up_done)
        gu = [f for n in range(0, len(g), 7) for f in g[n:n + 7] + u[n:n + 7]]
        _emit(
            (0, 1, gu),
            (1, 1.5, _matmul(pace, lambda i: act[i], ffn_weight(ffn_w[2]), DH, down_done)),
            (0.012, 0.619, softmax_steps(pace, q_v.at[nxt % 2], k_v.at[nxt], prob, range(0, T, SB))),
            (0.592, 0.99, value_steps(pace, prob, v_v.at[nxt], attn.at[slot], range(0, H, RB))),
            (1.014, 1.377, hn_steps(pace, 1 - slot, 0)),
            (1.39, 1.39, [c.start for c in out_copies(j, 0, DH - TN)]),
        )
        for c in out_copies(j, DH - TN, DH):
            c.start()

    def phase_ffn(t):
        @pl.when(t < NT)
        def _():
            pace = _Pacer(t)
            _emit((0, 1, output_steps(pace, t, t % 2)),
                  (-0.108, 1.029, hn_steps(pace, 0, jnp.where(t == 1, 0, 1))),
                  (0.045, 1.046, permute_q_steps(pace, last(t + 1), range(0, T, GROUP))))

        pl.when(t > 0)(lambda: ffn(t - 1))
    _loop("phase_ffn", NT + 1, phase_ffn)
    for j in range(NT):
        for c in out_copies(j, 0, DH - TN) + out_copies(j, DH - TN, DH):
            c.wait()


@jax.jit
def pallas_sequential_preLN__sliding_local_dilated__glu_gated_geglu__prompt_kernel(
    A_x: jax.Array,
    A_wqkv: jax.Array,
    A_wo: jax.Array,
    B_x: jax.Array,
    B_w_gate: jax.Array,
    B_w_up: jax.Array,
    B_w_down: jax.Array,
):
    del B_x
    B, S, D = A_x.shape
    F = B_w_gate.shape[1]
    DH, FH = D // 2, F // 2
    NT = S // T
    NI = NT // 2
    assert B == 1 and D == 8 * LANES and NI == 4 and NI * TN == DH and FH % GR == 0 and 2 * GR == DH
    any_spec = pl.BlockSpec(memory_space=pl.ANY)
    out = pl.pallas_call(
        _kernel,
        in_specs=[any_spec] * 6,
        out_specs=any_spec,
        out_shape=jax.ShapeDtypeStruct((S, D), A_x.dtype),
        scratch_shapes=[
            pltpu.VMEM((S + T, D), BF16),
            pltpu.VMEM((NI, D // GR, GR, 2 * TN), BF16),
            pltpu.VMEM((2, D // GR, GR, D), BF16),
            pltpu.VMEM((D, D), BF16),
            pltpu.VMEM((T, D), F32),
            [pltpu.VMEM((n * 7 * DH // GR, GR // 2, DH), U32)
             for n in (1, 2, 1)],
            [(pltpu.VMEM((k // GR, GR, n), BF16),
              pltpu.VMEM((3, k // 2 // GR, GR, n // 2), BF16))
             for k, n in ((D, F), (D, F), (F, D))],
            pltpu.VMEM((7 * NT + 7, H // 2, DH), U32),
            pltpu.VMEM((2, 7, H // 2, DH), U32),
            pltpu.VMEM((2, 7, H // 2, DH), U32),
            pltpu.VMEM((WINDOW, T, LANES), F32),
            pltpu.VMEM((7, H // 2, FH), U32),
            pltpu.VMEM((NT, 8, T, LANES), F32),
            pltpu.VMEM((2, 8, T, LANES), F32),
            pltpu.VMEM((NT + 1, 8, HALO + T, LANES), F32),
            pltpu.VMEM((NT + 1, 8, HALO + T, LANES), F32),
            pltpu.VMEM((2, T, D), F32),
            pltpu.VMEM((S, D), BF16),
            pltpu.SemaphoreType.DMA((NT + 1,)),
            pltpu.SemaphoreType.DMA((NI,)),
            pltpu.SemaphoreType.DMA((NI - 1,)),
            pltpu.SemaphoreType.DMA(()),
            pltpu.SemaphoreType.DMA((NT,)),
            pltpu.SemaphoreType.DMA((NT,)),
        ],
        compiler_params=pltpu.CompilerParams(vmem_limit_bytes=124 * 2**20),
    )(A_x.reshape(S, D), A_wqkv.reshape(D // GR, GR, 3 * D), A_wo,
      B_w_gate.reshape(D // GR, GR, F), B_w_up.reshape(D // GR, GR, F),
      B_w_down.reshape(F // GR, GR, D))
    return out.reshape(B, S, D)
```

```python
import jax
import jax.numpy as jnp
from jax import lax
import jax.experimental.pallas as pl
import jax.experimental.pallas.tpu as pltpu

HEAD_DIM = 32
WINDOW = 8
DILATION = 2
HALO = 16
LANES = 128
T = 256
H = T // 2
SB = 8
RB = 16
TN = 128
PLAIN = (1, 4)
GR = 256
SCOPES = False
F32 = jnp.float32
BF16 = jnp.bfloat16
U32 = jnp.uint32


def _words(x):
    return pltpu.bitcast(x, U32)


def _halves(x):
    return pltpu.bitcast(x, BF16)


def _loop(name, n, body):
    def step(j, carry):
        if SCOPES:
            with jax.named_scope(name):
                body(j)
        else:
            body(j)
        return carry
    lax.fori_loop(0, n, step, 0)


def _emit(*stages):
    order = []
    for s, (lo, hi, steps) in enumerate(stages):
        order += [(lo + (hi - lo) * i / len(steps), s, i, f) for i, f in enumerate(steps)]
    for _, _, _, f in sorted(order, key=lambda t: t[:3]):
        f()


def _pipelined(pieces, depth):
    def step(t):
        for g in reversed(pieces[max(t - depth + 1, 0):t + 1]):
            next(g, None)
    return [lambda t=t: step(t) for t in range(len(pieces) + depth - 1)]


class _Pacer:
    def __init__(self, value=None):
        if value is None:
            self.never = None
        else:
            value = jnp.broadcast_to(value, (8, LANES))
            self.never = (value > 1) & (value < -1)
        self.products = []
        self.due = []

    def _tie(self, x, others):
        rows = x.shape[0] // 8
        width = min(-(-len(others) // rows) * LANES, x.shape[1])
        regs = [[x[r:r + 8, c:c + LANES] for r in range(0, x.shape[0], 8)]
                for c in range(0, width, LANES)]
        for k, other in enumerate(others):
            col, other = regs[k // rows % len(regs)], other[:8, :LANES]
            if other.dtype != x.dtype:
                other = pltpu.bitcast(other, x.dtype)
            col[k % rows] = lax.select(self.never, other, col[k % rows])
        cols = [jnp.concatenate(col, axis=0) for col in regs]
        return jnp.concatenate(cols + [x[:, width:]] * (width < x.shape[1]), axis=1)

    def start(self, x, lag=3):
        if self.never is None or len(self.products) < lag:
            return x
        return self._tie(x, [self.products[-lag]] * (x.shape[0] // 8))

    def finish(self, x):
        if self.never is not None:
            self.due.append(x)

    def dot(self, lhs_words, rhs):
        if self.due:
            lhs_words = self._tie(lhs_words, self.due)
            self.due = []
        self.products.append(jnp.dot(_halves(lhs_words), rhs, preferred_element_type=F32))
        return self.products[-1]


def _gelu(x):
    c = 0.7978845608028654
    hx = 0.5 * x
    return hx + hx * jnp.tanh(x * (c + (c * 0.044715) * (x * x)))


def _lhs7(a11, a12, a21, a22):
    return [t.astype(BF16) for t in
            (a11 + a22, a21 + a22, a11, a22, a11 + a12, a21 - a11, a12 - a22)]


def _rhs7(b11, b12, b21, b22):
    f11, f12, f21, f22 = (b.astype(F32) for b in (b11, b12, b21, b22))
    return [t.astype(BF16) for t in
            (f11 + f22, b11, f12 - f22, f21 - f11, b22, f11 + f12, f21 + f22)]


def _strassen(pace, lhs, rhs, done):
    c = {}

    def m(i):
        return pace.dot(lhs(i), rhs(i))

    def s0():
        c["m1"] = m(0)

    def s1():
        c["m2"] = m(1)
        c[22] = c["m1"] - c["m2"]

    def s2():
        t = m(3)
        c[21] = c["m2"] + t
        c[11] = c["m1"] + t

    def s3():
        c["m5"] = m(4)
        c[11] = c[11] - c["m5"]

    def s4():
        t = m(2)
        c[12] = c["m5"] + t
        c[22] = c[22] + t

    def s5():
        c[11] = c[11] + m(6)

    def s6():
        done(c[11], c[12], c[21], c[22] + m(5))

    return [s0, s1, s2, s3, s4, s5, s6]


def _matmul(pace, lhs, rhs, width, done):
    steps = []
    for n in range(0, width, TN):
        steps += _strassen(pace, lhs, lambda i, n=n: rhs(i, n), lambda *c, n=n: done(n, *c))
    return steps


def _permute_cols(chunks):
    lane = lax.broadcasted_iota(jnp.int32, chunks[0].shape, 1)
    a = [pltpu.roll(chunks[c], 4 * c, 1) if c else chunks[c] for c in range(8)]
    yield
    e = [a[(-i) % 8] for i in range(8)]
    for s in (1, 2, 4):
        moved = (lane & 4 * s) != 0
        e = [lax.select(moved, e[(i - s) % 8], e[i]) for i in range(8)]
    e = [pltpu.roll(e[c], LANES - 4 * c, 1) if c else e[c] for c in range(8)]
    yield
    return e


def _transpose_row_groups(u):
    return [jnp.concatenate([t[2 * c:2 * c + 2] for t in u], axis=0) for c in range(4)]


def _kernel(x_hbm, wqkv_hbm, wo_hbm, wg_hbm, wu_hbm, wd_hbm, out_hbm,
            x_v, wq_raw, wkv_raw, wo_raw, centred, w_ops, ffn_w, a_ops, hn, attn, prob, act,
            q_raw, q_v, k_v, v_v, h_v, out_v,
            sem_x, sem_q, sem_kv, sem_o, sem_f, sem_out):
    S, D = x_hbm.shape
    DH = D // 2
    FH = wg_hbm.shape[2] // 2
    NT = S // T
    NI = NT // 2
    FR = GR // NT
    NG = 2 * GR // RB
    KG = -(-NG // (NI - 1))
    SKIP = KG * (NI - 1) - NG
    GROUP = H // NI
    PER = DH // GR
    WQ, WKV, WO = range(3)

    def ds(start, size):
        return pl.ds(start if isinstance(start, int) else pl.multiple_of(start, size), size)

    def last(j):
        return min(j, NT - 1) if isinstance(j, int) else jnp.minimum(j, NT - 1)

    def x_copy(j):
        return pltpu.make_async_copy(x_hbm.at[ds(last(j) * T, T)], x_v.at[ds(j * T, T)],
                                     sem_x.at[j])

    def wq_copy(n):
        return pltpu.make_async_copy(wqkv_hbm.at[:, :, ds(n * 2 * TN, 2 * TN)],
                                     wq_raw.at[n], sem_q.at[n])

    def wkv_copies(j):
        copies = []
        for m in range(2):
            lo = max((j * KG - SKIP) * RB - m * GR, 0)
            hi = min(((j + 1) * KG - SKIP) * RB - m * GR, GR)
            if lo < hi:
                copies.append(pltpu.make_async_copy(
                    wqkv_hbm.at[:, pl.ds(lo, hi - lo), pl.ds((1 + m) * D, D)],
                    wkv_raw.at[m, :, pl.ds(lo, hi - lo)], sem_kv.at[j]))
        return copies

    wo_copy = pltpu.make_async_copy(wo_hbm, wo_raw, sem_o)

    def ffn_copies(j):
        rows = ds(j * FR, FR)
        return [pltpu.make_async_copy(src.at[:, rows], dst.at[:, rows], sem_f.at[j])
                for src, (dst, _) in zip((wg_hbm, wu_hbm, wd_hbm), ffn_w)]

    def out_copies(j, lo, hi):
        return [pltpu.make_async_copy(out_v.at[ds(j * T, T), pl.ds(s * DH + lo, hi - lo)],
                                      out_hbm.at[ds(j * T, T), pl.ds(s * DH + lo, hi - lo)],
                                      sem_out.at[j]) for s in range(2)]

    def weight(m, first=0):
        return lambda i, n: _halves(
            w_ops[m][pl.ds(first + i * PER, PER), :, ds(n, TN)].reshape(DH // 2, TN))

    def norm_steps(pace, load_rows, store):
        def piece(r):
            def load():
                return jnp.concatenate([load_rows(s * H + r).astype(F32) for s in range(2)], axis=0)
            m = jnp.mean(pace.start(load()), axis=-1, keepdims=True)
            yield
            c = load() - m
            centred[ds(2 * r, 2 * RB), :] = c
            scale = lax.rsqrt(jnp.mean(c * c, axis=-1, keepdims=True) + 1e-5)
            yield
            y = centred[ds(2 * r, 2 * RB), :] * scale
            for i, t in enumerate(_lhs7(y[:RB, :DH], y[:RB, DH:], y[RB:, :DH], y[RB:, DH:])):
                store(i, ds(r // 2, RB // 2), _words(t))
                pace.finish(_words(t)[:, i % 4 * LANES:(i % 4 + 1) * LANES])
        return _pipelined([piece(r) for r in range(0, H, RB)], 3)

    def xn_steps(pace, j, copy):
        def store(i, where, t):
            a_ops[7 * j + i, where, :] = t
            copy[i, where, :] = t
        return norm_steps(pace, lambda r: x_v[ds(j * T + r, RB), :], store)

    def hn_steps(pace, slot, dest):
        def store(i, rows, t):
            hn[dest, i, rows, :] = t
        return norm_steps(pace, lambda r: h_v[slot, pl.ds(r, RB), :], store)

    def q_weight_steps(pace, n):
        def step(g, r):
            top, bot = (wq_raw[n, kh * PER + g, pl.ds(r, 2 * RB), :] for kh in range(2))
            b11 = pace.start(top[:, :TN].astype(F32))
            for i, t in enumerate(_rhs7(b11, top[:, TN:], bot[:, :TN], bot[:, TN:])):
                w_ops[WQ][i * PER + g, pl.ds(r // 2, RB), pl.ds(n * TN, TN)] = _words(t)
                pace.finish(_words(t)[i % 2 * 8:])
        return [lambda g=g, r=r: step(g, r) for g in range(PER) for r in range(0, GR, 2 * RB)]

    def kv_weight_steps(pace, j):
        def piece(g, group):
            m, row = group // (NG // 2), group % (NG // 2) * RB
            src, first, dst = ds(row, RB), m * 7 * PER + g, ds(row // 2, RB // 2)
            u = [jnp.concatenate(
                [_words(wkv_raw[m, kh * PER + g, src, pl.ds(c * LANES, LANES)])
                 for kh in range(2)], axis=0) for c in range(8)]
            u = yield from _permute_cols(u[:1] + [pace.start(u[1])] + u[2:])
            for c in range(4):
                b = [_halves(u[nh * 4 + c][kh * RB // 2:(kh + 1) * RB // 2])
                     for kh in range(2) for nh in range(2)]
                for i, t in enumerate(_rhs7(*b)):
                    w_ops[WKV][first + i * PER, dst, pl.ds(c * LANES, LANES)] = _words(t)
                    if i >= 5:
                        pace.finish(_words(t))
        return _pipelined([piece(g, jnp.maximum(j * KG - SKIP + r, 0)) for r in range(KG)
                           for g in range(PER)], 3)

    def ffn_index(w, i, g, rows, n, width):
        blocks, extra = w
        _, per, _, half = extra.shape
        if 1 <= i <= 4:
            g = pl.ds((i - 1) // 2 * per, per) if g is None else (i - 1) // 2 * per + g
            return blocks, (g, rows, pl.ds((i - 1) % 2 * half + n, width))
        return extra, (i % 4, slice(None) if g is None else g, rows, pl.ds(n, width))

    def ffn_weight_steps(pace, j):
        def step(w, g, n):
            where = [ffn_index(w, i, g, slice(None), n, 2 * LANES) for i in range(7)]
            blocks = [ref[idx] for ref, idx in where[1:5]]
            blocks[0] = pace.start(blocks[0].astype(F32), 3)
            pace.finish(blocks[0])
            for i, t in enumerate(_rhs7(*blocks)):
                if i not in PLAIN:
                    ref, idx = where[i]
                    ref[idx] = t
        chunk = [(blocks.at[:, ds(j * FR, FR)], extra.at[:, :, ds(j * FR, FR)])
                 for blocks, extra in ffn_w]
        steps = [[lambda w=w, g=g, n=n: step(w, g, n) for g in range(w[1].shape[1])
                  for n in range(0, w[1].shape[3], 2 * LANES)] for w in chunk]
        return [f for group in zip(*steps) for f in group]

    def ffn_weight(w):
        def load(i, n):
            ref, idx = ffn_index(w, i, None, slice(None), n, TN)
            return ref[idx].reshape(w[1].shape[1] * GR, TN)
        return load

    def permute_q_steps(pace, j, rows):
        slot = j % 2

        def piece(r):
            where = ds(r, GROUP)
            q = [q_raw[j, c, where, :] for c in range(8)]
            q = yield from _permute_cols(q[:1] + [pace.start(q[1])] + q[2:])
            for c in range(8):
                q_v[slot, c, where, :] = q[c]
                pace.finish(q[c][c * 8 % GROUP:])
        return _pipelined([piece(r) for r in rows], 3)

    def q_step(pace, j, lhs, n):
        def done(*c):
            for b, t in enumerate(c):
                q_raw[j, 2 * n + b % 2, pl.ds(b // 2 * H, H), :] = t
        return _strassen(pace, lambda i: lhs[i], lambda i: weight(WQ)(i, n * TN), done)

    def project(pace, j, rhs, dst):
        lhs, dst = a_ops.at[pl.ds(7 * j, 7)], dst.at[pl.ds(j, 2)]

        def done(n, *c):
            for b, t in enumerate(c):
                chunk = (b % 2 * DH + n) // LANES
                dst[0, chunk, pl.ds(HALO + b // 2 * H, H), :] = t
                if b // 2:
                    dst[1, chunk, pl.ds(0, HALO), :] = t[H - HALO:]
        return _matmul(pace, lambda i: lhs[i], rhs, DH, done)

    def softmax_steps(pace, q, k, out, rows, first=None):
        def piece(r):
            logits = [None] * WINDOW
            for c in range(8):
                qc = q[c, pl.ds(r, SB), :]
                if c == 0:
                    qc = pace.start(qc)
                for w in range(WINDOW):
                    t = qc * k[c, pl.ds(HALO + r - DILATION * w, SB), :]
                    logits[w] = t if c == 0 else logits[w] + t
            lane = lax.broadcasted_iota(jnp.int32, (SB, LANES), 1)
            for s in (1, 2):
                rolled = [(pltpu.roll(l, s, 1), pltpu.roll(l, LANES - s, 1)) for l in logits]
                yield
                upper = (lane & s) != 0
                logits = [l + lax.select(upper, a, b) for l, (a, b) in zip(logits, rolled)]
            for w in range(WINDOW):
                l = logits[w] * (HEAD_DIM ** -0.5)
                if first is not None and r < DILATION * w:
                    pos = first + r + lax.broadcasted_iota(jnp.int32, (SB, LANES), 0)
                    l = jnp.where(pos >= DILATION * w, l, -1e9)
                logits[w] = l
            m = logits[0]
            for w in range(1, WINDOW):
                m = jnp.maximum(m, logits[w])
            e = [jnp.exp(l - m) for l in logits]
            total = e[0]
            for w in range(1, WINDOW):
                total = total + e[w]
            inv = 1.0 / total
            for w in range(WINDOW):
                p = e[w] * inv
                out[w, pl.ds(r, SB), :] = p
                pace.finish(p)
        return _pipelined([piece(r) for r in rows], 3)

    def value_steps(pace, weights, v, out, rows):
        def piece(r, c):
            blocks = []
            for row in (r, H + r):
                for chunk in (c, c + 4):
                    for w in range(WINDOW):
                        p = weights[w, pl.ds(row, RB), :]
                        t = (pace.start(p, 6) if w == 0 else p) * v[
                            chunk, pl.ds(HALO + row - DILATION * w, RB), :]
                        o = t if w == 0 else o + t
                    blocks.append(o)
                    pace.finish(o)
                    pace.finish(o[8:])
                    yield
            for i, t in enumerate(_lhs7(*blocks)):
                out[i, pl.ds(r // 2, RB // 2), pl.ds(c * LANES, LANES)] = _words(t)
                pace.finish(_words(t))
        pieces = [piece(r, c) for r in rows for c in range(4)]
        return [lambda g=g: next(g, None) for g in pieces for _ in range(5)]

    def output_steps(pace, j, slot):
        def done(n, *c):
            for b, t in enumerate(c):
                cols = pl.ds(b % 2 * DH + n, TN)
                h_v[slot, pl.ds(b // 2 * H, H), cols] = (
                    x_v[ds(j * T + b // 2 * H, H), cols].astype(F32) + t)
        return _matmul(pace, lambda i: attn[slot, i], weight(WO), DH, done)

    def start(*copies):
        for c in copies:
            c.start()

    start(x_copy(0), wq_copy(0), x_copy(1))
    def clear(c):
        prob[c, pl.ds(0, H + GROUP), :] = jnp.zeros((H + GROUP, LANES), F32)
        v_v[0, c, pl.ds(0, HALO + H + GROUP), :] = jnp.zeros((HALO + H + GROUP, LANES), F32)
        k_v[0, c, pl.ds(0, HALO), :] = jnp.zeros((HALO, LANES), F32)
        h_v[0, ds(c * (T // 8), T // 8), :] = jnp.zeros((T // 8, D), F32)
    _loop("clear", 8, clear)
    x_copy(0).wait()
    start(wq_copy(1))
    _emit((0, 1, xn_steps(_Pacer(), 0, hn.at[0])))
    wq_copy(0).wait()
    start(wq_copy(2))
    _emit((0, 1, q_weight_steps(_Pacer(), 0)))

    def first_q(pace, n, tiles=(0, 1)):
        return [f for t in tiles for f in q_step(pace, t, (hn.at[0], attn.at[0])[t], n)]

    def wkv_batch(j):
        return [x_copy(2 * j + 3), x_copy(2 * j + 4)] + wkv_copies(j)

    x_copy(1).wait()
    start(wq_copy(3))
    pace = _Pacer(x_v[pl.ds(0, 8), pl.ds(0, LANES)].astype(F32))
    _emit((0, 1, first_q(pace, 0, [0])), (0.063, 1.356, xn_steps(pace, 1, attn.at[0])))
    start(x_copy(2))
    wq_copy(1).wait()
    start(*wkv_copies(0))
    pace = _Pacer(x_v[pl.ds(0, 8), pl.ds(0, LANES)].astype(F32))
    _emit((0, 1, first_q(pace, 0, [1])), (0.118, 0.9, q_weight_steps(pace, 1)))
    wq_copy(2).wait()
    start(x_copy(3), x_copy(4))
    pace = _Pacer(x_v[pl.ds(0, 8), pl.ds(0, LANES)].astype(F32))
    _emit((0, 1, first_q(pace, 1)), (0.136, 0.855, q_weight_steps(pace, 2)))
    wq_copy(3).wait()
    x_copy(2).wait()
    pace = _Pacer(x_v[pl.ds(0, 8), pl.ds(0, LANES)].astype(F32))
    _emit((0, 1, first_q(pace, 2)), (1, 2, first_q(pace, 3)),
          (0.049, 0.918, q_weight_steps(pace, 3)), (0.167, 1.817, xn_steps(pace, 2, attn.at[1])))
    following = [wkv_batch(1) + wkv_batch(2), [wo_copy] + ffn_copies(0), ffn_copies(1)]

    def phase_q(j):
        t = 2 * j + 2
        x_copy(t + 1).wait()
        x_copy(t + 2).wait()
        for k in range(NI - 1):
            @pl.when(j == k)
            def _():
                for c in wkv_copies(k):
                    c.wait()
                start(*following[k])
        pace = _Pacer(j)
        _emit(
            (0, 1, [f for n in range(NI) for f in q_step(pace, t, attn.at[1], n)]),
            (1, 2, [f for n in range(NI) for f in q_step(pace, t + 1, hn.at[0], n)]),
            (-0.131, 0.969, xn_steps(pace, t + 1, hn.at[0])),
            (0.82, 1.898, xn_steps(pace, t + 2, attn.at[1])),
            (0.1, 2.03, kv_weight_steps(pace, j)),
        )
    _loop("phase_q", NI - 1, phase_q)
    wo_copy.wait()

    def first_values(pace, g):
        for c in range(8):
            v_v[0, c, pl.ds(0, HALO), :] = jnp.broadcast_to(
                v_v[0, c, pl.ds(HALO, 1), :], (HALO, LANES))
        tile, row = g // NI, ds(g % NI * GROUP, GROUP).start
        return value_steps(pace, prob.at[:, pl.ds(row, H + GROUP)],
                           v_v.at[tile, :, pl.ds(row, HALO + H + GROUP)],
                           attn.at[tile, :, ds(row // 2, GROUP // 2)], range(0, GROUP, RB))

    def phase_kv(j):
        for c in ffn_copies(j):
            c.wait()
        pl.when(j + 2 < NT)(lambda: start(*ffn_copies(j + 2)))

        wo_src = [wo_raw.at[pl.ds(pl.multiple_of(j // NI * 64, 64), D - 64),
                            ds(s * DH + j % NI * LANES, LANES)] for s in range(2)]
        wo_dst = w_ops[WO].at[:, pl.ds(pl.multiple_of(j // NI * 32, 32), GR // 2 - 32),
                              ds(j % NI * LANES, LANES)]

        def wo_piece(hl, half):
            b = []
            for kh in range(2):
                for s in range(2):
                    u = [_words(wo_src[s][pl.ds(cp * LANES + hl * 32 + kh * 16, 16), :])
                         for cp in range(4 * half, 4 * half + 4)]
                    b.append(_transpose_row_groups([pace.start(t) for t in u]))
            for c in range(4):
                for i, t in enumerate(_rhs7(*[_halves(t[c]) for t in b])):
                    wo_dst[i * PER + c * LANES // GR,
                           pl.ds((c * LANES % GR + hl * 32 + half * 16) // 2, 8), :] = _words(t)
                    pace.finish(_words(t))
                yield

        wo_pieces = [wo_piece(hl, half) for hl in range(2) for half in range(2)]
        pace = _Pacer(j)
        tile, row = j // NI, pl.multiple_of(j % NI * GROUP, GROUP)
        _emit(
            (0, 1, project(pace, j, weight(WKV), k_v)),
            (1, 2, project(pace, j, weight(WKV, 7 * PER), v_v)),
            (0.051, 1.97, ffn_weight_steps(pace, j)),
            (0.447, 0.898, permute_q_steps(pace, tile, [row, H + row])),
            (0.05, 1.114, [lambda g=g: next(g) for g in wo_pieces for _ in range(4)]),
            (0.072, 1.017, first_values(pace, jnp.maximum(j - 1, 0))),
            (1.042, 2.045, softmax_steps(
                pace, q_v.at[tile, :, pl.ds(row, H + GROUP)],
                k_v.at[tile, :, pl.ds(row, HALO + H + GROUP)], prob.at[:, pl.ds(row, H + GROUP)],
                [s * H + r for s in range(2) for r in range(0, GROUP, SB)], tile * T + row)),
        )
    _loop("phase_kv", NT, phase_kv)
    _emit((0, 1, first_values(_Pacer(), NT - 1)))

    def ffn(j):
        nxt = last(j + 2)
        slot = j % 2
        pace = _Pacer(j)
        gate = {}

        def gate_done(n, *c):
            gate[n] = [_gelu(t) for t in c]

        def up_done(n, *c):
            for i, t in enumerate(_lhs7(*[g * u for g, u in zip(gate.pop(n), c)])):
                act[i, :, n:n + TN] = _words(t)

        def down_done(n, *c):
            for b, t in enumerate(c):
                cols = pl.ds(b % 2 * DH + n, TN)
                out_v[ds(j * T + b // 2 * H, H), cols] = (
                    h_v[slot, pl.ds(b // 2 * H, H), cols] + t).astype(BF16)

        g = _matmul(pace, lambda i: hn[0, i], ffn_weight(ffn_w[0]), FH, gate_done)
        u = _matmul(pace, lambda i: hn[0, i], ffn_weight(ffn_w[1]), FH, up_done)
        gu = [f for n in range(0, len(g), 7) for f in g[n:n + 7] + u[n:n + 7]]
        _emit(
            (0, 1, gu),
            (1, 1.5, _matmul(pace, lambda i: act[i], ffn_weight(ffn_w[2]), DH, down_done)),
            (0.012, 0.619, softmax_steps(pace, q_v.at[nxt % 2], k_v.at[nxt], prob, range(0, T, SB))),
            (0.592, 0.99, value_steps(pace, prob, v_v.at[nxt], attn.at[slot], range(0, H, RB))),
            (1.014, 1.377, hn_steps(pace, 1 - slot, 0)),
            (1.39, 1.39, [c.start for c in out_copies(j, 0, DH - TN)]),
        )
        for c in out_copies(j, DH - TN, DH):
            c.start()

    def phase_ffn(t):
        @pl.when(t < NT)
        def _():
            pace = _Pacer(t)
            _emit((0, 1, output_steps(pace, t, t % 2)),
                  (-0.108, 1.029, hn_steps(pace, 0, jnp.where(t == 1, 0, 1))),
                  (0.045, 1.046, permute_q_steps(pace, last(t + 1), range(0, T, GROUP))))

        pl.when(t > 0)(lambda: ffn(t - 1))
    _loop("phase_ffn", NT + 1, phase_ffn)
    for j in range(NT):
        for c in out_copies(j, 0, DH - TN) + out_copies(j, DH - TN, DH):
            c.wait()


@jax.jit
def pallas_sequential_preLN__sliding_local_dilated__glu_gated_geglu__prompt_kernel(
    A_x: jax.Array,
    A_wqkv: jax.Array,
    A_wo: jax.Array,
    B_x: jax.Array,
    B_w_gate: jax.Array,
    B_w_up: jax.Array,
    B_w_down: jax.Array,
):
    del B_x
    B, S, D = A_x.shape
    F = B_w_gate.shape[1]
    DH, FH = D // 2, F // 2
    NT = S // T
    NI = NT // 2
    assert B == 1 and D == 8 * LANES and NI == 4 and NI * TN == DH and FH % GR == 0 and 2 * GR == DH
    any_spec = pl.BlockSpec(memory_space=pl.ANY)
    out = pl.pallas_call(
        _kernel,
        in_specs=[any_spec] * 6,
        out_specs=any_spec,
        out_shape=jax.ShapeDtypeStruct((S, D), A_x.dtype),
        scratch_shapes=[
            pltpu.VMEM((S + T, D), BF16),
            pltpu.VMEM((NI, D // GR, GR, 2 * TN), BF16),
            pltpu.VMEM((2, D // GR, GR, D), BF16),
            pltpu.VMEM((D, D), BF16),
            pltpu.VMEM((T, D), F32),
            [pltpu.VMEM((n * 7 * DH // GR, GR // 2, DH), U32)
             for n in (1, 2, 1)],
            [(pltpu.VMEM((k // GR, GR, n), BF16),
              pltpu.VMEM((3, k // 2 // GR, GR, n // 2), BF16))
             for k, n in ((D, F), (D, F), (F, D))],
            pltpu.VMEM((7 * NT + 7, H // 2, DH), U32),
            pltpu.VMEM((2, 7, H // 2, DH), U32),
            pltpu.VMEM((2, 7, H // 2, DH), U32),
            pltpu.VMEM((WINDOW, T, LANES), F32),
            pltpu.VMEM((7, H // 2, FH), U32),
            pltpu.VMEM((NT, 8, T, LANES), F32),
            pltpu.VMEM((2, 8, T, LANES), F32),
            pltpu.VMEM((NT + 1, 8, HALO + T, LANES), F32),
            pltpu.VMEM((NT + 1, 8, HALO + T, LANES), F32),
            pltpu.VMEM((2, T, D), F32),
            pltpu.VMEM((S, D), BF16),
            pltpu.SemaphoreType.DMA((NT + 1,)),
            pltpu.SemaphoreType.DMA((NI,)),
            pltpu.SemaphoreType.DMA((NI - 1,)),
            pltpu.SemaphoreType.DMA(()),
            pltpu.SemaphoreType.DMA((NT,)),
            pltpu.SemaphoreType.DMA((NT,)),
        ],
        compiler_params=pltpu.CompilerParams(vmem_limit_bytes=124 * 2**20),
    )(A_x.reshape(S, D), A_wqkv.reshape(D // GR, GR, 3 * D), A_wo,
      B_w_gate.reshape(D // GR, GR, F), B_w_up.reshape(D // GR, GR, F),
      B_w_down.reshape(F // GR, GR, D))
    return out.reshape(B, S, D)
```

```python
import jax
import jax.numpy as jnp
from jax import lax
import jax.experimental.pallas as pl
import jax.experimental.pallas.tpu as pltpu

HEAD_DIM = 32
WINDOW = 8
DILATION = 2
HALO = 16
LANES = 128
T = 256
H = T // 2
SB = 8
RB = 16
TN = 128
PLAIN = (1, 4)
GR = 256
SCOPES = False
F32 = jnp.float32
BF16 = jnp.bfloat16
U32 = jnp.uint32


def _words(x):
    return pltpu.bitcast(x, U32)


def _halves(x):
    return pltpu.bitcast(x, BF16)


def _loop(name, n, body):
    def step(j, carry):
        if SCOPES:
            with jax.named_scope(name):
                body(j)
        else:
            body(j)
        return carry
    lax.fori_loop(0, n, step, 0)


def _emit(*stages):
    order = []
    for s, (lo, hi, steps) in enumerate(stages):
        order += [(lo + (hi - lo) * i / len(steps), s, i, f) for i, f in enumerate(steps)]
    for _, _, _, f in sorted(order, key=lambda t: t[:3]):
        f()


def _pipelined(pieces, depth):
    def step(t):
        for g in reversed(pieces[max(t - depth + 1, 0):t + 1]):
            next(g, None)
    return [lambda t=t: step(t) for t in range(len(pieces) + depth - 1)]


class _Pacer:
    def __init__(self, value=None):
        if value is None:
            self.never = None
        else:
            value = jnp.broadcast_to(value, (8, LANES))
            self.never = (value > 1) & (value < -1)
        self.products = []
        self.due = []

    def _tie(self, x, others):
        rows = x.shape[0] // 8
        width = min(-(-len(others) // rows) * LANES, x.shape[1])
        regs = [[x[r:r + 8, c:c + LANES] for r in range(0, x.shape[0], 8)]
                for c in range(0, width, LANES)]
        for k, other in enumerate(others):
            col, other = regs[k // rows % len(regs)], other[:8, :LANES]
            if other.dtype != x.dtype:
                other = pltpu.bitcast(other, x.dtype)
            col[k % rows] = lax.select(self.never, other, col[k % rows])
        cols = [jnp.concatenate(col, axis=0) for col in regs]
        return jnp.concatenate(cols + [x[:, width:]] * (width < x.shape[1]), axis=1)

    def start(self, x, lag=3):
        if self.never is None or len(self.products) < lag:
            return x
        return self._tie(x, [self.products[-lag]] * (x.shape[0] // 8))

    def finish(self, x):
        if self.never is not None:
            self.due.append(x)

    def dot(self, lhs_words, rhs):
        if self.due:
            lhs_words = self._tie(lhs_words, self.due)
            self.due = []
        self.products.append(jnp.dot(_halves(lhs_words), rhs, preferred_element_type=F32))
        return self.products[-1]


def _gelu(x):
    c = 0.7978845608028654
    hx = 0.5 * x
    return hx + hx * jnp.tanh(x * (c + (c * 0.044715) * (x * x)))


def _lhs7(a11, a12, a21, a22):
    return [t.astype(BF16) for t in
            (a11 + a22, a21 + a22, a11, a22, a11 + a12, a21 - a11, a12 - a22)]


def _rhs7(b11, b12, b21, b22):
    f11, f12, f21, f22 = (b.astype(F32) for b in (b11, b12, b21, b22))
    return [t.astype(BF16) for t in
            (f11 + f22, b11, f12 - f22, f21 - f11, b22, f11 + f12, f21 + f22)]


def _strassen(pace, lhs, rhs, done):
    c = {}

    def m(i):
        return pace.dot(lhs(i), rhs(i))

    def s0():
        c["m1"] = m(0)

    def s1():
        c["m2"] = m(1)
        c[22] = c["m1"] - c["m2"]

    def s2():
        t = m(3)
        c[21] = c["m2"] + t
        c[11] = c["m1"] + t

    def s3():
        c["m5"] = m(4)
        c[11] = c[11] - c["m5"]

    def s4():
        t = m(2)
        c[12] = c["m5"] + t
        c[22] = c[22] + t

    def s5():
        c[11] = c[11] + m(6)

    def s6():
        done(c[11], c[12], c[21], c[22] + m(5))

    return [s0, s1, s2, s3, s4, s5, s6]


def _matmul(pace, lhs, rhs, width, done):
    steps = []
    for n in range(0, width, TN):
        steps += _strassen(pace, lhs, lambda i, n=n: rhs(i, n), lambda *c, n=n: done(n, *c))
    return steps


def _permute_cols(chunks):
    lane = lax.broadcasted_iota(jnp.int32, chunks[0].shape, 1)
    a = [pltpu.roll(chunks[c], 4 * c, 1) if c else chunks[c] for c in range(8)]
    yield
    e = [a[(-i) % 8] for i in range(8)]
    for s in (1, 2, 4):
        moved = (lane & 4 * s) != 0
        e = [lax.select(moved, e[(i - s) % 8], e[i]) for i in range(8)]
    e = [pltpu.roll(e[c], LANES - 4 * c, 1) if c else e[c] for c in range(8)]
    yield
    return e


def _transpose_row_groups(u):
    return [jnp.concatenate([t[2 * c:2 * c + 2] for t in u], axis=0) for c in range(4)]


def _kernel(x_hbm, wqkv_hbm, wo_hbm, wg_hbm, wu_hbm, wd_hbm, out_hbm,
            x_v, wq_raw, wkv_raw, wo_raw, centred, w_ops, ffn_w, a_ops, hn, attn, prob, act,
            q_raw, q_v, k_v, v_v, h_v, out_v,
            sem_x, sem_q, sem_kv, sem_o, sem_f, sem_out):
    S, D = x_hbm.shape
    DH = D // 2
    FH = wg_hbm.shape[2] // 2
    NT = S // T
    NI = NT // 2
    FR = GR // NT
    NG = 2 * GR // RB
    KG = 13
    SKIP = KG * (NI - 1) - NG
    GROUP = H // NI
    PER = DH // GR
    WQ, WKV, WO = range(3)

    def ds(start, size):
        return pl.ds(start if isinstance(start, int) else pl.multiple_of(start, size), size)

    def last(j):
        return min(j, NT - 1) if isinstance(j, int) else jnp.minimum(j, NT - 1)

    def x_copy(j):
        return pltpu.make_async_copy(x_hbm.at[ds(last(j) * T, T)], x_v.at[ds(j * T, T)],
                                     sem_x.at[j])

    def wq_copy(n):
        return pltpu.make_async_copy(wqkv_hbm.at[:, :, ds(n * 2 * TN, 2 * TN)],
                                     wq_raw.at[n], sem_q.at[n])

    def wkv_copies(j):
        copies = []
        for m in range(2):
            lo = max((j * KG - SKIP) * RB - m * GR, 0)
            hi = min(((j + 1) * KG - SKIP) * RB - m * GR, GR)
            if lo < hi:
                copies.append(pltpu.make_async_copy(
                    wqkv_hbm.at[:, pl.ds(lo, hi - lo), pl.ds((1 + m) * D, D)],
                    wkv_raw.at[m, :, pl.ds(lo, hi - lo)], sem_kv.at[j]))
        return copies

    wo_copy = pltpu.make_async_copy(wo_hbm, wo_raw, sem_o)

    def ffn_copies(j):
        rows = ds(j * FR, FR)
        return [pltpu.make_async_copy(src.at[:, rows], dst.at[:, rows], sem_f.at[j])
                for src, (dst, _) in zip((wg_hbm, wu_hbm, wd_hbm), ffn_w)]

    def out_copies(j, lo, hi):
        return [pltpu.make_async_copy(out_v.at[ds(j * T, T), pl.ds(s * DH + lo, hi - lo)],
                                      out_hbm.at[ds(j * T, T), pl.ds(s * DH + lo, hi - lo)],
                                      sem_out.at[j]) for s in range(2)]

    def weight(m, first=0):
        return lambda i, n: _halves(
            w_ops[m][pl.ds(first + i * PER, PER), :, ds(n, TN)].reshape(DH // 2, TN))

    def norm_steps(pace, load_rows, store):
        def piece(r):
            def load():
                return jnp.concatenate([load_rows(s * H + r).astype(F32) for s in range(2)], axis=0)
            m = jnp.mean(pace.start(load()), axis=-1, keepdims=True)
            yield
            c = load() - m
            centred[ds(2 * r, 2 * RB), :] = c
            scale = lax.rsqrt(jnp.mean(c * c, axis=-1, keepdims=True) + 1e-5)
            yield
            y = centred[ds(2 * r, 2 * RB), :] * scale
            for i, t in enumerate(_lhs7(y[:RB, :DH], y[:RB, DH:], y[RB:, :DH], y[RB:, DH:])):
                store(i, ds(r // 2, RB // 2), _words(t))
                pace.finish(_words(t)[:, i % 4 * LANES:(i % 4 + 1) * LANES])
        return _pipelined([piece(r) for r in range(0, H, RB)], 3)

    def xn_steps(pace, j, copy):
        def store(i, where, t):
            a_ops[7 * j + i, where, :] = t
            copy[i, where, :] = t
        return norm_steps(pace, lambda r: x_v[ds(j * T + r, RB), :], store)

    def hn_steps(pace, slot, dest):
        def store(i, rows, t):
            hn[dest, i, rows, :] = t
        return norm_steps(pace, lambda r: h_v[slot, pl.ds(r, RB), :], store)

    def q_weight_steps(pace, n):
        def step(g, r):
            top, bot = (wq_raw[n, kh * PER + g, pl.ds(r, 2 * RB), :] for kh in range(2))
            b11 = pace.start(top[:, :TN].astype(F32))
            for i, t in enumerate(_rhs7(b11, top[:, TN:], bot[:, :TN], bot[:, TN:])):
                w_ops[WQ][i * PER + g, pl.ds(r // 2, RB), pl.ds(n * TN, TN)] = _words(t)
                pace.finish(_words(t)[i % 2 * 8:])
        return [lambda g=g, r=r: step(g, r) for g in range(PER) for r in range(0, GR, 2 * RB)]

    def kv_weight_steps(pace, j):
        def piece(g, group):
            m, row = group // (NG // 2), group % (NG // 2) * RB
            src, first, dst = ds(row, RB), m * 7 * PER + g, ds(row // 2, RB // 2)
            u = [jnp.concatenate(
                [_words(wkv_raw[m, kh * PER + g, src, pl.ds(c * LANES, LANES)])
                 for kh in range(2)], axis=0) for c in range(8)]
            u = yield from _permute_cols(u[:1] + [pace.start(u[1])] + u[2:])
            for c in range(4):
                b = [_halves(u[nh * 4 + c][kh * RB // 2:(kh + 1) * RB // 2])
                     for kh in range(2) for nh in range(2)]
                for i, t in enumerate(_rhs7(*b)):
                    w_ops[WKV][first + i * PER, dst, pl.ds(c * LANES, LANES)] = _words(t)
                    if i >= 5:
                        pace.finish(_words(t))
        return _pipelined([piece(g, jnp.maximum(j * KG - SKIP + r, 0)) for r in range(KG)
                           for g in range(PER)], 3)

    def ffn_index(w, i, g, rows, n, width):
        blocks, extra = w
        _, per, _, half = extra.shape
        if 1 <= i <= 4:
            g = pl.ds((i - 1) // 2 * per, per) if g is None else (i - 1) // 2 * per + g
            return blocks, (g, rows, pl.ds((i - 1) % 2 * half + n, width))
        return extra, (i % 4, slice(None) if g is None else g, rows, pl.ds(n, width))

    def ffn_weight_steps(pace, j):
        def step(w, g, n):
            where = [ffn_index(w, i, g, slice(None), n, 2 * LANES) for i in range(7)]
            blocks = [ref[idx] for ref, idx in where[1:5]]
            blocks[0] = pace.start(blocks[0].astype(F32), 3)
            pace.finish(blocks[0])
            for i, t in enumerate(_rhs7(*blocks)):
                if i not in PLAIN:
                    ref, idx = where[i]
                    ref[idx] = t
        chunk = [(blocks.at[:, ds(j * FR, FR)], extra.at[:, :, ds(j * FR, FR)])
                 for blocks, extra in ffn_w]
        steps = [[lambda w=w, g=g, n=n: step(w, g, n) for g in range(w[1].shape[1])
                  for n in range(0, w[1].shape[3], 2 * LANES)] for w in chunk]
        return [f for group in zip(*steps) for f in group]

    def ffn_weight(w):
        def load(i, n):
            ref, idx = ffn_index(w, i, None, slice(None), n, TN)
            return ref[idx].reshape(w[1].shape[1] * GR, TN)
        return load

    def permute_q_steps(pace, j, rows):
        slot = j % 2

        def piece(r):
            where = ds(r, GROUP)
            q = [q_raw[j, c, where, :] for c in range(8)]
            q = yield from _permute_cols(q[:1] + [pace.start(q[1])] + q[2:])
            for c in range(8):
                q_v[slot, c, where, :] = q[c]
                pace.finish(q[c][c * 8 % GROUP:])
        return _pipelined([piece(r) for r in rows], 3)

    def q_step(pace, j, lhs, n):
        def done(*c):
            for b, t in enumerate(c):
                q_raw[j, 2 * n + b % 2, pl.ds(b // 2 * H, H), :] = t
        return _strassen(pace, lambda i: lhs[i], lambda i: weight(WQ)(i, n * TN), done)

    def project(pace, j, rhs, dst):
        lhs, dst = a_ops.at[pl.ds(7 * j, 7)], dst.at[pl.ds(j, 2)]

        def done(n, *c):
            for b, t in enumerate(c):
                chunk = (b % 2 * DH + n) // LANES
                dst[0, chunk, pl.ds(HALO + b // 2 * H, H), :] = t
                if b // 2:
                    dst[1, chunk, pl.ds(0, HALO), :] = t[H - HALO:]
        return _matmul(pace, lambda i: lhs[i], rhs, DH, done)

    def softmax_steps(pace, q, k, out, rows, first=None):
        def piece(r):
            logits = [None] * WINDOW
            for c in range(8):
                qc = q[c, pl.ds(r, SB), :]
                if c == 0:
                    qc = pace.start(qc)
                for w in range(WINDOW):
                    t = qc * k[c, pl.ds(HALO + r - DILATION * w, SB), :]
                    logits[w] = t if c == 0 else logits[w] + t
            lane = lax.broadcasted_iota(jnp.int32, (SB, LANES), 1)
            for s in (1, 2):
                rolled = [(pltpu.roll(l, s, 1), pltpu.roll(l, LANES - s, 1)) for l in logits]
                yield
                upper = (lane & s) != 0
                logits = [l + lax.select(upper, a, b) for l, (a, b) in zip(logits, rolled)]
            for w in range(WINDOW):
                l = logits[w] * (HEAD_DIM ** -0.5)
                if first is not None and r < DILATION * w:
                    pos = first + r + lax.broadcasted_iota(jnp.int32, (SB, LANES), 0)
                    l = jnp.where(pos >= DILATION * w, l, -1e9)
                logits[w] = l
            m = logits[0]
            for w in range(1, WINDOW):
                m = jnp.maximum(m, logits[w])
            e = [jnp.exp(l - m) for l in logits]
            total = e[0]
            for w in range(1, WINDOW):
                total = total + e[w]
            inv = 1.0 / total
            for w in range(WINDOW):
                p = e[w] * inv
                out[w, pl.ds(r, SB), :] = p
                pace.finish(p)
        return _pipelined([piece(r) for r in rows], 3)

    def value_steps(pace, weights, v, out, rows):
        def piece(r, c):
            blocks = []
            for row in (r, H + r):
                for chunk in (c, c + 4):
                    for w in range(WINDOW):
                        p = weights[w, pl.ds(row, RB), :]
                        t = (pace.start(p, 6) if w == 0 else p) * v[
                            chunk, pl.ds(HALO + row - DILATION * w, RB), :]
                        o = t if w == 0 else o + t
                    blocks.append(o)
                    pace.finish(o)
                    pace.finish(o[8:])
                    yield
            for i, t in enumerate(_lhs7(*blocks)):
                out[i, pl.ds(r // 2, RB // 2), pl.ds(c * LANES, LANES)] = _words(t)
                pace.finish(_words(t))
        pieces = [piece(r, c) for r in rows for c in range(4)]
        return [lambda g=g: next(g, None) for g in pieces for _ in range(5)]

    def output_steps(pace, j, slot):
        def done(n, *c):
            for b, t in enumerate(c):
                cols = pl.ds(b % 2 * DH + n, TN)
                h_v[slot, pl.ds(b // 2 * H, H), cols] = (
                    x_v[ds(j * T + b // 2 * H, H), cols].astype(F32) + t)
        return _matmul(pace, lambda i: attn[slot, i], weight(WO), DH, done)

    def start(*copies):
        for c in copies:
            c.start()

    start(x_copy(0), wq_copy(0), x_copy(1))
    def clear(c):
        prob[c, pl.ds(0, H + GROUP), :] = jnp.zeros((H + GROUP, LANES), F32)
        v_v[0, c, pl.ds(0, HALO + H + GROUP), :] = jnp.zeros((HALO + H + GROUP, LANES), F32)
        k_v[0, c, pl.ds(0, HALO), :] = jnp.zeros((HALO, LANES), F32)
        h_v[0, ds(c * (T // 8), T // 8), :] = jnp.zeros((T // 8, D), F32)
    _loop("clear", 8, clear)
    x_copy(0).wait()
    start(wq_copy(1))
    _emit((0, 1, xn_steps(_Pacer(), 0, hn.at[0])))
    wq_copy(0).wait()
    start(wq_copy(2))
    _emit((0, 1, q_weight_steps(_Pacer(), 0)))

    def first_q(pace, n, tiles=(0, 1)):
        return [f for t in tiles for f in q_step(pace, t, (hn.at[0], attn.at[0])[t], n)]

    def wkv_batch(j):
        return [x_copy(2 * j + 3), x_copy(2 * j + 4)] + wkv_copies(j)

    x_copy(1).wait()
    start(wq_copy(3))
    pace = _Pacer(x_v[pl.ds(0, 8), pl.ds(0, LANES)].astype(F32))
    _emit((0, 1, first_q(pace, 0, [0])), (0.063, 1.356, xn_steps(pace, 1, attn.at[0])))
    start(x_copy(2))
    wq_copy(1).wait()
    start(*wkv_copies(0))
    pace = _Pacer(x_v[pl.ds(0, 8), pl.ds(0, LANES)].astype(F32))
    _emit((0, 1, first_q(pace, 0, [1])), (0.162, 0.9, q_weight_steps(pace, 1)))
    wq_copy(2).wait()
    start(x_copy(3), x_copy(4))
    pace = _Pacer(x_v[pl.ds(0, 8), pl.ds(0, LANES)].astype(F32))
    _emit((0, 1, first_q(pace, 1)), (0.004, 0.8, q_weight_steps(pace, 2)))
    wq_copy(3).wait()
    x_copy(2).wait()
    pace = _Pacer(x_v[pl.ds(0, 8), pl.ds(0, LANES)].astype(F32))
    _emit((0, 1, first_q(pace, 2)), (1, 2, first_q(pace, 3)),
          (0.011, 0.873, q_weight_steps(pace, 3)), (0.223, 1.831, xn_steps(pace, 2, attn.at[1])))
    following = [wkv_batch(1) + wkv_batch(2), [wo_copy] + ffn_copies(0), ffn_copies(1)]

    def phase_q(j):
        t = 2 * j + 2
        x_copy(t + 1).wait()
        x_copy(t + 2).wait()
        for k in range(NI - 1):
            @pl.when(j == k)
            def _():
                for c in wkv_copies(k):
                    c.wait()
                start(*following[k])
        pace = _Pacer(j)
        _emit(
            (0, 1, [f for n in range(NI) for f in q_step(pace, t, attn.at[1], n)]),
            (1, 2, [f for n in range(NI) for f in q_step(pace, t + 1, hn.at[0], n)]),
            (-0.123, 0.969, xn_steps(pace, t + 1, hn.at[0])),
            (0.9, 1.898, xn_steps(pace, t + 2, attn.at[1])),
            (0.1, 2.03, kv_weight_steps(pace, j)),
        )
    _loop("phase_q", NI - 1, phase_q)
    wo_copy.wait()

    def first_values(pace, g):
        for c in range(8):
            v_v[0, c, pl.ds(0, HALO), :] = jnp.broadcast_to(
                v_v[0, c, pl.ds(HALO, 1), :], (HALO, LANES))
        tile, row = g // NI, ds(g % NI * GROUP, GROUP).start
        return value_steps(pace, prob.at[:, pl.ds(row, H + GROUP)],
                           v_v.at[tile, :, pl.ds(row, HALO + H + GROUP)],
                           attn.at[tile, :, ds(row // 2, GROUP // 2)], range(0, GROUP, RB))

    def phase_kv(j):
        for c in ffn_copies(j):
            c.wait()
        pl.when(j + 2 < NT)(lambda: start(*ffn_copies(j + 2)))

        wo_src = [wo_raw.at[pl.ds(pl.multiple_of(j // NI * 64, 64), D - 64),
                            ds(s * DH + j % NI * LANES, LANES)] for s in range(2)]
        wo_dst = w_ops[WO].at[:, pl.ds(pl.multiple_of(j // NI * 32, 32), GR // 2 - 32),
                              ds(j % NI * LANES, LANES)]

        def wo_piece(hl, half):
            b = []
            for kh in range(2):
                for s in range(2):
                    u = [_words(wo_src[s][pl.ds(cp * LANES + hl * 32 + kh * 16, 16), :])
                         for cp in range(4 * half, 4 * half + 4)]
                    b.append(_transpose_row_groups([pace.start(t) for t in u]))
            for c in range(4):
                for i, t in enumerate(_rhs7(*[_halves(t[c]) for t in b])):
                    wo_dst[i * PER + c * LANES // GR,
                           pl.ds((c * LANES % GR + hl * 32 + half * 16) // 2, 8), :] = _words(t)
                    pace.finish(_words(t))
                yield

        wo_pieces = [wo_piece(hl, half) for hl in range(2) for half in range(2)]
        pace = _Pacer(j)
        tile, row = j // NI, pl.multiple_of(j % NI * GROUP, GROUP)
        _emit(
            (0, 1, project(pace, j, weight(WKV), k_v)),
            (1, 2, project(pace, j, weight(WKV, 7 * PER), v_v)),
            (0.051, 1.97, ffn_weight_steps(pace, j)),
            (0.447, 0.898, permute_q_steps(pace, tile, [row, H + row])),
            (0.05, 1.114, [lambda g=g: next(g) for g in wo_pieces for _ in range(4)]),
            (0.072, 1.017, first_values(pace, jnp.maximum(j - 1, 0))),
            (1.042, 2.045, softmax_steps(
                pace, q_v.at[tile, :, pl.ds(row, H + GROUP)],
                k_v.at[tile, :, pl.ds(row, HALO + H + GROUP)], prob.at[:, pl.ds(row, H + GROUP)],
                [s * H + r for s in range(2) for r in range(0, GROUP, SB)], tile * T + row)),
        )
    _loop("phase_kv", NT, phase_kv)
    _emit((0, 1, first_values(_Pacer(), NT - 1)))

    def ffn(j):
        nxt = last(j + 2)
        slot = j % 2
        pace = _Pacer(j)
        gate = {}

        def gate_done(n, *c):
            gate[n] = [_gelu(t) for t in c]

        def up_done(n, *c):
            for i, t in enumerate(_lhs7(*[g * u for g, u in zip(gate.pop(n), c)])):
                act[i, :, n:n + TN] = _words(t)

        def down_done(n, *c):
            for b, t in enumerate(c):
                cols = pl.ds(b % 2 * DH + n, TN)
                out_v[ds(j * T + b // 2 * H, H), cols] = (
                    h_v[slot, pl.ds(b // 2 * H, H), cols] + t).astype(BF16)

        g = _matmul(pace, lambda i: hn[0, i], ffn_weight(ffn_w[0]), FH, gate_done)
        u = _matmul(pace, lambda i: hn[0, i], ffn_weight(ffn_w[1]), FH, up_done)
        gu = [f for n in range(0, len(g), 7) for f in g[n:n + 7] + u[n:n + 7]]
        _emit(
            (0, 1, gu),
            (1, 1.5, _matmul(pace, lambda i: act[i], ffn_weight(ffn_w[2]), DH, down_done)),
            (0.012, 0.619, softmax_steps(pace, q_v.at[nxt % 2], k_v.at[nxt], prob, range(0, T, SB))),
            (0.592, 0.99, value_steps(pace, prob, v_v.at[nxt], attn.at[slot], range(0, H, RB))),
            (1.014, 1.377, hn_steps(pace, 1 - slot, 0)),
            (1.39, 1.39, [c.start for c in out_copies(j, 0, DH - TN)]),
        )
        for c in out_copies(j, DH - TN, DH):
            c.start()

    def phase_ffn(t):
        @pl.when(t < NT)
        def _():
            pace = _Pacer(t)
            _emit((0, 1, output_steps(pace, t, t % 2)),
                  (-0.108, 1.03, hn_steps(pace, 0, jnp.where(t == 1, 0, 1))),
                  (0.045, 1.046, permute_q_steps(pace, last(t + 1), range(0, T, GROUP))))

        pl.when(t > 0)(lambda: ffn(t - 1))
    _loop("phase_ffn", NT + 1, phase_ffn)
    for j in range(NT):
        for c in out_copies(j, 0, DH - TN) + out_copies(j, DH - TN, DH):
            c.wait()


@jax.jit
def pallas_sequential_preLN__sliding_local_dilated__glu_gated_geglu__prompt_kernel(
    A_x: jax.Array,
    A_wqkv: jax.Array,
    A_wo: jax.Array,
    B_x: jax.Array,
    B_w_gate: jax.Array,
    B_w_up: jax.Array,
    B_w_down: jax.Array,
):
    del B_x
    B, S, D = A_x.shape
    F = B_w_gate.shape[1]
    DH, FH = D // 2, F // 2
    NT = S // T
    NI = NT // 2
    assert B == 1 and D == 8 * LANES and NI == 4 and NI * TN == DH and FH % GR == 0 and 2 * GR == DH
    any_spec = pl.BlockSpec(memory_space=pl.ANY)
    out = pl.pallas_call(
        _kernel,
        in_specs=[any_spec] * 6,
        out_specs=any_spec,
        out_shape=jax.ShapeDtypeStruct((S, D), A_x.dtype),
        scratch_shapes=[
            pltpu.VMEM((S + T, D), BF16),
            pltpu.VMEM((NI, D // GR, GR, 2 * TN), BF16),
            pltpu.VMEM((2, D // GR, GR, D), BF16),
            pltpu.VMEM((D, D), BF16),
            pltpu.VMEM((T, D), F32),
            [pltpu.VMEM((n * 7 * DH // GR, GR // 2, DH), U32)
             for n in (1, 2, 1)],
            [(pltpu.VMEM((k // GR, GR, n), BF16),
              pltpu.VMEM((3, k // 2 // GR, GR, n // 2), BF16))
             for k, n in ((D, F), (D, F), (F, D))],
            pltpu.VMEM((7 * NT + 7, H // 2, DH), U32),
            pltpu.VMEM((2, 7, H // 2, DH), U32),
            pltpu.VMEM((2, 7, H // 2, DH), U32),
            pltpu.VMEM((WINDOW, T, LANES), F32),
            pltpu.VMEM((7, H // 2, FH), U32),
            pltpu.VMEM((NT, 8, T, LANES), F32),
            pltpu.VMEM((2, 8, T, LANES), F32),
            pltpu.VMEM((NT + 1, 8, HALO + T, LANES), F32),
            pltpu.VMEM((NT + 1, 8, HALO + T, LANES), F32),
            pltpu.VMEM((2, T, D), F32),
            pltpu.VMEM((S, D), BF16),
            pltpu.SemaphoreType.DMA((NT + 1,)),
            pltpu.SemaphoreType.DMA((NI,)),
            pltpu.SemaphoreType.DMA((NI - 1,)),
            pltpu.SemaphoreType.DMA(()),
            pltpu.SemaphoreType.DMA((NT,)),
            pltpu.SemaphoreType.DMA((NT,)),
        ],
        compiler_params=pltpu.CompilerParams(vmem_limit_bytes=124 * 2**20),
    )(A_x.reshape(S, D), A_wqkv.reshape(D // GR, GR, 3 * D), A_wo,
      B_w_gate.reshape(D // GR, GR, F), B_w_up.reshape(D // GR, GR, F),
      B_w_down.reshape(F // GR, GR, D))
    return out.reshape(B, S, D)
```
